```python
import jax
import jax.numpy as jnp

def _softmax(x, axis=-1):
    return jax.nn.softmax(x, axis=axis)

def _gelu(x):
    return jax.nn.gelu(x, approximate=True)

def _silu(x):
    return jax.nn.silu(x)

def _sigmoid(x):
    return jax.nn.sigmoid(x)

def _layernorm(x, axis=-1, eps=1e-05):
    m = jnp.mean(x, axis=axis, keepdims=True)
    v = jnp.var(x, axis=axis, keepdims=True)
    return (x - m) / jnp.sqrt(v + eps)

def _scatter_add(tgt, idx, src, axis=0):
    return tgt.at[idx].add(src)

def _segment_sum(src, seg, n):
    return jax.ops.segment_sum(src, seg, n)

class _Rng:

    def __init__(self, key):
        self._k = key

    def _next(self):
        self._k, sub = jax.random.split(self._k)
        return sub

    def normal(self, shape):
        return jax.random.normal(self._next(), shape, dtype=jnp.bfloat16)

    def randint(self, lo, hi, shape):
        return jax.random.randint(self._next(), shape, lo, hi, dtype=jnp.int32)

    def uniform(self, shape, lo=0.0, hi=1.0):
        return jax.random.uniform(self._next(), shape, jnp.bfloat16, lo, hi)

    def permutation(self, n):
        return jax.random.permutation(self._next(), n)
kernel_name = 'adaLN_cond__ssm_conv_h3__mixer_gmlp__prompt'

def setup_inputs():
    _rng = _Rng(jax.random.key(int.from_bytes(__import__("os").urandom(4), "little")))
    _w = lambda a: (lambda t: t.astype(jnp.bfloat16) if jnp.issubdtype(t.dtype, jnp.floating) else t)(jnp.asarray(a))

    def _A_setup():
        B, S, D = (1, 2048, 640)
        ks = 4
        return {'q': _w((lambda *s: _rng.normal(s) * 0.05)(B, S, D)), 'k': _w((lambda *s: _rng.normal(s) * 0.05)(B, S, D)), 'v': _w((lambda *s: _rng.normal(s) * 0.05)(B, S, D)), 'shift_k': _w((lambda *s: _rng.normal(s) * 0.05)(D, ks) * 0.5), 'ssm_k': _w((lambda *s: _rng.normal(s) * 0.05)(D, S) * (1.0 / S ** 0.5)), 'ssm_D': _w((lambda *s: _rng.normal(s) * 0.05)(D))}
    _A_in = _A_setup()

    def _B_setup():
        B, S, D, F = (1, 2048, 640, 1728)
        Fh = F // 2
        return {'x': _w((lambda *s: _rng.normal(s) * 0.05)(B, S, D)), 'w_in': _w((lambda *s: _rng.normal(s) * 0.05)(D, 2 * Fh)), 'w_sp': _w(0.01 * (lambda *s: _rng.normal(s) * 0.05)(S, S)), 'b_sp': _w(1.0 + 0.01 * (lambda *s: _rng.normal(s) * 0.05)(S)), 'w_out': _w((lambda *s: _rng.normal(s) * 0.05)(Fh, D))}
    _B_in = _B_setup()
    return {'A_q': _A_in['q'], 'A_k': _A_in['k'], 'A_v': _A_in['v'], 'A_shift_k': _A_in['shift_k'], 'A_ssm_k': _A_in['ssm_k'], 'A_ssm_D': _A_in['ssm_D'], 'B_x': _B_in['x'], 'B_w_in': _B_in['w_in'], 'B_w_sp': _B_in['w_sp'], 'B_b_sp': _B_in['b_sp'], 'B_w_out': _B_in['w_out'], 'c': _w((lambda *s: _rng.normal(s) * 0.05)(1, 640)), 'w_mod': _w((lambda *s: _rng.normal(s) * 0.05)(640, 6 * 640) * 640 ** (-0.5))}

def reference(A_q, A_k, A_v, A_shift_k, A_ssm_k, A_ssm_D, B_x, B_w_in, B_w_sp, B_b_sp, B_w_out, c, w_mod):

    def _A_ref(q, k, v, shift_k, ssm_k, ssm_D):
        B, S, D = q.shape
        ks = shift_k.shape[-1]
        k_pad = jnp.pad(k, ((0, 0), (ks - 1, 0), (0, 0)))
        k_shift = jnp.zeros_like(k)
        for t in range(ks):
            k_shift = k_shift + k_pad[:, t:t + S, :] * shift_k[:, ks - 1 - t][None, None, :]
        kv = k_shift * v
        L = 2 * S
        kv_pad = jnp.pad(kv, ((0, 0), (0, S), (0, 0)))
        kf_pad = jnp.pad(ssm_k, ((0, 0), (0, S)))
        kv_f = (lambda x, axes=(-2, -1): jnp.fft.rfft2(x.astype(jnp.float32), axes=axes))(kv_pad[:, None, :, :], axes=(1, 2))
        kf_f = (lambda x, axes=(-2, -1): jnp.fft.rfft2(x.astype(jnp.float32), axes=axes))(kf_pad[:, None, :], axes=(1, 2))
        kf_f = (lambda x, *d: x.transpose(*d))(kf_f, 1, 2, 0)
        y_f = kv_f * kf_f[None, :, :, :]
        y = (lambda x, s, axes=(-2, -1): jnp.fft.irfft2(x, s=s, axes=axes).astype(jnp.bfloat16))(y_f, (1, L), axes=(1, 2))[:, 0, :S, :]
        y = y + kv * ssm_D[None, None, :]
        return q * y

    def _B_ref(x, w_in, w_sp, b_sp, w_out):
        B, S, D = x.shape
        F = w_in.shape[-1]
        Fh = F // 2
        z = _gelu(jnp.einsum('bsd,df->bsf', x, w_in))
        z1 = z[..., :Fh].copy()
        z2 = _layernorm(z[..., Fh:], axis=-1)
        g = jnp.einsum('ts,bsf->btf', w_sp, z2) + b_sp[None, :, None]
        return jnp.einsum('bsf,fd->bsd', z1 * g, w_out)
    x = A_q
    mod = (_silu(c) @ w_mod).reshape(c.shape[0], 6, 1, -1)
    sa, ca, ga, sb, cb, gb = (mod[:, 0].copy(), mod[:, 1].copy(), mod[:, 2].copy(), mod[:, 3].copy(), mod[:, 4].copy(), mod[:, 5].copy())
    h = _layernorm(x, axis=-1) * (1 + ca) + sa
    x = x + ga * _A_ref(h, A_k, A_v, A_shift_k, A_ssm_k, A_ssm_D)
    h = _layernorm(x, axis=-1) * (1 + cb) + sb
    x = x + gb * _B_ref(h, B_w_in, B_w_sp, B_b_sp, B_w_out)
    return x
```

```python
import functools
import math

import jax
import jax.numpy as jnp
import numpy as np
from jax import lax
from jax.experimental import pallas as pl
from jax.experimental.pallas import tpu as pltpu

S, D, FH = 2048, 640, 864
C = 128
NC = S // C
CB = 128
NCB = D // CB
EPS = 1e-5
F32, BF16, U32 = jnp.float32, jnp.bfloat16, jnp.uint32
NT = (((1,), (1,)), ((), ()))


def _dft_matrices():
    g = np.arange(C, dtype=np.int64)[:, None]
    n = np.arange(C, dtype=np.int64)[None, :]
    th = 2.0 * np.pi * ((n * (4 * g + 1)) % (4 * C)) / (4 * C)
    f = np.concatenate([np.cos(th), -np.sin(th)], axis=0)
    return f.T.astype(BF16), (f / C).astype(BF16)


_FWD, _INV = _dft_matrices()


def _tree_sum(xs):
    xs = list(xs)
    while len(xs) > 1:
        xs = [xs[i] + xs[i + 1] if i + 1 < len(xs) else xs[i] for i in range(0, len(xs), 2)]
    return xs[0]


def make(T1=256, T2=256, RG=32, scopes=False, flags=None, skew=2, kara=False, prio=0, staged=False):
    NT1, NT2 = S // T1, S // T2

    def scope(name):
        import contextlib
        return jax.named_scope(name) if scopes else contextlib.nullcontext()

    def kernel(q_hbm, k_hbm, v_hbm, shift_hbm, ssmk_hbm, ssmd_hbm, win_hbm, wsp_hbm, bsp_hbm,
               wout_hbm, c_hbm, wmod_hbm, fwd_hbm, inv_hbm, out_hbm,
               q_s, k_s, v_s, shift_s, ssmk_s, ssmd_s, bspf_s, wsp_s, bsp_s, wout_s, c_s, wmod_s,
               fwd_s, inv_s, taps_s, kf_s, dsk_s, fwd_u, inv_u, kvt_s, yt_s, y_s, mod_s, wint_s, woutt_s,
               x_s, h0_s, h1_s, z2f_s, z1_s, z2_s, m0_s, m1_s, o_s,
               sem_in, sem_out):
        o_conv, o_big, o_q, o_wsp = 6, 6 + 3 * NCB, 9 + 3 * NCB, 9 + 3 * NCB + NT1
        small = [pltpu.make_async_copy(a, b, sem_in.at[i]) for i, (a, b) in enumerate(
            [(fwd_hbm, fwd_s), (inv_hbm, inv_s), (shift_hbm, shift_s), (ssmd_hbm, ssmd_s),
             (c_hbm, c_s), (bsp_hbm, bsp_s)])]

        def kv_copies(b):
            ch = pl.ds(pl.multiple_of(b * CB, CB), CB)
            return [pltpu.make_async_copy(k_hbm.at[:, ch], k_s.at[b], sem_in.at[o_conv + 3 * b + 1]),
                    pltpu.make_async_copy(v_hbm.at[:, ch], v_s.at[b], sem_in.at[o_conv + 3 * b + 2])]

        def ssmk_copy(b):
            r = pl.ds(pl.multiple_of(b * S, S), S)
            return pltpu.make_async_copy(ssmk_hbm.at[r, :], ssmk_s.at[r, :], sem_in.at[o_conv + 3 * b])

        cp_wmod = pltpu.make_async_copy(wmod_hbm, wmod_s, sem_in.at[o_big + 0])
        cp_win = [pltpu.make_async_copy(win_hbm.at[:, pl.ds(j * CB, CB)], wint_s.bitcast(BF16).at[j], sem_in.at[o_big + 1]) for j in range(NCB)]
        cp_wout = pltpu.make_async_copy(wout_hbm, wout_s, sem_in.at[o_big + 2])

        def q_copy(t):
            r = pl.ds(t * T1, T1)
            return pltpu.make_async_copy(q_hbm.at[r, :], q_s.at[r, :], sem_in.at[o_q + t])

        def wsp_copy(t):
            r = pl.ds(t * T2, T2)
            return pltpu.make_async_copy(wsp_hbm.at[r, :], wsp_s.at[r, :], sem_in.at[o_wsp + t])

        def out_copy(t):
            r = pl.ds(t * T2, T2)
            return pltpu.make_async_copy(o_s.at[r, :], out_hbm.at[r, :], sem_out.at[t])

        for cp in small:
            cp.start(priority=prio)
        for cp in kv_copies(0):
            cp.start(priority=prio)
        for b in range(NCB):
            ssmk_copy(b).start(priority=prio)
            if b + 1 < NCB:
                for cp in kv_copies(b + 1):
                    cp.start(priority=prio)
        cp_wmod.start(priority=prio)
        q_copy(0).start(priority=prio)
        for cp in cp_win:
            cp.start(priority=prio)
        def late():
            for t in range(1, NT1):
                q_copy(t).start(priority=prio)
            for t in range(NT2):
                wsp_copy(t).start(priority=prio)
            cp_wout.start(priority=prio)
        if not staged:
            late()

        def packed(x):
            return pltpu.bitcast(x.astype(BF16), U32)

        def bf(ref):
            return pltpu.bitcast(ref[...], BF16)

        def kv_tile(b, j):
            kc = k_s[b, j * C:(j + 1) * C, :].astype(F32)
            kf_s[j * C + 8:(j + 1) * C + 8, :] = kc
            acc = kc * taps_s[b, 0:1, :]
            for t in range(1, 4):
                acc = acc + kf_s[j * C + 8 - t:(j + 1) * C + 8 - t, :] * taps_s[b, t:t + 1, :]
            kv = (acc * v_s[b, j * C:(j + 1) * C, :].astype(F32)).astype(BF16)
            kvt_s[:, j] = kv.T.reshape(CB // 8, 8, C)

        def causal(u, w):
            n = len(u)
            if kara and n == NC:
                e, o = causal(u[0::2], w[0::2]), causal(u[1::2], w[1::2])
                m = causal([p + q for p, q in zip(u[0::2], u[1::2])],
                           [p + q for p, q in zip(w[0::2], w[1::2])])
                out = []
                for i in range(n // 2):
                    out += [e[i] + o[i - 1] if i else e[i], m[i] - e[i] - o[i]]
                return out
            return [_tree_sum([u[j] * w[i - j] for j in range(i + 1)]) for i in range(n)]

        def forward(b, g):
            kl = ssmk_s[pl.ds(pl.multiple_of(b * S + g * C, C), C), :]
            xl = kvt_s[g].reshape(C, C)
            return (jnp.dot(kl, bf(fwd_u), preferred_element_type=F32),
                    jnp.dot(xl, bf(fwd_u), preferred_element_type=F32))

        def product(b, g, kr, xr):
            def part(r, m, c):
                return r[m * 8:(m + 1) * 8, c * C:(c + 1) * C]
            dsk = dsk_s[pl.ds(pl.multiple_of(b * CB + g * 8, 8), 8), :]
            cc = [part(kr, m, 0) - part(kr, m - 1, 1) if m else part(kr, m, 0) + dsk for m in range(NC)]
            p1 = causal([part(xr, j, 0) for j in range(NC)], cc)
            dd = [part(kr, m, 1) + part(kr, m - 1, 0) if m else part(kr, m, 1) for m in range(NC)]
            p2 = causal([part(xr, j, 1) for j in range(NC)], dd)
            re = [p1[i] - p2[i] for i in range(NC)]
            ss = [p1[i] + p2[i] for i in range(NC)]
            p3 = causal([part(xr, j, 0) + part(xr, j, 1) for j in range(NC)],
                        [cc[m] + dd[m] for m in range(NC)])
            return jnp.concatenate([jnp.concatenate([re[i], p3[i] - ss[i]], axis=1)
                                    for i in range(NC)], axis=0).astype(BF16)

        def inverse(b, g, z):
            y = jnp.dot(z, bf(inv_u), preferred_element_type=F32)
            rows = pl.ds(pl.multiple_of(b * CB + g * 8, 8), 8)
            for i in range(NC):
                yt_s[i, rows, :] = y[i * 8:(i + 1) * 8]

        def conv_block(b, prep_next):
            ng = CB // 8
            f = {g: forward(b, g) for g in range(skew)}
            for g in range(ng):
                if g + skew < ng:
                    f[g + skew] = forward(b, g + skew)
                if g not in f:
                    f[g] = forward(b, g)
                inverse(b, g, product(b, g, *f.pop(g)))
            if prep_next:
                for j in range(NC):
                    kv_tile(b + 1, j)

        with scope("p0_wait0"):
            for cp in small:
                cp.wait()
            tp = shift_s[...].astype(F32)
            dsk = ssmd_s[...].astype(F32)
            for b in range(NCB):
                taps_s[b, 0:4, :] = tp[:, b * CB:(b + 1) * CB]
                dsk_s[b * CB:(b + 1) * CB, :] = jnp.broadcast_to(dsk[b:b + 1], (CB, CB)).T
            bspf_s[...] = bsp_s[...].astype(F32)
            kf_s[0:8, :] = jnp.zeros((8, CB), F32)
            fwd_u[...] = pltpu.bitcast(fwd_s[...], jnp.uint32)
            inv_u[...] = pltpu.bitcast(inv_s[...], jnp.uint32)
            for cp in kv_copies(0):
                cp.wait()

        with scope("p0_pro"):
            for j in range(NC):
                kv_tile(0, j)

        with scope("p0_main"):
            @pl.loop(0, NCB - 1)
            def _(b):
                ssmk_copy(b).wait()
                for cp in kv_copies(b + 1):
                    cp.wait()
                conv_block(b, True)

        with scope("p0_epi"):
            ssmk_copy(NCB - 1).wait()
            conv_block(NCB - 1, False)

        with scope("mod_wait"):
            cp_wmod.wait()
        with scope("mod"):
            cf = c_s[...].astype(F32)
            sc = (cf * jax.nn.sigmoid(cf)).astype(BF16)
            mod = jnp.dot(jnp.broadcast_to(sc, (16, D)), wmod_s[...], preferred_element_type=F32)[0:8]
            sa, ca, ga, sb, cb_, gb = (mod[:, i * D:(i + 1) * D] for i in range(6))
            mod_s[0] = ga * (1.0 + ca)
            mod_s[1] = ga * sa
            mod_s[2] = 1.0 + cb_
            mod_s[3] = sb
            mod_s[4] = 0.5 * gb
        with scope("win_wait"):
            for cp in cp_win:
                cp.wait()
            if staged:
                late()
        def row(i, n):
            v = mod_s[i]
            return jnp.concatenate([v] * (n // 8), axis=0)

        def elementwise(t, h_ref):
            for i in range(T1 // C):
                y_s[i * C:(i + 1) * C, :] = yt_s[t * (T1 // C) + i].T
            for r in range(T1 // RG):
                rows = pl.ds(pl.multiple_of(t * T1 + r * RG, RG), RG)
                q = q_s[rows, :].astype(F32)
                y = y_s[r * RG:(r + 1) * RG, :]
                qc = q - jnp.sum(q, axis=-1, keepdims=True) * (1.0 / D)
                rs = lax.rsqrt(jnp.sum(qc * qc, axis=-1, keepdims=True) * (1.0 / D) + EPS)
                x = q + (qc * rs * row(0, RG) + row(1, RG)) * y
                x_s[rows, :] = x
                xc = x - jnp.sum(x, axis=-1, keepdims=True) * (1.0 / D)
                rs = lax.rsqrt(jnp.sum(xc * xc, axis=-1, keepdims=True) * (1.0 / D) + EPS)
                h_ref[r * RG // 2:(r + 1) * RG // 2, :] = packed(xc * rs * row(2, RG) + row(3, RG))

        c1 = math.sqrt(2.0 / math.pi)
        c2 = c1 * 0.044715

        def gelu2(x):
            return x * jnp.tanh((x * x * c2 + c1) * x) + x

        def win_rows(i):
            return jnp.concatenate([pltpu.bitcast(wint_s[j, i * FH // 2:(i + 1) * FH // 2, :], BF16) for j in range(NCB)], axis=1)

        def proj_in(t, h_ref):
            h = bf(h_ref)
            z2 = gelu2(lax.dot_general(win_rows(1), h, NT, preferred_element_type=F32))
            z2f_s[...] = z2
            mean = jnp.sum(z2, axis=0, keepdims=True) * (1.0 / FH)
            z1 = gelu2(lax.dot_general(win_rows(0), h, NT, preferred_element_type=F32))
            z1_s[t] = packed(z1)
            zc = z2f_s[...] - mean
            rs = lax.rsqrt(jnp.sum(zc * zc, axis=0, keepdims=True) * (1.0 / FH) + 4.0 * EPS)
            z2_s[t] = packed((z2f_s[...] - mean) * rs)

        with scope("p1_pro"):
            q_copy(0).wait()
            elementwise(0, h0_s)

        with scope("p1_main"):
            @pl.loop(0, NT1)
            def _(t):
                @pl.when(t + 1 < NT1)
                def _():
                    q_copy(t + 1).wait()
                proj_in(t, h0_s)
                elementwise(jnp.minimum(t + 1, NT1 - 1), h0_s)

        with scope("wout_t"):
            cp_wout.wait()
            for j in range(FH // 128):
                woutt_s[:, j * 128:(j + 1) * 128] = pltpu.bitcast(wout_s[j * 128:(j + 1) * 128, :].T, U32)
            woutt_s[:, 768:FH] = pltpu.bitcast(wout_s[FH - 128:FH, :].T, U32)[:, 32:]

        def z1_block(t):
            if T2 < T1:
                n = T1 // T2
                return pltpu.bitcast(z1_s[t // n, :, pl.ds(pl.multiple_of((t % n) * T2, T2), T2)], BF16)
            if T2 == T1:
                return bf(z1_s.at[t])
            n = T2 // T1
            return jnp.concatenate([bf(z1_s.at[t * n + i]) for i in range(n)], axis=1)

        def spatial(t, m_ref):
            r0 = pl.multiple_of(t * T2, T2)
            z2 = jnp.concatenate([bf(z2_s.at[i]) for i in range(NT1)], axis=1)
            g = lax.dot_general(z2, wsp_s[pl.ds(r0, T2), :], NT, preferred_element_type=F32)
            g = g + jnp.concatenate([bspf_s[pl.ds(t * (T2 // C) + i, 1), :] for i in range(T2 // C)], axis=1)
            m_ref[...] = packed(z1_block(t).astype(F32) * g)

        def proj_out(t, m_ref):
            rows = pl.ds(pl.multiple_of(t * T2, T2), T2)
            o = jnp.dot(bf(woutt_s), bf(m_ref), preferred_element_type=F32)
            o_s[rows, :] = (x_s[rows, :] + row(4, T2) * o.T).astype(BF16)

        with scope("p2_main"):
            @pl.loop(0, NT2 // 2)
            def _(u):
                t = 2 * u
                wsp_copy(t).wait()
                wsp_copy(t + 1).wait()
                spatial(t, m0_s)
                spatial(t + 1, m1_s)
                proj_out(t, m0_s)
                proj_out(t + 1, m1_s)
                out_copy(t).start()
                out_copy(t + 1).start()

        with scope("out_wait"):
            for t in range(NT2):
                out_copy(t).wait()

    vm = pltpu.VMEM
    scratch = [
        vm((S, D), BF16), vm((NCB, S, CB), BF16), vm((NCB, S, CB), BF16), vm((4, D), BF16),
        vm((NCB * S, C), BF16), vm((NCB, CB), BF16), vm((NC, C), F32), vm((S, S), BF16),
        vm((NC, C), BF16), vm((FH, D), BF16), vm((1, D), BF16), vm((D, 6 * D), BF16),
        vm((C, 2 * C), BF16), vm((2 * C, C), BF16), vm((NCB, 8, CB), F32), vm((S + 8, CB), F32),
        vm((D, CB), F32), vm((C // 2, 2 * C), jnp.uint32), vm((C, C), jnp.uint32),
    ] + [vm((CB // 8, NC, 8, C), BF16)] + [
        vm((NC, D, C), F32), vm((T1, D), F32), vm((5, 8, D), F32), vm((NCB, FH, CB), U32), vm((D // 2, FH), U32),
        vm((S, D), F32), vm((T1 // 2, D), U32), vm((T1 // 2, D), U32), vm((FH, T1), F32),
        vm((NT1, FH // 2, T1), U32), vm((NT1, FH // 2, T1), U32), vm((FH // 2, T2), U32), vm((FH // 2, T2), U32),
        vm((S, D), BF16),
        pltpu.SemaphoreType.DMA((9 + 3 * NCB + NT1 + NT2,)), pltpu.SemaphoreType.DMA((NT2,)),
    ]

    @jax.jit
    def fn(A_q, A_k, A_v, A_shift_k, A_ssm_k, A_ssm_D, B_x, B_w_in, B_w_sp, B_b_sp, B_w_out, c, w_mod):
        del B_x
        out = pl.pallas_call(
            kernel,
            out_shape=jax.ShapeDtypeStruct((S, D), BF16),
            in_specs=[pl.BlockSpec(memory_space=pltpu.HBM)] * 14,
            out_specs=pl.BlockSpec(memory_space=pltpu.HBM),
            scratch_shapes=scratch,
            compiler_params=pltpu.CompilerParams(vmem_limit_bytes=110 * 2**20, flags=flags),
        )(A_q.reshape(S, D), A_k.reshape(S, D), A_v.reshape(S, D), A_shift_k.T, A_ssm_k.reshape(D // 8, 8, NC, C).transpose(0, 2, 1, 3).reshape(NCB * S, C),
          A_ssm_D.reshape(NCB, CB), B_w_in.T, B_w_sp, B_b_sp.reshape(NC, C), B_w_out, c, w_mod, _FWD, _INV)
        return out.reshape(1, S, D)

    return fn


pallas_adaLN_cond__ssm_conv_h3__mixer_gmlp__prompt_kernel = make()
```

```python
import contextlib
import math

import jax
import jax.numpy as jnp
import numpy as np
from jax import lax
from jax.experimental import pallas as pl
from jax.experimental.pallas import tpu as pltpu

S, D, FH = 2048, 640, 864
C = 128
NC = S // C
CB = 128
NCB = D // CB
NG = CB // 8
FP = 896
EPS = 1e-5
F32, BF16, U32 = jnp.float32, jnp.bfloat16, jnp.uint32
NT = (((1,), (1,)), ((), ()))


def _dft_matrices():
    g = np.arange(C, dtype=np.int64)[:, None]
    n = np.arange(C, dtype=np.int64)[None, :]
    th = 2.0 * np.pi * ((n * (4 * g + 1)) % (4 * C)) / (4 * C)
    f = np.concatenate([np.cos(th), -np.sin(th)], axis=0)
    return f.T.astype(BF16), (f / C).astype(BF16)


_FWD, _INV = _dft_matrices()


def _tree_sum(xs):
    xs = list(xs)
    while len(xs) > 1:
        xs = [xs[i] + xs[i + 1] if i + 1 < len(xs) else xs[i] for i in range(0, len(xs), 2)]
    return xs[0]


def _quads(x, n):
    h = n // 2
    return [{(i, j): x[i + a * h, j + b * h] for i in range(h) for j in range(h)}
            for a in range(2) for b in range(2)]


def _add(x, y):
    return {k: y[k] if x[k] is None else x[k] if y[k] is None else x[k] + y[k] for k in x}


def _sub(x, y):
    return {k: x[k] if y[k] is None else -y[k] if x[k] is None else x[k] - y[k] for k in x}


def _lhs_operands(a, n):
    a11, a12, a21, a22 = _quads(a, n)
    return [_add(a21, a22), _add(a11, a12), _add(a11, a22), a22, _sub(a12, a22), a11, _sub(a21, a11)]


def _strassen(operand, b, n, rec):
    b11, b12, b21, b22 = _quads(b, n)
    m2, m5 = rec(operand(0), b11), rec(operand(1), b22)
    m1 = rec(operand(2), _add(b11, b22))
    m4 = rec(operand(3), _sub(b21, b11))
    m7 = rec(operand(4), _add(b21, b22))
    c11 = _add(_add(_sub(m1, m5), m4), m7)
    c21 = _add(m2, m4)
    m3 = rec(operand(5), _sub(b12, b22))
    m6 = rec(operand(6), _add(b11, b12))
    c12 = _add(m3, m5)
    c22 = _add(_add(_sub(m1, m2), m3), m6)
    h, out = n // 2, {}
    for (p, q), c in zip([(0, 0), (0, 1), (1, 0), (1, 1)], [c11, c12, c21, c22]):
        out.update({(i + p * h, j + q * h): v for (i, j), v in c.items()})
    return out


def _assemble(blocks, n):
    return jnp.concatenate([jnp.concatenate([blocks[i, j] for j in range(n)], axis=1)
                            for i in range(n)], axis=0)


def make(T1=256, TB=512, TO=256, RG=32, scopes=False, flags=None, skew=2, N1=16, NA=5, gelu_late=True):
    NT1 = S // T1
    HF, HS, HT = FH // 4, 128, TB // 4
    SB = 4 * HS
    NSB = S // SB
    ND = NC - N1

    def scope(name):
        return jax.named_scope(name) if scopes else contextlib.nullcontext()

    def kernel(q_hbm, k_hbm, v_hbm, shift_hbm, ssmk_hbm, ssmd_hbm, win_hbm, wsp_hbm, bsp_hbm,
               wout_hbm, c_hbm, wmod_hbm, fwd_hbm, inv_hbm, out_hbm,
               q_s, k_s, v_s, shift_s, ssmk_s, ssmd_s, wint_s, wsp_s, bsp_s, wout_s, c_s, wmod_s,
               wgate_s, fwd_s, inv_s,
               taps_s, kf_s, dsk_s, bspf_s, sc_s, fwd_u, inv_u, kvt_s, keep_s, yt_s, y_s, acc_s, mod_s,
               woutt_s, x_s, h_s, st_s, z2f_s, z1_s, z2_s, o_s, sem_in, sem_out):
        o_conv = 6
        o_big = o_conv + 4 * NCB
        o_q = o_big + 4
        o_wsp = o_q + NT1

        def copy(src, dst, i):
            return pltpu.make_async_copy(src, dst, sem_in.at[i])

        small = [copy(a, b, i) for i, (a, b) in enumerate(
            [(shift_hbm, shift_s), (ssmd_hbm, ssmd_s), (fwd_hbm, fwd_s), (inv_hbm, inv_s),
             (c_hbm, c_s), (bsp_hbm, bsp_s)])]

        def kv_copies(b):
            ch = pl.ds(pl.multiple_of(b * CB, CB), CB)
            return [copy(k_hbm.at[:, ch], k_s.at[b], o_conv + 4 * b),
                    copy(v_hbm.at[:, ch], v_s.at[b], o_conv + 4 * b + 1)]

        def ssmk_copy(b):
            r = pl.ds(pl.multiple_of(b * S, S), S)
            return copy(ssmk_hbm.at[r, :], ssmk_s.at[r, :], o_conv + 4 * b + 2)

        def wmod_copy(b):
            r = pl.ds(pl.multiple_of(b * CB, CB), CB)
            return copy(wmod_hbm.at[r, pl.ds(0, 5 * D)], wmod_s.at[b], o_conv + 4 * b + 3)

        def win_copies(i):
            return [copy(win_hbm.at[pl.ds(i * FH, FH), pl.ds(j * CB, CB)],
                         wint_s.bitcast(BF16).at[i, j], o_big + i) for j in range(NCB)]

        cp_wout = copy(wout_hbm, wout_s.at[pl.ds(0, FH), :], o_big + 2)
        cp_wgate = copy(wmod_hbm.at[:, pl.ds(5 * D, D)], wgate_s, o_big + 3)

        def q_copy(t):
            r = pl.ds(pl.multiple_of(t * T1, T1), T1)
            return copy(q_hbm.at[r, :], q_s.at[r, :], o_q + t)

        def wsp_copy(u):
            r = pl.ds(pl.multiple_of(u * TB, TB), TB)
            return copy(wsp_hbm.at[r, :], wsp_s.at[r, :], o_wsp + u)

        def out_copy(t):
            r = pl.ds(pl.multiple_of(t * TO, TO), TO)
            return pltpu.make_async_copy(o_s.at[r, :], out_hbm.at[r, :], sem_out.at[t])

        for cp in small[:1] + kv_copies(0) + small[1:]:
            cp.start()
        for b in range(NCB):
            ssmk_copy(b).start()
            if b + 1 < NCB:
                for cp in kv_copies(b + 1):
                    cp.start()
            wmod_copy(b).start()
        for cp in [q_copy(0)] + win_copies(1) + [q_copy(1)] + win_copies(0):
            cp.start()
        for t in range(2, NT1):
            q_copy(t).start()
        cp_wout.start()
        cp_wgate.start()
        for u in range(S // TB):
            wsp_copy(u).start()

        def bf(ref):
            return pltpu.bitcast(ref[...], BF16)

        def kv_tile(b, j):
            kc = k_s[b, j * C:(j + 1) * C, :].astype(F32)
            kf_s[j * C + 8:(j + 1) * C + 8, :] = kc
            acc = kc * taps_s[b, 0:1, :]
            for t in range(1, 4):
                acc = acc + kf_s[j * C + 8 - t:(j + 1) * C + 8 - t, :] * taps_s[b, t:t + 1, :]
            kv = (acc * v_s[b, j * C:(j + 1) * C, :].astype(F32)).astype(BF16)
            kvt_s[j] = pltpu.bitcast(kv.T, U32)

        def forward(b, g):
            kl = ssmk_s[pl.ds(pl.multiple_of(b * S + g * C, C), C), :]
            xl = jnp.concatenate([kvt_s[m, g * 4:(g + 1) * 4, :] for m in range(NC)], axis=0)
            return (jnp.dot(kl, bf(fwd_u), preferred_element_type=F32),
                    jnp.dot(pltpu.bitcast(xl, BF16), bf(fwd_u), preferred_element_type=F32))

        def convolve(aa, bb, cc, dd, outs):
            def causal(u, w):
                return [_tree_sum([u[j] * w[i - j] for j in range(i + 1)]) for i in outs]
            n = outs[-1] + 1
            p1, p2 = causal(aa, cc), causal(bb, dd)
            p3 = causal([aa[j] + bb[j] for j in range(n)], [cc[j] + dd[j] for j in range(n)])
            return jnp.concatenate([jnp.concatenate([p - q, r - (p + q)], axis=1)
                                    for p, q, r in zip(p1, p2, p3)], axis=0)

        def product(b, g, kr, xr):
            def part(r, m, c):
                return r[m * 8:(m + 1) * 8, c * C:(c + 1) * C]
            dsk = dsk_s[pl.ds(pl.multiple_of(b * CB + g * 8, 8), 8), :]
            cc = [part(kr, m, 0) - part(kr, m - 1, 1) if m else part(kr, m, 0) + dsk for m in range(NC)]
            dd = [part(kr, m, 1) + part(kr, m - 1, 0) if m else part(kr, m, 1) for m in range(NC)]
            aa = [part(xr, j, 0) for j in range(NC)]
            bb = [part(xr, j, 1) for j in range(NC)]
            if ND:
                for i, v in enumerate((aa, bb, cc, dd)):
                    keep_s[b * NG + g, i] = jnp.concatenate(v, axis=0)
            return convolve(aa, bb, cc, dd, range(N1))

        def inverse(b, g, z, outs):
            y = jnp.dot(z.astype(BF16), bf(inv_u), preferred_element_type=F32)
            n = len(outs)
            for u in range(z.shape[0] // (8 * n)):
                rows = pl.ds(pl.multiple_of(b * CB + (g + u) * 8, 8), 8)
                for p, i in enumerate(outs):
                    yt_s[i, rows, :] = y[(u * n + p) * 8:(u * n + p + 1) * 8]

        def conv_block(b, prep_next):
            f = {g: forward(b, g) for g in range(skew)}
            for g in range(NG):
                if g + skew < NG:
                    f[g + skew] = forward(b, g + skew)
                inverse(b, g, product(b, g, *f.pop(g)), range(N1))
            if prep_next:
                for cp in kv_copies(b + 1):
                    cp.wait()
                for j in range(NC):
                    kv_tile(b + 1, j)
            wmod_copy(b).wait()
            acc_s[...] += jnp.dot(sc_s[b], wmod_s[b], preferred_element_type=F32)[0:8]

        def conv_tail(b):
            outs = range(N1, NC)
            per = NC // ND
            for g0 in range(0, NG, per):
                zs = []
                for g in range(g0, g0 + per):
                    ops = [[keep_s[b * NG + g, i, m * 8:(m + 1) * 8, :] for m in range(NC)]
                           for i in range(4)]
                    zs.append(convolve(*ops, outs))
                inverse(b, g0, jnp.concatenate(zs, axis=0), outs)

        with scope("p0_wait0"):
            kf_s[0:8, :] = jnp.zeros((8, CB), F32)
            acc_s[...] = jnp.zeros(acc_s.shape, F32)
            wout_s[FH:, :] = jnp.zeros((FP - FH, D), BF16)
            small[0].wait()
            tp = shift_s[...].astype(F32)
            for b in range(NCB):
                taps_s[b, 0:4, :] = tp[:, b * CB:(b + 1) * CB]
            for cp in kv_copies(0):
                cp.wait()

        with scope("p0_pro"):
            for j in range(NC):
                kv_tile(0, j)
            for cp in small[1:]:
                cp.wait()
            dsk = ssmd_s[...].astype(F32)
            cf = c_s[...].astype(F32)
            sc = jnp.broadcast_to(cf * jax.nn.sigmoid(cf), (16, D)).astype(BF16)
            for b in range(NCB):
                dsk_s[b * CB:(b + 1) * CB, :] = jnp.broadcast_to(dsk[b:b + 1], (CB, CB)).T
                sc_s[b] = sc[:, b * CB:(b + 1) * CB]
            bspf_s[...] = bsp_s[...].astype(F32)
            fwd_u[...] = pltpu.bitcast(fwd_s[...], U32)
            inv_u[...] = pltpu.bitcast(inv_s[...], U32)

        with scope("p0_main"):
            @pl.loop(0, NCB - 1)
            def _(b):
                ssmk_copy(b).wait()
                conv_block(b, True)

        with scope("p0_epi"):
            ssmk_copy(NCB - 1).wait()
            conv_block(NCB - 1, False)
            sa, ca, ga, sb, cb_ = (acc_s[:, i * D:(i + 1) * D] for i in range(5))
            mod_s[0] = ga * (1.0 + ca)
            mod_s[1] = ga * sa
            mod_s[2] = 1.0 + cb_
            mod_s[3] = sb

        def row(i, n):
            return jnp.concatenate([mod_s[i]] * (n // 8), axis=0)

        def elementwise(t):
            for r in range(T1 // RG):
                if (r * RG) % C == 0:
                    i = r * RG // C
                    y_s[i * C:(i + 1) * C, :] = yt_s[t * (T1 // C) + i].T
                rows = pl.ds(pl.multiple_of(t * T1 + r * RG, RG), RG)
                q = q_s[rows, :].astype(F32)
                y = y_s[r * RG:(r + 1) * RG, :]
                qc = q - jnp.sum(q, axis=-1, keepdims=True) * (1.0 / D)
                rs = lax.rsqrt(jnp.sum(qc * qc, axis=-1, keepdims=True) * (1.0 / D) + EPS)
                x = q + (qc * rs * row(0, RG) + row(1, RG)) * y
                x_s[rows, :] = x
                xc = x - jnp.sum(x, axis=-1, keepdims=True) * (1.0 / D)
                rs = lax.rsqrt(jnp.sum(xc * xc, axis=-1, keepdims=True) * (1.0 / D) + EPS)
                h_s[rows, :] = (xc * rs * row(2, RG) + row(3, RG)).astype(BF16)

        c1 = math.sqrt(2.0 / math.pi)
        c2 = c1 * 0.044715

        def gelu2(x):
            return x * jnp.tanh((x * x * c2 + c1) * x) + x

        def fold8(x):
            return jnp.sum(x.reshape(x.shape[0] // 8, 8, x.shape[1]), axis=0)

        def proj_in(i, t):
            w = jnp.concatenate([pltpu.bitcast(wint_s[i, j], BF16) for j in range(NCB)], axis=1)
            h = h_s[pl.ds(pl.multiple_of(t * T1, T1), T1), :]
            return lax.dot_general(w, h, NT, preferred_element_type=F32)

        def gate_branch(t):
            z2 = gelu2(proj_in(1, t))
            z2 = z2 - z2[0:1]
            z2f_s[...] = z2
            st_s[0] = fold8(z2)
            st_s[1] = fold8(z2 * z2)

        def value_branch(t):
            z1 = proj_in(0, t)
            z1_s[t] = (z1 if gelu_late else gelu2(z1)).astype(BF16)

        def normalize(t):
            mean = jnp.sum(st_s[0], axis=0, keepdims=True) * (1.0 / FH)
            var = jnp.sum(st_s[1], axis=0, keepdims=True) * (1.0 / FH) - mean * mean
            rs = lax.rsqrt(jnp.maximum(var, 0.0) + 4.0 * EPS)
            zn = (z2f_s[...] - mean) * rs
            hf, hs = FH // 2, T1 // 2
            blocks = {(i, j): zn[i * hf:(i + 1) * hf, j * hs:(j + 1) * hs]
                      for i in range(2) for j in range(2)}
            for i, a in enumerate(_lhs_operands(blocks, 2)):
                z2_s[i, t] = a[0, 0]

        with scope("p1_pro"):
            q_copy(0).wait()
            elementwise(0)
        with scope("p1_pro2"):
            for cp in win_copies(1) + [q_copy(1)]:
                cp.wait()
            gate_branch(0)
            elementwise(1)
            for cp in win_copies(0):
                cp.wait()

        def p1_step(t, tail):
            @pl.when(t + 1 < NT1)
            def _():
                q_copy(t + 1).wait()
            normalize(t - 1)
            value_branch(t - 1)
            gate_branch(t)
            if tail:
                conv_tail(t - 1)
            elementwise(jnp.minimum(t + 1, NT1 - 1))

        if ND:
            with scope("p1_mainA"):
                pl.loop(1, NCB + 1)(lambda t: p1_step(t, True))
        with scope("p1_mainB"):
            pl.loop(NCB + 1 if ND else 1, NT1)(lambda t: p1_step(t, False))

        with scope("p1_epi"):
            cp_wout.wait()
            cp_wgate.wait()
            normalize(NT1 - 1)
            value_branch(NT1 - 1)
            for j in range(FP // 128):
                woutt_s[j] = pltpu.bitcast(wout_s[j * 128:(j + 1) * 128, :].T, U32)
            sc = jnp.concatenate([sc_s[b] for b in range(NCB)], axis=1)
            mod_s[4] = 0.5 * jnp.dot(sc, wgate_s[...], preferred_element_type=F32)[0:8]

        def spatial(u):
            hs = T1 // 2
            nh = NT1 // 2

            def w_block(si, ti):
                rows = pl.ds(pl.multiple_of(u * TB + ti * HT, HT), HT)
                t0 = (si % 2) * nh
                return jnp.concatenate(
                    [wsp_s[rows, t * T1 + (si // 2) * hs:t * T1 + (si // 2 + 1) * hs]
                     for t in range(t0, t0 + nh)], axis=1).astype(F32)

            def z_operand(i):
                return {(p, q): jnp.concatenate([z2_s[i, t, p * HF:(p + 1) * HF, :]
                                                 for t in range(q * nh, (q + 1) * nh)], axis=1)
                        for p in range(2) for q in range(2)}

            def leaf(a, b):
                return {(0, 0): lax.dot_general(a[0, 0], b[0, 0], NT, preferred_element_type=F32)}

            def inner(a, b):
                ops = _lhs_operands(a, 2)
                return _strassen(lambda i: ops[i], b, 2, leaf)

            w = {(si, ti): w_block(si, ti) for si in range(4) for ti in range(4)}
            return _assemble(_strassen(z_operand, w, 4, inner), 4)

        def proj_out(u, g):
            for j in range(TB // TO):
                t = u * (TB // TO) + j
                bias = jnp.concatenate([bspf_s[pl.ds(t * (TO // C) + i, 1), :]
                                        for i in range(TO // C)], axis=1)
                if TO >= T1:
                    z1 = jnp.concatenate([z1_s[t * (TO // T1) + i] for i in range(TO // T1)], axis=1)
                else:
                    n = T1 // TO
                    z1 = z1_s[u * (TB // T1) + j // n, :, (j % n) * TO:(j % n + 1) * TO]
                z1 = z1.astype(F32)
                if gelu_late:
                    z1 = gelu2(z1)
                m = (z1 * (g[:, j * TO:(j + 1) * TO] + bias)).astype(BF16)
                m = jnp.concatenate([m, jnp.zeros((FP - FH, TO), BF16)], axis=0)
                w = jnp.concatenate([bf(woutt_s.at[i]) for i in range(FP // 128)], axis=1)
                o = jnp.dot(w, m, preferred_element_type=F32)
                rows = pl.ds(pl.multiple_of(t * TO, TO), TO)
                o_s[rows, :] = (x_s[rows, :] + row(4, TO) * o.T).astype(BF16)
                out_copy(t).start()

        with scope("p2_main"):
            @pl.loop(0, S // TB)
            def _(u):
                wsp_copy(u).wait()
                proj_out(u, spatial(u))

        with scope("out_wait"):
            for t in range(S // TO):
                out_copy(t).wait()

    vm = pltpu.VMEM
    scratch = [
        vm((S, D), BF16), vm((NCB, S, CB), BF16), vm((NCB, S, CB), BF16), vm((4, D), BF16),
        vm((NCB * S, C), BF16), vm((NCB, CB), BF16), vm((2, NCB, FH // 2, CB), U32), vm((S, S), BF16),
        vm((NC, C), BF16), vm((FP, D), BF16), vm((1, D), BF16), vm((NCB, CB, 5 * D), BF16),
        vm((D, D), BF16), vm((C, 2 * C), BF16), vm((2 * C, C), BF16),
        vm((NCB, 8, CB), F32), vm((S + 8, CB), F32), vm((D, CB), F32), vm((NC, C), F32),
        vm((NCB, 16, CB), BF16), vm((C // 2, 2 * C), U32), vm((C, C), U32), vm((NC, CB // 2, C), U32),
        vm((NCB * NG if ND else 1, 4, NC * 8, C), F32),
        vm((NC, D, C), F32), vm((T1, D), F32), vm((8, 5 * D), F32), vm((5, 8, D), F32),
        vm((FP // 128, D // 2, 128), U32), vm((S, D), F32), vm((S, D), BF16), vm((2, 8, T1), F32),
        vm((FH, T1), F32), vm((NT1, FH, T1), BF16), vm((7, NT1, FH // 2, T1 // 2), F32),
        vm((S, D), BF16),
        pltpu.SemaphoreType.DMA((10 + 4 * NCB + NT1 + S // TB,)), pltpu.SemaphoreType.DMA((S // TO,)),
    ]

    @jax.jit
    def fn(A_q, A_k, A_v, A_shift_k, A_ssm_k, A_ssm_D, B_x, B_w_in, B_w_sp, B_b_sp, B_w_out, c, w_mod):
        del B_x
        out = pl.pallas_call(
            kernel,
            out_shape=jax.ShapeDtypeStruct((S, D), BF16),
            in_specs=[pl.BlockSpec(memory_space=pltpu.HBM)] * 14,
            out_specs=pl.BlockSpec(memory_space=pltpu.HBM),
            scratch_shapes=scratch,
            compiler_params=pltpu.CompilerParams(vmem_limit_bytes=120 * 2**20, flags=flags),
        )(A_q.reshape(S, D), A_k.reshape(S, D), A_v.reshape(S, D), A_shift_k.T,
          A_ssm_k.reshape(D // 8, 8, NC, C).transpose(0, 2, 1, 3).reshape(NCB * S, C),
          A_ssm_D.reshape(NCB, CB), B_w_in.T, B_w_sp, B_b_sp.reshape(NC, C), B_w_out, c, w_mod,
          _FWD, _INV)
        return out.reshape(1, S, D)

    return fn


pallas_adaLN_cond__ssm_conv_h3__mixer_gmlp__prompt_kernel = make()
```

```python
import contextlib
import math

import jax
import jax.numpy as jnp
import numpy as np
from jax import lax
from jax.experimental import pallas as pl
from jax.experimental.pallas import tpu as pltpu

S, D, FH = 2048, 640, 864
C = 128
NC = S // C
CB = 128
NCB = D // CB
NG = CB // 8
FP = 896
KH = 3
KT = (3, 2, 3, 2, 2, 3, 3)
W_SAME = {(0, 2): (0, 2), (2, 2): (1, 2), (3, 0): (0, 3), (3, 1): (0, 4),
          (5, 0): (1, 0), (5, 1): (1, 1), (5, 2): (1, 2)}
EPS = 1e-5
F32, BF16, U32 = jnp.float32, jnp.bfloat16, jnp.uint32
NT = (((1,), (1,)), ((), ()))


L = 2 * C
NL = S // L


def _dft_matrices():
    g = np.arange(C, dtype=np.int64)[None, :]
    lane = np.arange(C, dtype=np.int64)

    def mat(samples):
        th = 2.0 * np.pi * ((samples[:, None] * (4 * g + 1)) % (4 * L)) / (4 * L)
        return [np.cos(th), -np.sin(th)]

    fwd = [m for p in range(2) for m in mat((lane % 2 ^ p) * C + lane // 2 * 2 + p)]
    inv = [m.T / L for p in range(2) for m in mat((lane + p * C // 2) % C * 2 + p)]
    return np.concatenate(fwd + inv).astype(BF16)


_DFT = _dft_matrices()


def _tree_sum(xs):
    xs = list(xs)
    while len(xs) > 1:
        xs = [xs[i] + xs[i + 1] if i + 1 < len(xs) else xs[i] for i in range(0, len(xs), 2)]
    return xs[0]


def _quads(x, n):
    h = n // 2
    return [{(i, j): x[i + a * h, j + b * h] for i in range(h) for j in range(h)}
            for a in range(2) for b in range(2)]


def _mix(x, y, sign):
    if isinstance(x, list):
        n = min(len(x), len(y))
        return ([_mix(p, q, sign) for p, q in zip(x, y)] + x[n:]
                + [q if sign > 0 else -q for q in y[n:]])
    return x + y if sign > 0 else x - y


def _add(x, y):
    return {k: _mix(x[k], y[k], 1) for k in x}


def _sub(x, y):
    return {k: _mix(x[k], y[k], -1) for k in x}


def _lhs_operands(a, n):
    a11, a12, a21, a22 = _quads(a, n)
    return [_add(a21, a22), _add(a11, a12), _add(a11, a22), a22, _sub(a12, a22), a11, _sub(a21, a11)]


def _rhs_operands(b, n):
    b11, b12, b21, b22 = _quads(b, n)
    return [b11, b22, _add(b11, b22), _sub(b11, b21), _add(b21, b22), _sub(b12, b22), _add(b11, b12)]


def _combine(products, n):
    m2, m5, m1, m4, m7, m3, m6 = products
    quads = [_add(_sub(_sub(m1, m5), m4), m7), _add(m3, m5),
             _sub(m2, m4), _add(_add(_sub(m1, m2), m3), m6)]
    h, out = n // 2, {}
    for (p, q), c in zip([(0, 0), (0, 1), (1, 0), (1, 1)], quads):
        out.update({(i + p * h, j + q * h): v for (i, j), v in c.items()})
    return out


def _strassen(a, b, n, dot):
    if n == 1:
        return {(0, 0): dot(a[0, 0], b[0, 0])}
    return _combine([_strassen(p, q, n // 2, dot)
                     for p, q in zip(_lhs_operands(a, n), _rhs_operands(b, n))], n)


def _assemble(blocks, n):
    return jnp.concatenate([jnp.concatenate([blocks[i, j] for j in range(n)], axis=1)
                            for i in range(n)], axis=0)


def make(T1=256, TB=512, TO=256, RG=32, scopes=False, flags=None, gauss=2, wait_at=8, mod_at=10, nmod=3, gelu_late=False, SO=2, TW=256):
    NT1 = S // T1
    HF, HS, HT = FH // 4, 128, TB // 4
    SB = 4 * HS
    NSB = S // SB

    def scope(name):
        return jax.named_scope(name) if scopes else contextlib.nullcontext()

    def kernel(q_hbm, k_hbm, v_hbm, shift_hbm, ssmk_hbm, ssmd_hbm, win_hbm, wsp_hbm, bsp_hbm,
               wout_hbm, c_hbm, wmod_hbm, dft_hbm, out_hbm,
               q_s, k_s, v_s, shift_s, ssmk_s, ssmd_s, wint_s, wsp_s, bsp_s, wout_s, c_s, wmod_s,
               wgate_s, dft_s,
               taps_s, dsk_s, bspf_s, sc_s, kvt_s, yt_s, y_s, acc_s, mod_s,
               woutt_s, wsum_s, x_s, h_s, st_s, z2f_s, z1_s, z2_s, o_s, sem_in, sem_out):
        o_conv = 6
        o_big = o_conv + 4 * NCB
        o_q = o_big + 4
        o_wsp = o_q + NT1
        o_wout = o_wsp + S // TB

        def copy(src, dst, i):
            return pltpu.make_async_copy(src, dst, sem_in.at[i])

        small = [copy(a, b, i) for i, (a, b) in enumerate(
            [(shift_hbm, shift_s), (ssmd_hbm, ssmd_s), (dft_hbm, dft_s.bitcast(BF16)),
             (c_hbm, c_s), (bsp_hbm, bsp_s)])]

        def kv_copies(b):
            ch = pl.ds(pl.multiple_of(b * CB, CB), CB)
            return [copy(k_hbm.at[:, ch], k_s.bitcast(BF16).at[b, pl.ds(16, S), :], o_conv + 4 * b),
                    copy(v_hbm.at[:, ch], v_s.bitcast(BF16).at[b], o_conv + 4 * b + 1)]

        def ssmk_copy(b):
            r = pl.ds(pl.multiple_of(b * S, S), S)
            return copy(ssmk_hbm.at[r, :], ssmk_s.bitcast(BF16).at[r, :], o_conv + 4 * b + 2)

        def wmod_copy(b):
            r = pl.ds(pl.multiple_of(b * CB, CB), CB)
            return copy(wmod_hbm.at[r, pl.ds(0, 5 * D)], wmod_s.at[b], o_conv + 4 * b + 3)

        def win_copies(i):
            return [copy(win_hbm.at[pl.ds(i * FH, FH), pl.ds(j * CB, CB)],
                         wint_s.bitcast(BF16).at[i, j], o_big + i) for j in range(NCB)]

        def wout_copy(j):
            return copy(wout_hbm.at[pl.ds(pl.multiple_of(j * 128, 128), 128), :], wout_s.at[j], o_wout + j)

        wout_last = copy(wout_hbm.at[pl.ds(FP - 128, FH + 128 - FP), :],
                         wout_s.at[FP // 128 - 1, pl.ds(0, FH + 128 - FP), :], o_big + 2)
        cp_wgate = copy(wmod_hbm.at[:, pl.ds(5 * D, D)], wgate_s, o_big + 3)

        def q_copy(t):
            r = pl.ds(pl.multiple_of(t * T1, T1), T1)
            return copy(q_hbm.at[r, :], q_s.at[r, :], o_q + t)

        def wsp_copy(u):
            r = pl.ds(pl.multiple_of(u * TB, TB), TB)
            return copy(wsp_hbm.at[r, :], wsp_s.at[r, :], o_wsp + u)

        def out_copy(t):
            r = pl.ds(pl.multiple_of(t * TW, TW), TW)
            return pltpu.make_async_copy(o_s.at[r, :], out_hbm.at[r, :], sem_out.at[t])

        for cp in small[:1] + kv_copies(0) + small[1:]:
            cp.start()
        for b in range(NCB):
            ssmk_copy(b).start()
            if b + 1 < NCB:
                for cp in kv_copies(b + 1):
                    cp.start()
        for b in range(NCB):
            wmod_copy(b).start()
        for cp in [q_copy(0)] + win_copies(1) + win_copies(0) + [q_copy(1)]:
            cp.start()
        for t in range(2, NT1):
            q_copy(t).start()
            wout_copy(t - 2).start()
        wout_last.start()
        cp_wgate.start()
        for u in range(S // TB):
            wsp_copy(u).start()

        def bf(ref):
            return pltpu.bitcast(ref[...], BF16)

        def dft(i, n):
            return pltpu.bitcast(dft_s[i * C // 2:(i + n) * C // 2, :], BF16)

        def low(w):
            return pltpu.bitcast(w << 16, F32)

        def high(w):
            return pltpu.bitcast(w & np.uint32(0xFFFF0000), F32)

        def kv_chunk(b, m):
            kw = [k_s[b, pl.ds(8 + m * C + j, C), :] for j in range(-2, 1)]
            vw = v_s[b, m * C:(m + 1) * C, :]
            kk = [high(kw[0]), low(kw[1]), high(kw[1]), low(kw[2]), high(kw[2])]
            for p, vv in enumerate((low(vw), high(vw))):
                kv = _tree_sum([kk[3 + p - t] * taps_s[b, t:t + 1, :] for t in range(4)]) * vv
                halves = [kv[:C // 2], kv[C // 2:]]
                w = pltpu.pack_elementwise([halves[p], halves[1 - p]], packed_dtype=BF16)
                kvt_s[2 * m + p] = pltpu.bitcast(pltpu.bitcast(w, BF16).T, U32)

        def forward(b, g):
            base = pl.multiple_of(b * (S // 2), S // 2)
            t0, t1 = [jnp.concatenate([ssmk_s[pl.ds(base + (g * NC + 2 * m + j) * 4, 4), :]
                                       for m in range(NL)], axis=0) for j in range(2)]
            odd = (lax.broadcasted_iota(jnp.int32, t0.shape, 1) & 1) == 1
            kt = [jnp.where(odd, pltpu.roll(t1, 1, 1), t0), jnp.where(odd, t0, pltpu.roll(t1, C - 1, 1))]
            out = []
            for p in range(2):
                xt = jnp.concatenate([kvt_s[2 * m + p, g * 4:(g + 1) * 4, :] for m in range(NL)], axis=0)
                lhs = jnp.concatenate([t[i:i + 8] for i in range(0, 4 * NL, 8) for t in (kt[p], xt)], axis=0)
                out.append([jnp.dot(pltpu.bitcast(lhs, BF16), dft(2 * p + c, 1), preferred_element_type=F32)
                            for c in range(2)])
            return out

        def butterfly(a, b):
            return (a[0] + b[0], a[1] + b[1]), (a[0] - b[0], a[1] - b[1])

        def product(b, g, f):
            def part(i, m, p):
                r = (m // 2 * 4 + i * 2 + m % 2) * 8
                return f[p][0][r:r + 8], f[p][1][r:r + 8]

            def window(m, p):
                re, im = part(0, m, p)
                if m:
                    pre, pim = part(0, m - 1, p)
                    return re - pim, im + pre
                if p == 0:
                    re = re + dsk_s[pl.ds(pl.multiple_of(b * CB + g * 8, 8), 8), :]
                return re, im

            kf = [butterfly(window(m, 0), window(m, 1)) for m in range(NL)]
            xf = [butterfly(part(1, m, 0), part(1, m, 1)) for m in range(NL)]
            out = []
            for i in range(NL):
                z = []
                for h in range(2):
                    terms = [(xf[j][h], kf[i - j][h]) for j in range(i + 1)]
                    if i >= gauss:
                        p1 = _tree_sum([x[0] * k[0] for x, k in terms])
                        p2 = _tree_sum([x[1] * k[1] for x, k in terms])
                        p3 = _tree_sum([(x[0] + x[1]) * (k[0] + k[1]) for x, k in terms])
                        z.append((p1 - p2, p3 - (p1 + p2)))
                    else:
                        z.append((_tree_sum([x[0] * k[0] - x[1] * k[1] for x, k in terms]),
                                  _tree_sum([x[0] * k[1] + x[1] * k[0] for x, k in terms])))
                out.append(butterfly(*z))
            return out

        def inverse(b, g, z):
            rows = pl.ds(pl.multiple_of(b * CB + g * 8, 8), 8)
            ys = []
            for p in range(2):
                zp = jnp.concatenate([jnp.concatenate([z[i][p][c] for i in range(NL)], axis=0)
                                      for c in range(2)], axis=1)
                ys.append(jnp.dot(zp.astype(BF16), dft(4 + 2 * p, 2), preferred_element_type=F32))
            first = lax.broadcasted_iota(jnp.int32, ys[0].shape, 1) < C // 2
            for j in range(2):
                y = jnp.where(first, ys[j], ys[1 - j])
                for i in range(NL):
                    yt_s[2 * i + j, rows, :] = y[i * 8:(i + 1) * 8]

        def modulation(blocks):
            for b in blocks:
                wmod_copy(b).wait()
            acc_s[...] += _tree_sum([jnp.dot(sc_s[b], wmod_s[b], preferred_element_type=F32)[0:8]
                                     for b in blocks])

        def conv_block(b, last):
            ssmk_copy(b).wait()
            f = {0: forward(b, 0)}
            for g in range(NG):
                if g + 1 < NG:
                    f[g + 1] = forward(b, g + 1)
                if g == wait_at and not last:
                    for cp in kv_copies(b + 1):
                        cp.wait()
                if g == mod_at and last:
                    modulation(range(nmod))
                inverse(b, g, product(b, g, f.pop(g)))
            if last:
                modulation(range(nmod, NCB))
            else:
                for m in range(NL):
                    kv_chunk(b + 1, m)

        with scope("p0_wait0"):
            for b in range(NCB):
                k_s[b, 0:8, :] = jnp.zeros((8, CB), U32)
            acc_s[...] = jnp.zeros(acc_s.shape, F32)
            wout_s[FP // 128 - 1, FH + 128 - FP:, :] = jnp.zeros((FP - FH, D), BF16)
            small[0].wait()
            tp = shift_s[...].astype(F32)
            for b in range(NCB):
                taps_s[b, 0:4, :] = tp[:, b * CB:(b + 1) * CB]
            for cp in kv_copies(0):
                cp.wait()

        with scope("p0_pro"):
            for m in range(NL):
                kv_chunk(0, m)
            for cp in small[1:]:
                cp.wait()
            dsk = ssmd_s[...].astype(F32)
            cf = c_s[...].astype(F32)
            sc = jnp.broadcast_to(cf * jax.nn.sigmoid(cf), (16, D)).astype(BF16)
            for b in range(NCB):
                dsk_s[b * CB:(b + 1) * CB, :] = jnp.broadcast_to(dsk[b:b + 1], (CB, CB)).T
                sc_s[b] = sc[:, b * CB:(b + 1) * CB]
            bspf_s[...] = bsp_s[...].astype(F32)

        with scope("p0_main"):
            @pl.loop(0, NCB - 1)
            def _(b):
                conv_block(b, False)

        with scope("p0_epi"):
            conv_block(NCB - 1, True)
            sa, ca, ga, sb, cb_ = (acc_s[:, i * D:(i + 1) * D] for i in range(5))
            mod_s[0] = ga * (1.0 + ca)
            mod_s[1] = ga * sa
            mod_s[2] = 1.0 + cb_
            mod_s[3] = sb

        def row(i, n):
            return jnp.concatenate([mod_s[i]] * (n // 8), axis=0)

        def elementwise(t):
            hs = []
            for r in range(T1 // RG):
                if (r * RG) % C == 0:
                    i = r * RG // C
                    y = yt_s[t * (T1 // C) + i].T
                    for p in range(2):
                        for b in range(NCB):
                            y_s[b, pl.ds(i * C + (i + p) % 2, C // 2, stride=2), :] = \
                                y[p * C // 2:(p + 1) * C // 2, b * CB:(b + 1) * CB]
                rows = pl.ds(pl.multiple_of(t * T1 + r * RG, RG), RG)
                q = q_s[rows, :].astype(F32)
                y = jnp.concatenate([y_s[b, r * RG:(r + 1) * RG, :] for b in range(NCB)], axis=1)
                qc = q - jnp.sum(q, axis=-1, keepdims=True) * (1.0 / D)
                rs = lax.rsqrt(jnp.sum(qc * qc, axis=-1, keepdims=True) * (1.0 / D) + EPS)
                x = q + (qc * rs * row(0, RG) + row(1, RG)) * y
                x_s[rows, :] = x
                xc = x - jnp.sum(x, axis=-1, keepdims=True) * (1.0 / D)
                rs = lax.rsqrt(jnp.sum(xc * xc, axis=-1, keepdims=True) * (1.0 / D) + EPS)
                hs.append(xc * rs * row(2, RG) + row(3, RG))
            return jnp.concatenate(hs, axis=0)

        def split(tiles):
            return tiles[:KH], tiles[KH:]

        def store_h(h):
            blocks = {(i, j): split([h[j * T1 // 2:(j + 1) * T1 // 2, b * CB:(b + 1) * CB]
                                     for b in range(NCB)])[i] for i in range(2) for j in range(2)}
            for i, op in enumerate(_rhs_operands(blocks, 2)):
                h_s[i, :, :KT[i] * CB] = jnp.concatenate(op[0, 0][:KT[i]], axis=1).astype(BF16)

        def store_w_in():
            blocks = {(i, j): split([bf(wint_s.at[1 - i, b]).astype(F32) for b in range(NCB)])[j]
                      for i in range(2) for j in range(2)}
            for i, op in enumerate(_lhs_operands(blocks, 2)):
                for b in range(KT[i]):
                    if (i, b) not in W_SAME:
                        wsum_s[i, b] = pltpu.bitcast(op[0, 0][b].astype(BF16), U32)

        c1 = math.sqrt(2.0 / math.pi)
        c2 = c1 * 0.044715

        def gelu2(x):
            return x * jnp.tanh((x * x * c2 + c1) * x) + x

        def fold8(x):
            return jnp.sum(x.reshape(x.shape[0] // 8, 8, x.shape[1]), axis=0)

        def proj_in_plain(i, h):
            w = jnp.concatenate([bf(wint_s.at[i, b]) for b in range(NCB)], axis=1)
            return lax.dot_general(w, h, NT, preferred_element_type=F32)

        def proj_in():
            prods = []
            for i in range(7):
                w = jnp.concatenate([bf(wint_s.at[W_SAME[i, b]] if (i, b) in W_SAME else wsum_s.at[i, b])
                                     for b in range(KT[i])], axis=1)
                prods.append({(0, 0): lax.dot_general(w, h_s[i, :, :KT[i] * CB], NT,
                                                      preferred_element_type=F32)})
            z = _combine(prods, 2)
            return [jnp.concatenate([z[i, 0], z[i, 1]], axis=1) for i in range(2)]

        def gate_branch(z):
            z = gelu2(z)
            z = z - z[0:1]
            z2f_s[...] = z
            st_s[0] = fold8(z)
            st_s[1] = fold8(z * z)

        def value_branch(t, z):
            z1_s[t] = (z if gelu_late else gelu2(z)).astype(BF16)

        def normalize(t):
            mean = jnp.sum(st_s[0], axis=0, keepdims=True) * (1.0 / FH)
            var = jnp.sum(st_s[1], axis=0, keepdims=True) * (1.0 / FH) - mean * mean
            rs = lax.rsqrt(jnp.maximum(var, 0.0) + 4.0 * EPS)
            zn = (z2f_s[...] - mean) * rs
            hf, hs = FH // 2, T1 // 2
            blocks = {(i, j): zn[i * hf:(i + 1) * hf, j * hs:(j + 1) * hs]
                      for i in range(2) for j in range(2)}
            for i, a in enumerate(_lhs_operands(blocks, 2)):
                z2_s[i, t] = a[0, 0]

        with scope("p1_pro"):
            q_copy(0).wait()
            h0 = elementwise(0).astype(BF16)
        with scope("p1_pro2"):
            for cp in win_copies(1):
                cp.wait()
            gate_branch(proj_in_plain(1, h0))
            for cp in win_copies(0) + [q_copy(1)]:
                cp.wait()
            value_branch(0, proj_in_plain(0, h0))
            store_w_in()
            store_h(elementwise(1))

        with scope("p1_main"):
            @pl.loop(1, NT1)
            def _(t):
                @pl.when(t + 1 < NT1)
                def _():
                    q_copy(t + 1).wait()

                @pl.when(t < NT1 - 1)
                def _():
                    wout_copy(t - 1).wait()

                @pl.when(t == NT1 - 1)
                def _():
                    wout_last.wait()
                normalize(t - 1)
                z2, z1 = proj_in()
                gate_branch(z2)
                value_branch(t, z1)
                store_h(elementwise(jnp.minimum(t + 1, NT1 - 1)))
                woutt_s[t - 1] = wout_s[t - 1].astype(F32).T

        with scope("p1_epi"):
            cp_wgate.wait()
            normalize(NT1 - 1)
            sc = jnp.concatenate([sc_s[b] for b in range(NCB)], axis=1)
            mod_s[4] = 0.5 * jnp.dot(sc, wgate_s[...], preferred_element_type=F32)[0:8]

        def spatial(u):
            hs = T1 // 2
            nh = NT1 // 2

            def w_block(si, ti):
                rows = pl.ds(pl.multiple_of(u * TB + ti * HT, HT), HT)
                t0 = (si % 2) * nh
                return jnp.concatenate(
                    [wsp_s[rows, t * T1 + (si // 2) * hs:t * T1 + (si // 2 + 1) * hs]
                     for t in range(t0, t0 + nh)], axis=1).astype(F32)

            def z_operand(i):
                return {(p, q): jnp.concatenate([z2_s[i, t, p * HF:(p + 1) * HF, :]
                                                 for t in range(q * nh, (q + 1) * nh)], axis=1)
                        for p in range(2) for q in range(2)}

            def dot_nt(a, b):
                return lax.dot_general(a, b, NT, preferred_element_type=F32)

            w = {(si, ti): w_block(si, ti) for si in range(4) for ti in range(4)}
            return _assemble(_combine([_strassen(z_operand(i), op, 2, dot_nt)
                                       for i, op in enumerate(_rhs_operands(w, 4))], 4), 4)

        def proj_out(u, g):
            bias = jnp.concatenate([bspf_s[pl.ds(u * (TB // C) + i, 1), :] for i in range(TB // C)], axis=1)
            z1 = jnp.concatenate([z1_s[u * (TB // T1) + i] for i in range(TB // T1)], axis=1).astype(F32)
            if gelu_late:
                z1 = gelu2(z1)
            m = jnp.concatenate([z1 * (g + bias), jnp.zeros((FP - FH, TB), F32)], axis=0)
            groups = {1: [range(7)], 2: [range(4), range(4, 7)],
                      4: [range(2), range(2, 4), range(4, 6), range(6, 7)]}[SO]
            hd, ht = D // SO, TO // SO

            def dot(a, b):
                n = min(len(a), len(b))
                return jnp.dot(jnp.concatenate(a[:n], axis=1), jnp.concatenate(b[:n], axis=0),
                               preferred_element_type=F32)

            for j in range(TB // TO):
                a = {(i, p): [woutt_s[f, i * hd:(i + 1) * hd, :] for f in groups[p]]
                     for i in range(SO) for p in range(SO)}
                b = {(p, i): [m[f * 128:(f + 1) * 128, j * TO + i * ht:j * TO + (i + 1) * ht]
                              for f in groups[p]] for i in range(SO) for p in range(SO)}
                o = _assemble(_strassen(a, b, SO, dot), SO)
                for i in range(TO // TW):
                    t = u * (TB // TW) + j * (TO // TW) + i
                    rows = pl.ds(pl.multiple_of(t * TW, TW), TW)
                    o_s[rows, :] = (x_s[rows, :] + row(4, TW) * o[:, i * TW:(i + 1) * TW].T).astype(BF16)
                    out_copy(t).start()

        with scope("p2_main"):
            @pl.loop(0, S // TB)
            def _(u):
                wsp_copy(u).wait()
                proj_out(u, spatial(u))

        with scope("out_wait"):
            for t in range(S // TW):
                out_copy(t).wait()

    vm = pltpu.VMEM
    scratch = [
        vm((S, D), BF16), vm((NCB, S // 2 + 8, CB), U32), vm((NCB, S // 2, CB), U32), vm((4, D), BF16),
        vm((NCB * S // 2, C), U32), vm((NCB, CB), BF16), vm((2, NCB, FH // 2, CB), U32), vm((S, S), BF16),
        vm((NC, C), BF16), vm((FP // 128, 128, D), BF16), vm((1, D), BF16), vm((NCB, CB, 5 * D), BF16),
        vm((D, D), BF16), vm((4 * C, C), U32),
        vm((NCB, 8, CB), F32), vm((D, CB), F32), vm((NC, C), F32),
        vm((NCB, 16, CB), BF16), vm((NC, CB // 2, C), U32),
        vm((NC, D, C), F32), vm((NCB, T1, CB), F32), vm((8, 5 * D), F32), vm((5, 8, D), F32),
        vm((FP // 128, D, 128), F32), vm((7, KH, FH // 2, CB), U32), vm((S, D), F32),
        vm((7, T1 // 2, KH * CB), BF16), vm((2, 8, T1), F32),
        vm((FH, T1), F32), vm((NT1, FH, T1), BF16), vm((7, NT1, FH // 2, T1 // 2), F32),
        vm((S, D), BF16),
        pltpu.SemaphoreType.DMA((10 + 4 * NCB + NT1 + S // TB + 6,)), pltpu.SemaphoreType.DMA((S // TW,)),
    ]

    @jax.jit
    def fn(A_q, A_k, A_v, A_shift_k, A_ssm_k, A_ssm_D, B_x, B_w_in, B_w_sp, B_b_sp, B_w_out, c, w_mod):
        del B_x
        out = pl.pallas_call(
            kernel,
            out_shape=jax.ShapeDtypeStruct((S, D), BF16),
            in_specs=[pl.BlockSpec(memory_space=pltpu.HBM)] * 13,
            out_specs=pl.BlockSpec(memory_space=pltpu.HBM),
            scratch_shapes=scratch,
            compiler_params=pltpu.CompilerParams(vmem_limit_bytes=120 * 2**20, flags=flags),
        )(A_q.reshape(S, D), A_k.reshape(S, D), A_v.reshape(S, D), A_shift_k.T,
          A_ssm_k.reshape(D // 8, 8, NC, C).transpose(0, 2, 1, 3).reshape(NCB * S, C),
          A_ssm_D.reshape(NCB, CB), B_w_in.T, B_w_sp, B_b_sp.reshape(NC, C), B_w_out, c, w_mod,
          _DFT)
        return out.reshape(1, S, D)

    return fn


pallas_adaLN_cond__ssm_conv_h3__mixer_gmlp__prompt_kernel = make()
```

```python
import contextlib
import math

import jax
import jax.numpy as jnp
import numpy as np
from jax import lax
from jax.experimental import pallas as pl
from jax.experimental.pallas import tpu as pltpu

S, D, FH = 2048, 640, 864
C = 128
NC = S // C
CB = 128
NCB = D // CB
NG = CB // 8
FP = 896
KH = 3
KT = (3, 2, 3, 2, 2, 3, 3)
W_SAME = {(0, 2): (0, 2), (2, 2): (1, 2), (3, 0): (0, 3), (3, 1): (0, 4),
          (5, 0): (1, 0), (5, 1): (1, 1), (5, 2): (1, 2)}
EPS = 1e-5
F32, BF16, U32 = jnp.float32, jnp.bfloat16, jnp.uint32
NT = (((1,), (1,)), ((), ()))


L = 2 * C
NL = S // L


def _dft_matrices():
    g = np.arange(C, dtype=np.int64)[None, :]
    lane = np.arange(C, dtype=np.int64)

    def mat(samples):
        th = 2.0 * np.pi * ((samples[:, None] * (4 * g + 1)) % (4 * L)) / (4 * L)
        return [np.cos(th), -np.sin(th)]

    fwd = [m for p in range(2) for m in mat((lane % 2 ^ p) * C + lane // 2 * 2 + p)]
    inv = [m.T / L for p in range(2) for m in mat((lane + p * C // 2) % C * 2 + p)]
    return np.concatenate(fwd + inv).astype(BF16)


_DFT = _dft_matrices()


def _tree_sum(xs):
    xs = list(xs)
    while len(xs) > 1:
        xs = [xs[i] + xs[i + 1] if i + 1 < len(xs) else xs[i] for i in range(0, len(xs), 2)]
    return xs[0]


def _quads(x, n):
    h = n // 2
    return [{(i, j): x[i + a * h, j + b * h] for i in range(h) for j in range(h)}
            for a in range(2) for b in range(2)]


def _mix(x, y, sign):
    if isinstance(x, list):
        n = min(len(x), len(y))
        return ([_mix(p, q, sign) for p, q in zip(x, y)] + x[n:]
                + [q if sign > 0 else -q for q in y[n:]])
    return x + y if sign > 0 else x - y


def _add(x, y):
    return {k: _mix(x[k], y[k], 1) for k in x}


def _sub(x, y):
    return {k: _mix(x[k], y[k], -1) for k in x}


def _lhs_operands(a, n):
    a11, a12, a21, a22 = _quads(a, n)
    return [_add(a21, a22), _add(a11, a12), _add(a11, a22), a22, _sub(a12, a22), a11, _sub(a21, a11)]


def _rhs_operands(b, n):
    b11, b12, b21, b22 = _quads(b, n)
    return [b11, b22, _add(b11, b22), _sub(b11, b21), _add(b21, b22), _sub(b12, b22), _add(b11, b12)]


def _combine(products, n):
    m2, m5, m1, m4, m7, m3, m6 = products
    quads = [_add(_sub(_sub(m1, m5), m4), m7), _add(m3, m5),
             _sub(m2, m4), _add(_add(_sub(m1, m2), m3), m6)]
    h, out = n // 2, {}
    for (p, q), c in zip([(0, 0), (0, 1), (1, 0), (1, 1)], quads):
        out.update({(i + p * h, j + q * h): v for (i, j), v in c.items()})
    return out


def _strassen(a, b, n, dot):
    if n == 1:
        return {(0, 0): dot(a[0, 0], b[0, 0])}
    return _combine([_strassen(p, q, n // 2, dot)
                     for p, q in zip(_lhs_operands(a, n), _rhs_operands(b, n))], n)


def _assemble(blocks, n):
    return jnp.concatenate([jnp.concatenate([blocks[i, j] for j in range(n)], axis=1)
                            for i in range(n)], axis=0)


def make(T1=256, TB=512, TO=512, RG=32, scopes=False, flags={'XLA_TPU_EVENLY_DISTRIBUTE_CRITICAL_NODES': True}, gauss=2, wait_at=8, mod_at=10, nmod=3, gelu_late=True, SO=2, TW=128, WR=8, RG0=64, o16=True, s16=False):
    NT1 = S // T1
    HF, HS, HT = FH // 4, 128, TB // 4
    SB = 4 * HS
    NSB = S // SB

    def scope(name):
        return jax.named_scope(name) if scopes else contextlib.nullcontext()

    def kernel(q_hbm, k_hbm, v_hbm, shift_hbm, ssmk_hbm, ssmd_hbm, win_hbm, wsp_hbm, bsp_hbm,
               wout_hbm, c_hbm, wmod_hbm, dft_hbm, out_hbm,
               q_s, k_s, v_s, shift_s, ssmk_s, ssmd_s, wint_s, wsp_s, bsp_s, wout_s, c_s, wmod_s,
               wgate_s, dft_s,
               taps_s, dsk_s, bspf_s, sc_s, kvt_s, yt_s, y_s, acc_s, mod_s,
               woutt_s, wsum_s, x_s, qn_s, h_s, st_s, z2f_s, z1_s, z2_s, o_s, sem_in, sem_out):
        o_conv = 6
        o_big = o_conv + 4 * NCB
        o_q = o_big + 4
        o_wsp = o_q + NT1
        o_wout = o_wsp + S // TB

        def copy(src, dst, i):
            return pltpu.make_async_copy(src, dst, sem_in.at[i])

        small = [copy(a, b, i) for i, (a, b) in enumerate(
            [(shift_hbm, shift_s), (ssmd_hbm, ssmd_s), (dft_hbm, dft_s.bitcast(BF16)),
             (c_hbm, c_s), (bsp_hbm, bsp_s)])]

        def kv_copies(b):
            ch = pl.ds(pl.multiple_of(b * CB, CB), CB)
            return [copy(k_hbm.at[:, ch], k_s.bitcast(BF16).at[b, pl.ds(16, S), :], o_conv + 4 * b),
                    copy(v_hbm.at[:, ch], v_s.bitcast(BF16).at[b], o_conv + 4 * b + 1)]

        def ssmk_copy(b):
            r = pl.ds(pl.multiple_of(b * S, S), S)
            return copy(ssmk_hbm.at[r, :], ssmk_s.bitcast(BF16).at[r, :], o_conv + 4 * b + 2)

        def wmod_copy(b):
            r = pl.ds(pl.multiple_of(b * CB, CB), CB)
            return copy(wmod_hbm.at[r, pl.ds(0, 5 * D)], wmod_s.at[b], o_conv + 4 * b + 3)

        def win_copies(i):
            return [copy(win_hbm.at[pl.ds(i * FH, FH), pl.ds(j * CB, CB)],
                         wint_s.bitcast(BF16).at[i, j], o_big + i) for j in range(NCB)]

        def wout_copy(j):
            return copy(wout_hbm.at[pl.ds(pl.multiple_of(j * 128, 128), 128), :], wout_s.at[j], o_wout + j)

        wout_last = copy(wout_hbm.at[pl.ds(FP - 128, FH + 128 - FP), :],
                         wout_s.at[FP // 128 - 1, pl.ds(0, FH + 128 - FP), :], o_big + 2)
        cp_wgate = copy(wmod_hbm.at[:, pl.ds(5 * D, D)], wgate_s, o_big + 3)

        def q_copy(t):
            r = pl.ds(pl.multiple_of(t * T1, T1), T1)
            return copy(q_hbm.at[r, :], q_s.at[r, :], o_q + t)

        def wsp_copy(u):
            r = pl.ds(pl.multiple_of(u * TB, TB), TB)
            return copy(wsp_hbm.at[r, :], wsp_s.at[r, :], o_wsp + u)

        def out_copy(t):
            r = pl.ds(pl.multiple_of(t * TW, TW), TW)
            return pltpu.make_async_copy(o_s.at[r, :], out_hbm.at[r, :], sem_out.at[t])

        for cp in small[:1] + kv_copies(0) + small[1:]:
            cp.start()
        for b in range(NCB):
            ssmk_copy(b).start()
            if b + 1 < NCB:
                for cp in kv_copies(b + 1):
                    cp.start()
        q_copy(0).start()
        for b in range(NCB):
            wmod_copy(b).start()
        for cp in win_copies(1) + [q_copy(1)] + win_copies(0):
            cp.start()
        for t in range(2, NT1):
            q_copy(t).start()
            wout_copy(t - 2).start()
        wout_last.start()
        cp_wgate.start()
        for u in range(S // TB):
            wsp_copy(u).start()

        def bf(ref):
            return pltpu.bitcast(ref[...], BF16)

        def dft(i, n):
            return pltpu.bitcast(dft_s[i * C // 2:(i + n) * C // 2, :], BF16)

        def low(w):
            return pltpu.bitcast(w << 16, F32)

        def high(w):
            return pltpu.bitcast(w & np.uint32(0xFFFF0000), F32)

        def kv_chunk(b, m):
            kw = [k_s[b, pl.ds(8 + m * C + j, C), :] for j in range(-2, 1)]
            vw = v_s[b, m * C:(m + 1) * C, :]
            kk = [high(kw[0]), low(kw[1]), high(kw[1]), low(kw[2]), high(kw[2])]
            for p, vv in enumerate((low(vw), high(vw))):
                kv = _tree_sum([kk[3 + p - t] * taps_s[b, t:t + 1, :] for t in range(4)]) * vv
                halves = [kv[:C // 2], kv[C // 2:]]
                w = pltpu.pack_elementwise([halves[p], halves[1 - p]], packed_dtype=BF16)
                kvt_s[(2 * m + p) * 64:(2 * m + p + 1) * 64, :] = pltpu.bitcast(pltpu.bitcast(w, BF16).T, U32)

        def forward(b, g):
            base = pl.multiple_of(b * (S // 2), S // 2) + g * NC * 4
            top = lax.broadcasted_iota(jnp.int32, (8, C), 0) < 4
            words = [ssmk_s[pl.ds(base + 4 * i, 8), :] if i % 4 < 3 else None for i in range(NC)]
            t0, t1 = [jnp.concatenate([jnp.where(top, words[i + j], words[i + j + 1])
                                       for i in range(0, NC, 4)], axis=0) for j in range(2)]
            odd = (lax.broadcasted_iota(jnp.int32, t0.shape, 1) & 1) == 1
            kt = [jnp.where(odd, pltpu.roll(t1, 1, 1), t0), jnp.where(odd, t0, pltpu.roll(t1, C - 1, 1))]
            out = []
            for p in range(2):
                xt = jnp.concatenate(
                    [jnp.where(top, kvt_s[pl.ds((2 * m + p) * 64 + 4 * g, 8), :],
                               kvt_s[pl.ds((2 * m + 2 + p) * 64 + 4 * g - 4, 8), :])
                     for m in range(0, NL, 2)], axis=0)
                lhs = jnp.concatenate([t[i:i + 8] for i in range(0, 4 * NL, 8) for t in (kt[p], xt)], axis=0)
                out.append([jnp.dot(pltpu.bitcast(lhs, BF16), dft(2 * p + c, 1), preferred_element_type=F32)
                            for c in range(2)])
            return out

        def butterfly(a, b):
            return (a[0] + b[0], a[1] + b[1]), (a[0] - b[0], a[1] - b[1])

        def product(b, g, f):
            def part(i, m, p):
                r = (m // 2 * 4 + i * 2 + m % 2) * 8
                return f[p][0][r:r + 8], f[p][1][r:r + 8]

            def window(m, p):
                re, im = part(0, m, p)
                if m:
                    pre, pim = part(0, m - 1, p)
                    return re - pim, im + pre
                if p == 0:
                    re = re + dsk_s[pl.ds(pl.multiple_of(b * CB + g * 8, 8), 8), :]
                return re, im

            kf = [butterfly(window(m, 0), window(m, 1)) for m in range(NL)]
            xf = [butterfly(part(1, m, 0), part(1, m, 1)) for m in range(NL)]
            out = []
            for i in range(NL):
                z = []
                for h in range(2):
                    terms = [(xf[j][h], kf[i - j][h]) for j in range(i + 1)]
                    if i >= gauss:
                        p1 = _tree_sum([x[0] * k[0] for x, k in terms])
                        p2 = _tree_sum([x[1] * k[1] for x, k in terms])
                        p3 = _tree_sum([(x[0] + x[1]) * (k[0] + k[1]) for x, k in terms])
                        z.append((p1 - p2, p3 - (p1 + p2)))
                    else:
                        z.append((_tree_sum([x[0] * k[0] - x[1] * k[1] for x, k in terms]),
                                  _tree_sum([x[0] * k[1] + x[1] * k[0] for x, k in terms])))
                out.append(butterfly(*z))
            return out

        def inverse(b, g, z):
            rows = pl.ds(pl.multiple_of(b * CB + g * 8, 8), 8)
            ys = []
            for p in range(2):
                zp = jnp.concatenate([jnp.concatenate([z[i][p][c] for i in range(NL)], axis=0)
                                      for c in range(2)], axis=1)
                ys.append(jnp.dot(zp.astype(BF16), dft(4 + 2 * p, 2), preferred_element_type=F32))
            first = lax.broadcasted_iota(jnp.int32, ys[0].shape, 1) < C // 2
            for j in range(2):
                y = jnp.where(first, ys[j], ys[1 - j])
                for i in range(NL):
                    yt_s[2 * i + j, rows, :] = y[i * 8:(i + 1) * 8]

        def modulation(blocks):
            for b in blocks:
                wmod_copy(b).wait()
            acc_s[...] += _tree_sum([jnp.dot(sc_s[b], wmod_s[b], preferred_element_type=F32)[0:8]
                                     for b in blocks])

        def row(i, n):
            return jnp.concatenate([mod_s[i]] * (n // 8), axis=0)

        def time_major(t, i, blocks):
            for b in blocks:
                y = yt_s[t * (T1 // C) + i, b * CB:(b + 1) * CB, :].T
                for p in range(2):
                    y_s[b, pl.ds(i * C + (i + p) % 2, C // 2, stride=2), :] = y[p * C // 2:(p + 1) * C // 2]

        def standardize(x):
            xc = x - jnp.sum(x, axis=-1, keepdims=True) * (1.0 / D)
            return xc * lax.rsqrt(jnp.sum(xc * xc, axis=-1, keepdims=True) * (1.0 / D) + EPS)

        def residual(t, r, n, qn=None):
            rows = pl.ds(pl.multiple_of(t * T1 + r, n), n)
            q = q_s[rows, :].astype(F32)
            y = jnp.concatenate([y_s[b, r:r + n, :] for b in range(NCB)], axis=1)
            x = q + ((standardize(q) if qn is None else qn) * row(0, n) + row(1, n)) * y
            x_s[rows, :] = x
            return standardize(x) * row(2, n) + row(3, n)

        def elementwise(t):
            hs = []
            for r in range(0, T1, RG):
                if r % C == 0:
                    time_major(t, r // C, range(NCB))
                hs.append(residual(t, r, RG))
            return jnp.concatenate(hs, axis=0)

        def conv_block(b, last):
            ssmk_copy(b).wait()
            f = {0: forward(b, 0)}
            for g in range(NG):
                if g + 1 < NG:
                    f[g + 1] = forward(b, g + 1)
                if g == wait_at and not last:
                    for cp in kv_copies(b + 1):
                        cp.wait()
                if g == mod_at and last:
                    q_copy(0).wait()
                    modulation(range(nmod))
                    for i in range(T1 // C):
                        time_major(0, i, range(NCB - 1))
                    for r in range(0, T1, RG):
                        qn_s[r:r + RG, :] = standardize(q_s[r:r + RG, :].astype(F32))
                inverse(b, g, product(b, g, f.pop(g)))
            if last:
                for i in range(T1 // C):
                    time_major(0, i, [NCB - 1])
                modulation(range(nmod, NCB))
            else:
                for m in range(NL):
                    kv_chunk(b + 1, m)

        with scope("p0_wait0"):
            for b in range(NCB):
                k_s[b, 0:8, :] = jnp.zeros((8, CB), U32)
            acc_s[...] = jnp.zeros(acc_s.shape, F32)
            wout_s[FP // 128 - 1, FH + 128 - FP:, :] = jnp.zeros((FP - FH, D), BF16)
            small[0].wait()
            tp = shift_s[...].astype(F32)
            for b in range(NCB):
                taps_s[b, 0:4, :] = tp[:, b * CB:(b + 1) * CB]
            for cp in kv_copies(0):
                cp.wait()

        with scope("p0_pro"):
            for m in range(NL):
                kv_chunk(0, m)
            for cp in small[1:]:
                cp.wait()
            dsk = ssmd_s[...].astype(F32)
            cf = c_s[...].astype(F32)
            sc = jnp.broadcast_to(cf * jax.nn.sigmoid(cf), (16, D)).astype(BF16)
            for b in range(NCB):
                dsk_s[b * CB:(b + 1) * CB, :] = jnp.broadcast_to(dsk[b:b + 1], (CB, CB)).T
                sc_s[b] = sc[:, b * CB:(b + 1) * CB]
            bspf_s[...] = bsp_s[...].astype(F32)

        with scope("p0_main"):
            @pl.loop(0, NCB - 1)
            def _(b):
                conv_block(b, False)

        with scope("p0_epi"):
            conv_block(NCB - 1, True)
            sa, ca, ga, sb, cb_ = (acc_s[:, i * D:(i + 1) * D] for i in range(5))
            mod_s[0] = ga * (1.0 + ca)
            mod_s[1] = ga * sa
            mod_s[2] = 1.0 + cb_
            mod_s[3] = sb

        def split(tiles):
            return tiles[:KH], tiles[KH:]

        def store_h(h):
            blocks = {(i, j): split([h[j * T1 // 2:(j + 1) * T1 // 2, b * CB:(b + 1) * CB]
                                     for b in range(NCB)])[i] for i in range(2) for j in range(2)}
            for i, op in enumerate(_rhs_operands(blocks, 2)):
                h_s[i, :, :KT[i] * CB] = jnp.concatenate(op[0, 0][:KT[i]], axis=1).astype(BF16)

        def store_w_in():
            for r in range(0, FH // 2, WR):
                words = [[wint_s[1 - i, b, r:r + WR, :] for b in range(NCB)] for i in range(2)]
                lo, hi = [_lhs_operands({(i, j): split([f(w) for w in words[i]])[j]
                                         for i in range(2) for j in range(2)}, 2) for f in (low, high)]
                for i in range(7):
                    for b in range(KT[i]):
                        if (i, b) not in W_SAME:
                            wsum_s[i, b, r:r + WR, :] = pltpu.pack_elementwise(
                                [lo[i][0, 0][b], hi[i][0, 0][b]], packed_dtype=BF16)

        c1 = math.sqrt(2.0 / math.pi)
        c2 = c1 * 0.044715

        def gelu2(x):
            return x * jnp.tanh((x * x * c2 + c1) * x) + x

        def fold8(x):
            return jnp.sum(x.reshape(x.shape[0] // 8, 8, x.shape[1]), axis=0)

        def proj_in_plain(i, h):
            w = jnp.concatenate([bf(wint_s.at[i, b]) for b in range(NCB)], axis=1)
            return lax.dot_general(w, h, NT, preferred_element_type=F32)

        def proj_in():
            prods = []
            for i in range(7):
                w = jnp.concatenate([bf(wint_s.at[W_SAME[i, b]] if (i, b) in W_SAME else wsum_s.at[i, b])
                                     for b in range(KT[i])], axis=1)
                prods.append({(0, 0): lax.dot_general(w, h_s[i, :, :KT[i] * CB], NT,
                                                      preferred_element_type=F32)})
            z = _combine(prods, 2)
            return [jnp.concatenate([z[i, 0], z[i, 1]], axis=1) for i in range(2)]

        def gate_branch(z):
            z = gelu2(z)
            z = z - z[0:1]
            z2f_s[...] = z
            st_s[0] = fold8(z)
            st_s[1] = fold8(z * z)

        def value_branch(t, z):
            z1_s[t] = (z if gelu_late else gelu2(z)).astype(BF16)

        def normalize(t):
            mean = jnp.sum(st_s[0], axis=0, keepdims=True) * (1.0 / FH)
            var = jnp.sum(st_s[1], axis=0, keepdims=True) * (1.0 / FH) - mean * mean
            rs = lax.rsqrt(jnp.maximum(var, 0.0) + 4.0 * EPS)
            zn = (z2f_s[...] - mean) * rs
            hf, hs = FH // 2, T1 // 2
            blocks = {(i, j): zn[i * hf:(i + 1) * hf, j * hs:(j + 1) * hs]
                      for i in range(2) for j in range(2)}
            for i, a in enumerate(_lhs_operands(blocks, 2)):
                z2_s[i, t] = a[0, 0]

        with scope("p1_pro"):
            h0 = jnp.concatenate([residual(0, r, RG0, qn_s[r:r + RG0, :]) for r in range(0, T1, RG0)],
                                 axis=0).astype(BF16)
        with scope("p1_pro2"):
            for cp in win_copies(1) + [q_copy(1)]:
                cp.wait()
            gate_branch(proj_in_plain(1, h0))
            store_h(elementwise(1))
            for cp in win_copies(0):
                cp.wait()
            value_branch(0, proj_in_plain(0, h0))
            store_w_in()

        with scope("p1_main"):
            @pl.loop(1, NT1)
            def _(t):
                @pl.when(t + 1 < NT1)
                def _():
                    q_copy(t + 1).wait()

                @pl.when(t < NT1 - 1)
                def _():
                    wout_copy(t - 1).wait()

                @pl.when(t == NT1 - 1)
                def _():
                    wout_last.wait()
                normalize(t - 1)
                z2, z1 = proj_in()
                gate_branch(z2)
                value_branch(t, z1)
                store_h(elementwise(jnp.minimum(t + 1, NT1 - 1)))
                woutt_s[t - 1] = wout_s[t - 1].astype(F32).T

        with scope("p1_epi"):
            cp_wgate.wait()
            normalize(NT1 - 1)
            sc = jnp.concatenate([sc_s[b] for b in range(NCB)], axis=1)
            mod_s[4] = 0.5 * jnp.dot(sc, wgate_s[...], preferred_element_type=F32)[0:8]

        def spatial(u):
            hs = T1 // 2
            nh = NT1 // 2

            def w_block(si, ti):
                rows = pl.ds(pl.multiple_of(u * TB + ti * HT, HT), HT)
                t0 = (si % 2) * nh
                return jnp.concatenate(
                    [wsp_s[rows, t * T1 + (si // 2) * hs:t * T1 + (si // 2 + 1) * hs]
                     for t in range(t0, t0 + nh)], axis=1).astype(F32)

            def z_operand(i):
                return {(p, q): jnp.concatenate([z2_s[i, t, p * HF:(p + 1) * HF, :]
                                                 for t in range(q * nh, (q + 1) * nh)], axis=1)
                        for p in range(2) for q in range(2)}

            def dot_nt(a, b):
                if s16:
                    a, b = a.astype(BF16), b.astype(BF16)
                return lax.dot_general(a, b, NT, preferred_element_type=F32)

            w = {(si, ti): w_block(si, ti) for si in range(4) for ti in range(4)}
            return _assemble(_combine([_strassen(z_operand(i), op, 2, dot_nt)
                                       for i, op in enumerate(_rhs_operands(w, 4))], 4), 4)

        def proj_out(u, g):
            bias = jnp.concatenate([bspf_s[pl.ds(u * (TB // C) + i, 1), :] for i in range(TB // C)], axis=1)
            z1 = jnp.concatenate([z1_s[u * (TB // T1) + i] for i in range(TB // T1)], axis=1).astype(F32)
            if gelu_late:
                z1 = gelu2(z1)
            m = jnp.concatenate([z1 * (g + bias), jnp.zeros((FP - FH, TB), F32)], axis=0)
            groups = {1: [range(7)], 2: [range(4), range(4, 7)],
                      4: [range(2), range(2, 4), range(4, 6), range(6, 7)]}[SO]
            hd, ht = D // SO, TO // SO

            def dot(a, b):
                n = min(len(a), len(b))
                a, b = jnp.concatenate(a[:n], axis=1), jnp.concatenate(b[:n], axis=0)
                if o16:
                    a, b = a.astype(BF16), b.astype(BF16)
                return jnp.dot(a, b, preferred_element_type=F32)

            for j in range(TB // TO):
                a = {(i, p): [woutt_s[f, i * hd:(i + 1) * hd, :] for f in groups[p]]
                     for i in range(SO) for p in range(SO)}
                b = {(p, i): [m[f * 128:(f + 1) * 128, j * TO + i * ht:j * TO + (i + 1) * ht]
                              for f in groups[p]] for i in range(SO) for p in range(SO)}
                o = _assemble(_strassen(a, b, SO, dot), SO)
                for i in range(TO // TW):
                    t = u * (TB // TW) + j * (TO // TW) + i
                    rows = pl.ds(pl.multiple_of(t * TW, TW), TW)
                    o_s[rows, :] = (x_s[rows, :] + row(4, TW) * o[:, i * TW:(i + 1) * TW].T).astype(BF16)
                    out_copy(t).start()

        with scope("p2_main"):
            @pl.loop(0, S // TB)
            def _(u):
                wsp_copy(u).wait()
                proj_out(u, spatial(u))

        with scope("out_wait"):
            for t in range(S // TW):
                out_copy(t).wait()

    vm = pltpu.VMEM
    scratch = [
        vm((S, D), BF16), vm((NCB, S // 2 + 8, CB), U32), vm((NCB, S // 2, CB), U32), vm((4, D), BF16),
        vm((NCB * S // 2, C), U32), vm((NCB, CB), BF16), vm((2, NCB, FH // 2, CB), U32), vm((S, S), BF16),
        vm((NC, C), BF16), vm((FP // 128, 128, D), BF16), vm((1, D), BF16), vm((NCB, CB, 5 * D), BF16),
        vm((D, D), BF16), vm((4 * C, C), U32),
        vm((NCB, 8, CB), F32), vm((D, CB), F32), vm((NC, C), F32),
        vm((NCB, 16, CB), BF16), vm((NC * CB // 2, C), U32),
        vm((NC, D, C), F32), vm((NCB, T1, CB), F32), vm((8, 5 * D), F32), vm((5, 8, D), F32),
        vm((FP // 128, D, 128), F32), vm((7, KH, FH // 2, CB), U32), vm((S, D), F32), vm((T1, D), F32),
        vm((7, T1 // 2, KH * CB), BF16), vm((2, 8, T1), F32),
        vm((FH, T1), F32), vm((NT1, FH, T1), BF16), vm((7, NT1, FH // 2, T1 // 2), F32),
        vm((S, D), BF16),
        pltpu.SemaphoreType.DMA((10 + 4 * NCB + NT1 + S // TB + 6,)), pltpu.SemaphoreType.DMA((S // TW,)),
    ]

    @jax.jit
    def fn(A_q, A_k, A_v, A_shift_k, A_ssm_k, A_ssm_D, B_x, B_w_in, B_w_sp, B_b_sp, B_w_out, c, w_mod):
        del B_x
        out = pl.pallas_call(
            kernel,
            out_shape=jax.ShapeDtypeStruct((S, D), BF16),
            in_specs=[pl.BlockSpec(memory_space=pltpu.HBM)] * 13,
            out_specs=pl.BlockSpec(memory_space=pltpu.HBM),
            scratch_shapes=scratch,
            compiler_params=pltpu.CompilerParams(vmem_limit_bytes=120 * 2**20, flags=flags),
        )(A_q.reshape(S, D), A_k.reshape(S, D), A_v.reshape(S, D), A_shift_k.T,
          A_ssm_k.reshape(D // 8, 8, NC, C).transpose(0, 2, 1, 3).reshape(NCB * S, C),
          A_ssm_D.reshape(NCB, CB), B_w_in.T, B_w_sp, B_b_sp.reshape(NC, C), B_w_out, c, w_mod,
          _DFT)
        return out.reshape(1, S, D)

    return fn


pallas_adaLN_cond__ssm_conv_h3__mixer_gmlp__prompt_kernel = make()
```

```python
import contextlib
import math

import jax
import jax.numpy as jnp
import numpy as np
from jax import lax
from jax.experimental import pallas as pl
from jax.experimental.pallas import tpu as pltpu

S, D, FH = 2048, 640, 864
C = 128
NC = S // C
CB = 128
NCB = D // CB
NG = CB // 8
FP = 896
KH = 3
KT = (3, 2, 3, 2, 2, 3, 3)
W_SAME = {(0, 2): (0, 2), (2, 2): (1, 2), (3, 0): (0, 3), (3, 1): (0, 4),
          (5, 0): (1, 0), (5, 1): (1, 1), (5, 2): (1, 2)}
KPAD = 32
EPS = 1e-5
F32, BF16, U32 = jnp.float32, jnp.bfloat16, jnp.uint32
NT = (((1,), (1,)), ((), ()))


L = 2 * C
NL = S // L


def _dft_matrices():
    g = np.arange(C, dtype=np.int64)[None, :]
    lane = np.arange(C, dtype=np.int64)

    def mat(samples):
        th = 2.0 * np.pi * ((samples[:, None] * (4 * g + 1)) % (4 * L)) / (4 * L)
        return [np.cos(th), -np.sin(th)]

    fwd = [m for p in range(2) for m in mat((lane % 2 ^ p) * C + lane // 2 * 2 + p)]
    inv = [m.T / L for p in range(2) for m in mat((lane + p * C // 2) % C * 2 + p)]
    return np.concatenate(fwd + inv).astype(BF16)


_DFT = _dft_matrices()


def _tree_sum(xs):
    xs = list(xs)
    while len(xs) > 1:
        xs = [xs[i] + xs[i + 1] if i + 1 < len(xs) else xs[i] for i in range(0, len(xs), 2)]
    return xs[0]


def _quads(x, n):
    h = n // 2
    return [{(i, j): x[i + a * h, j + b * h] for i in range(h) for j in range(h)}
            for a in range(2) for b in range(2)]


def _mix(x, y, sign):
    if isinstance(x, list):
        n = min(len(x), len(y))
        return ([_mix(p, q, sign) for p, q in zip(x, y)] + x[n:]
                + [q if sign > 0 else -q for q in y[n:]])
    return x + y if sign > 0 else x - y


def _add(x, y):
    return {k: _mix(x[k], y[k], 1) for k in x}


def _sub(x, y):
    return {k: _mix(x[k], y[k], -1) for k in x}


def _lhs_operands(a, n):
    a11, a12, a21, a22 = _quads(a, n)
    return [_add(a21, a22), _add(a11, a12), _add(a11, a22), a22, _sub(a12, a22), a11, _sub(a21, a11)]


def _rhs_operands(b, n):
    b11, b12, b21, b22 = _quads(b, n)
    return [b11, b22, _add(b11, b22), _sub(b11, b21), _add(b21, b22), _sub(b12, b22), _add(b11, b12)]


def _combine(products, n):
    m2, m5, m1, m4, m7, m3, m6 = products
    quads = [_add(_sub(_sub(m1, m5), m4), m7), _add(m3, m5),
             _sub(m2, m4), _add(_add(_sub(m1, m2), m3), m6)]
    h, out = n // 2, {}
    for (p, q), c in zip([(0, 0), (0, 1), (1, 0), (1, 1)], quads):
        out.update({(i + p * h, j + q * h): v for (i, j), v in c.items()})
    return out


def _strassen(a, b, n, dot):
    if n == 1:
        return {(0, 0): dot(a[0, 0], b[0, 0])}
    return _combine([_strassen(p, q, n // 2, dot)
                     for p, q in zip(_lhs_operands(a, n), _rhs_operands(b, n))], n)


def _assemble(blocks, n):
    return jnp.concatenate([jnp.concatenate([blocks[i, j] for j in range(n)], axis=1)
                            for i in range(n)], axis=0)


def make(T1=256, TB=512, TO=512, RG=64, scopes=False, flags={'XLA_TPU_EVENLY_DISTRIBUTE_CRITICAL_NODES': True}, gauss=1, wait_at=8, mod_at=10, nmod=3, gelu_late=True, SO=2, TW=128, WR=8, wt=18, nt=0, x16=False, pa=0, wlate=False, TE=256, olate=False, zp=0, zq=0, zn=7, lvl1=True, n0=0, n1=3, RG0=64, o16=True, s16=False):
    NT1 = S // T1
    HF, HS, HT = FH // 4, 128, TB // 4
    SB = 4 * HS
    NSB = S // SB

    def scope(name):
        return jax.named_scope(name) if scopes else contextlib.nullcontext()

    def kernel(q_hbm, k_hbm, v_hbm, shift_hbm, ssmk_hbm, ssmd_hbm, win_hbm, wsp_hbm, bsp_hbm,
               wout_hbm, c_hbm, wmod_hbm, dft_hbm, out_hbm,
               q_s, k_s, v_s, ssmk_s, wint_s, wsp_s, wout_s, wmod_s, wgate_s, dft_s,
               dsk_s, kvt_s, yt_s, y_s, woutt_s, wsum_s, x_s, qn_s, h_s, z2f_s, z1_s, z2_s, m_s, o_s,
               st_s, mod_s, acc_s, taps_s, bspf_s, sc_s, shift_s, ssmd_s, bsp_s, c_s,
               sem_in, sem_out, spare_s):
        spare_s[0] = 7
        o_conv = 6
        o_big = o_conv + 4 * NCB
        o_q = o_big + 4
        o_wsp = o_q + NT1
        o_wout = o_wsp + S // TB

        def copy(src, dst, i):
            return pltpu.make_async_copy(src, dst, sem_in.at[i])

        small = [copy(a, b, i) for i, (a, b) in enumerate(
            [(shift_hbm, shift_s), (ssmd_hbm, ssmd_s), (dft_hbm, dft_s.bitcast(BF16)),
             (c_hbm, c_s), (bsp_hbm, bsp_s)])]

        def kv_copies(b):
            ch = pl.ds(pl.multiple_of(b * CB, CB), CB)
            return [copy(k_hbm.at[:, ch], k_s.bitcast(BF16).at[b, pl.ds(2 * KPAD, S), :], o_conv + 4 * b),
                    copy(v_hbm.at[:, ch], v_s.bitcast(BF16).at[b], o_conv + 4 * b + 1)]

        def ssmk_copy(b):
            r = pl.ds(pl.multiple_of(b * S, S), S)
            return copy(ssmk_hbm.at[r, :], ssmk_s.bitcast(BF16).at[r, :], o_conv + 4 * b + 2)

        def wmod_copy(b):
            r = pl.ds(pl.multiple_of(b * CB, CB), CB)
            return copy(wmod_hbm.at[r, pl.ds(0, 5 * D)], wmod_s.at[b], o_conv + 4 * b + 3)

        def win_copies(i):
            return [copy(win_hbm.at[pl.ds(i * FH, FH), pl.ds(j * CB, CB)],
                         wint_s.bitcast(BF16).at[i, j], o_big + i) for j in range(NCB)]

        def wout_copy(j):
            return copy(wout_hbm.at[pl.ds(pl.multiple_of(j * 128, 128), 128), :], wout_s.at[j], o_wout + j)

        wout_last = copy(wout_hbm.at[pl.ds(FP - 128, FH + 128 - FP), :],
                         wout_s.at[FP // 128 - 1, pl.ds(0, FH + 128 - FP), :], o_big + 2)
        cp_wgate = copy(wmod_hbm.at[:, pl.ds(5 * D, D)], wgate_s, o_big + 3)

        def q_copy(t):
            r = pl.ds(pl.multiple_of(t * T1, T1), T1)
            return copy(q_hbm.at[r, :], q_s.at[r, :], o_q + t)

        def wsp_copy(u):
            r = pl.ds(pl.multiple_of(u * TB, TB), TB)
            return copy(wsp_hbm.at[r, :], wsp_s.at[r, :], o_wsp + u)

        def out_copy(t, n):
            r = pl.ds(pl.multiple_of(t * TW, TW), n)
            return pltpu.make_async_copy(o_s.at[r, :], out_hbm.at[r, :], sem_out.at[t])

        for cp in small[:1] + kv_copies(0) + small[1:]:
            cp.start()
        for b in range(NCB):
            ssmk_copy(b).start()
            if b + 1 < NCB:
                for cp in kv_copies(b + 1):
                    cp.start()
        q_copy(0).start()
        for b in range(NCB):
            wmod_copy(b).start()
        for cp in win_copies(1) + [q_copy(1)] + win_copies(0):
            cp.start()
        for t in range(2, NT1):
            q_copy(t).start()
            wout_copy(t - 2).start()
        wout_last.start()
        cp_wgate.start()
        for u in range(1 if wlate else S // TB):
            wsp_copy(u).start()

        def bf(ref):
            return pltpu.bitcast(ref[...], BF16)

        def dft(i, n):
            return pltpu.bitcast(dft_s[i * C // 2:(i + n) * C // 2, :], BF16)

        def low(w):
            return pltpu.bitcast(w << 16, F32)

        def high(w):
            return pltpu.bitcast(w & np.uint32(0xFFFF0000), F32)

        def kv_chunk(b, m):
            kw = [k_s[b, pl.ds(KPAD + m * C + j, C), :] for j in range(-2, 1)]
            vw = v_s[b, m * C:(m + 1) * C, :]
            kk = [high(kw[0]), low(kw[1]), high(kw[1]), low(kw[2]), high(kw[2])]
            for p, vv in enumerate((low(vw), high(vw))):
                kv = _tree_sum([kk[3 + p - t] * taps_s[b, t:t + 1, :] for t in range(4)]) * vv
                halves = [kv[:C // 2], kv[C // 2:]]
                w = pltpu.pack_elementwise([halves[p], halves[1 - p]], packed_dtype=BF16)
                kvt_s[(2 * m + p) * 64:(2 * m + p + 1) * 64, :] = pltpu.bitcast(pltpu.bitcast(w, BF16).T, U32)

        def forward(b, g):
            base = pl.multiple_of(b * (S // 2), S // 2) + g * NC * 4
            top = lax.broadcasted_iota(jnp.int32, (8, C), 0) < 4
            words = [ssmk_s[pl.ds(base + 4 * i, 8), :] if i % 4 < 3 else None for i in range(NC)]
            t0, t1 = [jnp.concatenate([jnp.where(top, words[i + j], words[i + j + 1])
                                       for i in range(0, NC, 4)], axis=0) for j in range(2)]
            odd = (lax.broadcasted_iota(jnp.int32, t0.shape, 1) & 1) == 1
            kt = [jnp.where(odd, pltpu.roll(t1, 1, 1), t0), jnp.where(odd, t0, pltpu.roll(t1, C - 1, 1))]
            out = []
            for p in range(2):
                xt = jnp.concatenate(
                    [jnp.where(top, kvt_s[pl.ds((2 * m + p) * 64 + 4 * g, 8), :],
                               kvt_s[pl.ds((2 * m + 2 + p) * 64 + 4 * g - 4, 8), :])
                     for m in range(0, NL, 2)], axis=0)
                lhs = jnp.concatenate([t[i:i + 8] for i in range(0, 4 * NL, 8) for t in (kt[p], xt)], axis=0)
                out.append([jnp.dot(pltpu.bitcast(lhs, BF16), dft(2 * p + c, 1), preferred_element_type=F32)
                            for c in range(2)])
            return out

        def butterfly(a, b):
            return (a[0] + b[0], a[1] + b[1]), (a[0] - b[0], a[1] - b[1])

        def product(b, g, f):
            def part(i, m, p):
                r = (m // 2 * 4 + i * 2 + m % 2) * 8
                return f[p][0][r:r + 8], f[p][1][r:r + 8]

            def window(m, p):
                re, im = part(0, m, p)
                if m:
                    pre, pim = part(0, m - 1, p)
                    return re - pim, im + pre
                if p == 0:
                    re = re + dsk_s[pl.ds(pl.multiple_of(b * CB + g * 8, 8), 8), :]
                return re, im

            kf = [butterfly(window(m, 0), window(m, 1)) for m in range(NL)]
            xf = [butterfly(part(1, m, 0), part(1, m, 1)) for m in range(NL)]
            out = []
            for i in range(NL):
                z = []
                for h in range(2):
                    terms = [(xf[j][h], kf[i - j][h]) for j in range(i + 1)]
                    if i >= gauss:
                        p1 = _tree_sum([x[0] * k[0] for x, k in terms])
                        p2 = _tree_sum([x[1] * k[1] for x, k in terms])
                        p3 = _tree_sum([(x[0] + x[1]) * (k[0] + k[1]) for x, k in terms])
                        z.append((p1 - p2, p3 - (p1 + p2)))
                    else:
                        z.append((_tree_sum([x[0] * k[0] - x[1] * k[1] for x, k in terms]),
                                  _tree_sum([x[0] * k[1] + x[1] * k[0] for x, k in terms])))
                out.append(butterfly(*z))
            return out

        def inverse(b, g, z):
            rows = pl.ds(pl.multiple_of(b * CB + g * 8, 8), 8)
            ys = []
            for p in range(2):
                zp = jnp.concatenate([jnp.concatenate([z[i][p][c] for i in range(NL)], axis=0)
                                      for c in range(2)], axis=1)
                ys.append(jnp.dot(zp.astype(BF16), dft(4 + 2 * p, 2), preferred_element_type=F32))
            first = lax.broadcasted_iota(jnp.int32, ys[0].shape, 1) < C // 2
            for j in range(2):
                y = jnp.where(first, ys[j], ys[1 - j])
                for i in range(NL):
                    yt_s[2 * i + j, rows, :] = y[i * 8:(i + 1) * 8]

        def modulation(blocks):
            with scope("w_mod%d" % len(blocks)):
                for b in blocks:
                    wmod_copy(b).wait()
            acc_s[...] += _tree_sum([jnp.dot(sc_s[b], wmod_s[b], preferred_element_type=F32)[0:8]
                                     for b in blocks])

        def row(i, n):
            return jnp.concatenate([mod_s[i]] * (n // 8), axis=0)

        def time_major(t, i, blocks):
            for b in blocks:
                y = yt_s[t * (T1 // C) + i, b * CB:(b + 1) * CB, :].T
                for p in range(2):
                    y_s[b, pl.ds(i * C + (i + p) % 2, C // 2, stride=2), :] = y[p * C // 2:(p + 1) * C // 2]

        def standardize(x):
            xc = x - jnp.sum(x, axis=-1, keepdims=True) * (1.0 / D)
            return xc * lax.rsqrt(jnp.sum(xc * xc, axis=-1, keepdims=True) * (1.0 / D) + EPS)

        def residual(t, r, n, qn=None):
            rows = pl.ds(pl.multiple_of(t * T1 + r, n), n)
            q = q_s[rows, :].astype(F32)
            y = jnp.concatenate([y_s[b, r:r + n, :] for b in range(NCB)], axis=1)
            x = q + ((standardize(q) if qn is None else qn) * row(0, n) + row(1, n)) * y
            x_s[rows, :] = x.astype(x_s.dtype)
            return standardize(x) * row(2, n) + row(3, n)

        def elementwise(t):
            hs = []
            for r in range(0, T1, RG):
                if r % C == 0:
                    time_major(t, r // C, range(NCB))
                hs.append(residual(t, r, RG))
            return jnp.concatenate(hs, axis=0)

        def conv_block(b, last):
            with scope('w_ssmk'):
                ssmk_copy(b).wait()
            f = {0: forward(b, 0)}
            for g in range(NG):
                if g + 1 < NG:
                    f[g + 1] = forward(b, g + 1)
                if g == wait_at and not last:
                    with scope("w_kv"):
                        for cp in kv_copies(b + 1):
                            cp.wait()
                if g == mod_at and last:
                    q_copy(0).wait()
                    modulation(range(nmod))
                    for i in range(T1 // C):
                        time_major(0, i, range(NCB - 1))
                    for r in range(0, T1, RG):
                        qn_s[r:r + RG, :] = standardize(q_s[r:r + RG, :].astype(F32))
                inverse(b, g, product(b, g, f.pop(g)))
            if last:
                for i in range(T1 // C):
                    time_major(0, i, [NCB - 1])
                modulation(range(nmod, NCB))
            else:
                for m in range(NL):
                    kv_chunk(b + 1, m)

        with scope("p0_wait0"):
            for b in range(NCB):
                k_s[b, KPAD - 8:KPAD, :] = jnp.zeros((8, CB), U32)
            acc_s[...] = jnp.zeros(acc_s.shape, F32)
            m_s[FH:, :] = jnp.zeros((FP - FH, TB), F32)
            wout_s[FP // 128 - 1, FH + 128 - FP:, :] = jnp.zeros((FP - FH, D), BF16)
            small[0].wait()
            tp = shift_s[...].astype(F32)
            for b in range(NCB):
                taps_s[b, 0:4, :] = tp[:, b * CB:(b + 1) * CB]
            for cp in kv_copies(0):
                cp.wait()

        with scope("p0_pro"):
            for m in range(NL):
                kv_chunk(0, m)
            for cp in small[1:]:
                cp.wait()
            dsk = ssmd_s[...].astype(F32)
            cf = c_s[...].astype(F32)
            sc = jnp.broadcast_to(cf * jax.nn.sigmoid(cf), (16, D)).astype(BF16)
            for b in range(NCB):
                dsk_s[b * CB:(b + 1) * CB, :] = jnp.broadcast_to(dsk[b:b + 1], (CB, CB)).T
                sc_s[b] = sc[:, b * CB:(b + 1) * CB]
            bspf_s[...] = bsp_s[...].astype(F32)

        with scope("p0_main"):
            @pl.loop(0, NCB - 1)
            def _(b):
                conv_block(b, False)

        with scope("p0_epi"):
            conv_block(NCB - 1, True)
            sa, ca, ga, sb, cb_ = (acc_s[:, i * D:(i + 1) * D] for i in range(5))
            mod_s[0] = ga * (1.0 + ca)
            mod_s[1] = ga * sa
            mod_s[2] = 1.0 + cb_
            mod_s[3] = sb

        def split(tiles):
            return tiles[:KH], tiles[KH:]

        def store_h(h):
            blocks = {(i, j): split([h[j * T1 // 2:(j + 1) * T1 // 2, b * CB:(b + 1) * CB]
                                     for b in range(NCB)])[i] for i in range(2) for j in range(2)}
            for i, op in enumerate(_rhs_operands(blocks, 2)):
                h_s[i, :, :KT[i] * CB] = jnp.concatenate(op[0, 0][:KT[i]], axis=1).astype(BF16)

        def store_w_in(z, spare):
            marks = [z[r:r + 8, n:n + C] for n in range(0, T1, C) for r in range(0, FH, 2 * FH // wt)]
            for r in range(0, FH // 2, WR):
                if r % (FH // 2 // wt) == 0:
                    wsum_s[spare, 0, 0:8, :] = pltpu.bitcast(marks.pop(0), U32)
                words = [[wint_s[1 - i, b, r:r + WR, :] for b in range(NCB)] for i in range(2)]
                lo, hi = [_lhs_operands({(i, j): split([f(w) for w in words[i]])[j]
                                         for i in range(2) for j in range(2)}, 2) for f in (low, high)]
                for i in range(7):
                    for b in range(KT[i]):
                        if (i, b) not in W_SAME:
                            wsum_s[i, b, r:r + WR, :] = pltpu.pack_elementwise(
                                [lo[i][0, 0][b], hi[i][0, 0][b]], packed_dtype=BF16)

        c1 = math.sqrt(2.0 / math.pi)
        c2 = c1 * 0.044715

        def gelu2(x):
            return x * jnp.tanh((x * x * c2 + c1) * x) + x

        def fold8(x):
            return jnp.sum(x.reshape(x.shape[0] // 8, 8, x.shape[1]), axis=0)

        def proj_in_plain(i, h):
            w = jnp.concatenate([bf(wint_s.at[i, b]) for b in range(NCB)], axis=1)
            return lax.dot_general(w, h, NT, preferred_element_type=F32)

        def proj_in():
            prods = []
            for i in range(7):
                w = jnp.concatenate([bf(wint_s.at[W_SAME[i, b]] if (i, b) in W_SAME else wsum_s.at[i, b])
                                     for b in range(KT[i])], axis=1)
                prods.append({(0, 0): lax.dot_general(w, h_s[i, :, :KT[i] * CB], NT,
                                                      preferred_element_type=F32)})
            z = _combine(prods, 2)
            marks = [p[0, 0][r:r + 8] for p in prods[n0:n1] for r in range(0, FH, FH * (n1 - n0) // nt)] if nt else ()
            return [jnp.concatenate([z[i, 0], z[i, 1]], axis=1) for i in range(2)] + [marks]

        def gate_branch(z):
            z = gelu2(z)
            z = z - z[0:1]
            z2f_s[...] = z
            st_s[0] = fold8(z)
            st_s[1] = fold8(z * z)

        def value_branch(t, z):
            z1_s[t] = (z if gelu_late else gelu2(z)).astype(BF16)

        def normalize(t, marks=()):
            mean = jnp.sum(st_s[0], axis=0, keepdims=True) * (1.0 / FH)
            var = jnp.sum(st_s[1], axis=0, keepdims=True) * (1.0 / FH) - mean * mean
            rs = lax.rsqrt(jnp.maximum(var, 0.0) + 4.0 * EPS)
            hf, hs = FH // 2, T1 // 2
            n = hf // max(len(marks), 1)
            for r in range(0, hf, n):
                zn = [(z2f_s[i * hf + r:i * hf + r + n, :] - mean) * rs for i in range(2)]
                blocks = {(i, j): zn[i][:, j * hs:(j + 1) * hs] for i in range(2) for j in range(2)}
                for i, a in enumerate(_lhs_operands(blocks, 2) if lvl1 else _quads(blocks, 2)):
                    z2_s[i, t // (NT1 // 2), pl.ds(pl.multiple_of(t % (NT1 // 2) * (hf + zp) + r, 8), n), :] = a[0, 0]
                if marks:
                    z2_s[spare_s[0], 0, 0:8, :] = marks[r // n]

        with scope("p1_pro"):
            h0 = jnp.concatenate([residual(0, r, RG0, qn_s[r:r + RG0, :]) for r in range(0, T1, RG0)],
                                 axis=0).astype(BF16)
        with scope("p1_pro2"):
            with scope("w_a"):
                for cp in win_copies(1) + [q_copy(1)]:
                    cp.wait()
            gate_branch(proj_in_plain(1, h0))
            store_h(elementwise(1))
            with scope("w_b"):
                for cp in win_copies(0):
                    cp.wait()
            with scope("pro_b"):
                z1 = proj_in_plain(0, h0)
                value_branch(0, z1)
                store_w_in(z1, spare_s[0])

        with scope("p1_main"):
            @pl.loop(1, NT1)
            def _(t):
                @pl.when(t + 1 < NT1)
                def _():
                    q_copy(t + 1).wait()

                @pl.when(t < NT1 - 1)
                def _():
                    wout_copy(t - 1).wait()

                @pl.when(t == NT1 - 1)
                def _():
                    wout_last.wait()
                z2, z1, marks = proj_in()
                normalize(t - 1, marks)
                gate_branch(z2)
                value_branch(t, z1)
                store_h(elementwise(jnp.minimum(t + 1, NT1 - 1)))
                woutt_s[t - 1] = wout_s[t - 1].astype(F32).T

        with scope("p1_epi"):
            cp_wgate.wait()
            normalize(NT1 - 1)
            sc = jnp.concatenate([sc_s[b] for b in range(NCB)], axis=1)
            mod_s[4] = 0.5 * jnp.dot(sc, wgate_s[...], preferred_element_type=F32)[0:8]

        def spatial(u):
            hs = T1 // 2
            nh = NT1 // 2

            def w_block(si, ti):
                rows = pl.ds(pl.multiple_of(u * TB + ti * HT, HT), HT)
                t0 = (si % 2) * nh
                return jnp.concatenate(
                    [wsp_s[rows, t * T1 + (si // 2) * hs:t * T1 + (si // 2 + 1) * hs]
                     for t in range(t0, t0 + nh)], axis=1).astype(F32)

            def z_operand(i):
                return {(p, q): jnp.concatenate([z2_s[i, q, t * (2 * HF + zp) + p * HF:t * (2 * HF + zp) + (p + 1) * HF, :]
                                                 for t in range(nh)], axis=1)
                        for p in range(2) for q in range(2)}

            def dot_nt(a, b):
                if s16:
                    a, b = a.astype(BF16), b.astype(BF16)
                return lax.dot_general(a, b, NT, preferred_element_type=F32)

            w = {(si, ti): w_block(si, ti) for si in range(4) for ti in range(4)}
            if not lvl1:
                z = {(2 * (i // 2) + p, 2 * (i % 2) + q): v for i in range(4) for (p, q), v in z_operand(i).items()}
                return _assemble(_strassen(z, w, 4, dot_nt), 4)
            return _assemble(_combine([_strassen(z_operand(i), op, 2, dot_nt)
                                       for i, op in enumerate(_rhs_operands(w, 4))], 4), 4)

        def gated(u):
            g = spatial(u)
            bias = jnp.concatenate([bspf_s[pl.ds(u * (TB // C) + i, 1), :] for i in range(TB // C)], axis=1)
            z1 = jnp.concatenate([z1_s[u * (TB // T1) + i] for i in range(TB // T1)], axis=1).astype(F32)
            m_s[:FH, :] = gelu2(z1) * (g + bias)

        def proj_out(u, to, eager):
            groups = [range(4), range(4, 7)]
            hd, ht = D // 2, to // 2

            def dot(a, b):
                n = min(len(a), len(b))
                return jnp.dot(jnp.concatenate(a[:n], axis=1).astype(BF16),
                               jnp.concatenate(b[:n], axis=0).astype(BF16), preferred_element_type=F32)

            for j in range(0, TB, to):
                a = {(i, p): [woutt_s[f, i * hd:(i + 1) * hd, :] for f in groups[p]]
                     for i in range(2) for p in range(2)}
                b = {(p, i): [m_s[f * 128:(f + 1) * 128, j + i * ht:j + (i + 1) * ht] for f in groups[p]]
                     for i in range(2) for p in range(2)}
                o = _assemble(_strassen(a, b, 2, dot), 2)
                for i in range(0, to, TW):
                    t = u * (TB // TW) + (j + i) // TW
                    rows = pl.ds(pl.multiple_of(t * TW, TW), TW)
                    o_s[rows, :] = (x_s[rows, :] + row(4, TW) * o[:, i:i + TW].T).astype(BF16)
                    if eager:
                        out_copy(t, TW).start()

        with scope("p2_pro"):
            wsp_copy(0).wait()
            gated(0)

        with scope("p2_main"):
            @pl.loop(1, S // TB)
            def _(u):
                wsp_copy(u).wait()
                with scope("p2_it"):
                    proj_out(u - 1, TO, False)
                    gated(u)
                if not olate:
                    out_copy((u - 1) * (TB // TW), TB).start()

        with scope("p2_epi"):
            if olate:
                out_copy(0, S - TB).start()
            proj_out(S // TB - 1, TE, True)

        with scope("out_wait"):
            if olate:
                out_copy(0, S - TB).wait()
            else:
                for u in range(S // TB - 1):
                    out_copy(u * (TB // TW), TB).wait()
            for t in range((S - TB) // TW, S // TW):
                out_copy(t, TW).wait()

    vm = pltpu.VMEM
    scratch = [
        vm((S, D), BF16), vm((NCB, S // 2 + KPAD, CB), U32), vm((NCB, S // 2, CB), U32),
        vm((NCB * S // 2, C), U32), vm((2, NCB, FH // 2, CB), U32), vm((S, S), BF16),
        vm((FP // 128, 128, D), BF16), vm((NCB, CB, 5 * D), BF16), vm((D, D), BF16), vm((4 * C, C), U32),
        vm((D, CB), F32), vm((NC * CB // 2, C), U32), vm((NC, D, C), F32), vm((NCB, T1, CB), F32),
        vm((FP // 128, D, 128), F32), vm((8, KH, FH // 2, CB), U32), vm((S, D), F32), vm((T1, D), F32),
        vm((7, T1 // 2, KH * CB), BF16), vm((FH, T1), F32), vm((NT1, FH, T1), BF16),
        vm((zn, 2, NT1 // 2 * (FH // 2 + zp) + zq, T1 // 2), F32), vm((FP, TB), F32), vm((S, D), BF16),
        vm((2, 8, T1), F32), vm((8, 8, D), F32), vm((8, 5 * D), F32), vm((NCB + pa, 8, CB), F32),
        vm((NC, C), F32), vm((NCB, 16, CB), BF16), vm((4, D), BF16), vm((NCB, CB), BF16),
        vm((NC, C), BF16), vm((1, D), BF16),
        pltpu.SemaphoreType.DMA((10 + 4 * NCB + NT1 + S // TB + 6,)), pltpu.SemaphoreType.DMA((S // TW,)),
        pltpu.SMEM((1,), jnp.int32),
    ]

    @jax.jit
    def fn(A_q, A_k, A_v, A_shift_k, A_ssm_k, A_ssm_D, B_x, B_w_in, B_w_sp, B_b_sp, B_w_out, c, w_mod):
        del B_x
        out = pl.pallas_call(
            kernel,
            out_shape=jax.ShapeDtypeStruct((S, D), BF16),
            in_specs=[pl.BlockSpec(memory_space=pltpu.HBM)] * 13,
            out_specs=pl.BlockSpec(memory_space=pltpu.HBM),
            scratch_shapes=scratch,
            compiler_params=pltpu.CompilerParams(vmem_limit_bytes=120 * 2**20, flags=flags),
        )(A_q.reshape(S, D), A_k.reshape(S, D), A_v.reshape(S, D), A_shift_k.T,
          A_ssm_k.reshape(D // 8, 8, NC, C).transpose(0, 2, 1, 3).reshape(NCB * S, C),
          A_ssm_D.reshape(NCB, CB), B_w_in.T, B_w_sp, B_b_sp.reshape(NC, C), B_w_out, c, w_mod,
          _DFT)
        return out.reshape(1, S, D)

    return fn


pallas_adaLN_cond__ssm_conv_h3__mixer_gmlp__prompt_kernel = make()
```

```python
import contextlib
import math

import jax
import jax.numpy as jnp
import numpy as np
from jax import lax
from jax.experimental import pallas as pl
from jax.experimental.pallas import tpu as pltpu

S, D, FH = 2048, 640, 864
C = 128
NC = S // C
CB = 128
NCB = D // CB
NG = CB // 8
FP = 896
KH = 3
KT = (3, 2, 3, 2, 2, 3, 3)
W_SAME = {(0, 2): (0, 2), (2, 2): (1, 2), (3, 0): (0, 3), (3, 1): (0, 4),
          (5, 0): (1, 0), (5, 1): (1, 1), (5, 2): (1, 2)}
KPAD = 32
EPS = 1e-5
F32, BF16, U32 = jnp.float32, jnp.bfloat16, jnp.uint32
NT = (((1,), (1,)), ((), ()))


L = 2 * C
NL = S // L


def _tree_sum(xs):
    xs = list(xs)
    while len(xs) > 1:
        xs = [xs[i] + xs[i + 1] if i + 1 < len(xs) else xs[i] for i in range(0, len(xs), 2)]
    return xs[0]


def _quads(x, n):
    h = n // 2
    return [{(i, j): x[i + a * h, j + b * h] for i in range(h) for j in range(h)}
            for a in range(2) for b in range(2)]


def _mix(x, y, sign):
    if isinstance(x, list):
        n = min(len(x), len(y))
        return ([_mix(p, q, sign) for p, q in zip(x, y)] + x[n:]
                + [q if sign > 0 else -q for q in y[n:]])
    return x + y if sign > 0 else x - y


def _add(x, y):
    return {k: _mix(x[k], y[k], 1) for k in x}


def _sub(x, y):
    return {k: _mix(x[k], y[k], -1) for k in x}


def _lhs_operands(a, n):
    a11, a12, a21, a22 = _quads(a, n)
    return [_add(a21, a22), _add(a11, a12), _add(a11, a22), a22, _sub(a12, a22), a11, _sub(a21, a11)]


def _rhs_operands(b, n):
    b11, b12, b21, b22 = _quads(b, n)
    return [b11, b22, _add(b11, b22), _sub(b11, b21), _add(b21, b22), _sub(b12, b22), _add(b11, b12)]


def _combine(products, n):
    m2, m5, m1, m4, m7, m3, m6 = products
    quads = [_add(_sub(_sub(m1, m5), m4), m7), _add(m3, m5),
             _sub(m2, m4), _add(_add(_sub(m1, m2), m3), m6)]
    h, out = n // 2, {}
    for (p, q), c in zip([(0, 0), (0, 1), (1, 0), (1, 1)], quads):
        out.update({(i + p * h, j + q * h): v for (i, j), v in c.items()})
    return out


def _strassen(a, b, n, dot):
    if n == 1:
        return {(0, 0): dot(a[0, 0], b[0, 0])}
    return _combine([_strassen(p, q, n // 2, dot)
                     for p, q in zip(_lhs_operands(a, n), _rhs_operands(b, n))], n)


def _assemble(blocks, n):
    return jnp.concatenate([jnp.concatenate([blocks[i, j] for j in range(n)], axis=1)
                            for i in range(n)], axis=0)


def make(T1=256, TB=512, TO=512, RG=256, scopes=False, flags={'XLA_TPU_EVENLY_DISTRIBUTE_CRITICAL_NODES': True}, gauss=1, wait_at=8, mod_at=12, nmod=4, gelu_late=True, SO=2, TW=128, WR=8, wt=18, nt=0, x16=False, pa=0, wlate=False, TE=256, olate=False, zp=16, zq=0, zn=7, lvl1=True, n0=0, n1=3, RG0=256, o16=True, s16=False):
    NT1 = S // T1
    HF, HS, HT = FH // 4, 128, TB // 4
    SB = 4 * HS
    NSB = S // SB

    def scope(name):
        return jax.named_scope(name) if scopes else contextlib.nullcontext()

    def kernel(q_hbm, k_hbm, v_hbm, shift_hbm, ssmk_hbm, ssmd_hbm, win_hbm, wsp_hbm, bsp_hbm,
               wout_hbm, c_hbm, wmod_hbm, out_hbm,
               q_s, k_s, v_s, ssmk_s, wint_s, wsp_s, wout_s, wmod_s, wgate_s, dft_s,
               dsk_s, kvt_s, yt_s, y_s, woutt_s, wsum_s, x_s, qn_s, h_s, z2f_s, z1_s, z2_s, m_s, o_s,
               st_s, mod_s, acc_s, taps_s, bspf_s, sc_s, shift_s, ssmd_s, bsp_s, c_s,
               sem_in, sem_out, spare_s):
        spare_s[0] = 7
        o_conv = 6
        o_big = o_conv + 4 * NCB
        o_q = o_big + 4
        o_wsp = o_q + NT1
        o_wout = o_wsp + S // TB

        def copy(src, dst, i):
            return pltpu.make_async_copy(src, dst, sem_in.at[i])

        small = [copy(a, b, i) for i, (a, b) in enumerate(
            [(shift_hbm, shift_s), (ssmd_hbm, ssmd_s), (c_hbm, c_s), (bsp_hbm, bsp_s)])]

        def kv_copies(b):
            ch = pl.ds(pl.multiple_of(b * CB, CB), CB)
            return [copy(k_hbm.at[:, ch], k_s.bitcast(BF16).at[b, pl.ds(2 * KPAD, S), :], o_conv + 4 * b),
                    copy(v_hbm.at[:, ch], v_s.bitcast(BF16).at[b], o_conv + 4 * b + 1)]

        def ssmk_copy(b):
            r = pl.ds(pl.multiple_of(b * S, S), S)
            return copy(ssmk_hbm.at[r, :], ssmk_s.bitcast(BF16).at[r, :], o_conv + 4 * b + 2)

        def wmod_copy(b):
            r = pl.ds(pl.multiple_of(b * CB, CB), CB)
            return copy(wmod_hbm.at[r, pl.ds(0, 5 * D)], wmod_s.at[b], o_conv + 4 * b + 3)

        def win_copies(i):
            return [copy(win_hbm.at[pl.ds(i * FH, FH), pl.ds(j * CB, CB)],
                         wint_s.bitcast(BF16).at[i, j], o_big + i) for j in range(NCB)]

        cp_wout = copy(wout_hbm, wout_s.at[pl.ds(0, FH), :], o_big + 2)
        cp_wgate = copy(wmod_hbm.at[:, pl.ds(5 * D, D)], wgate_s, o_big + 3)

        def q_copy(t):
            r = pl.ds(pl.multiple_of(t * T1, T1), T1)
            return copy(q_hbm.at[r, :], q_s.at[r, :], o_q + t)

        def wsp_copy(u):
            r = pl.ds(pl.multiple_of(u * TB, TB), TB)
            return copy(wsp_hbm.at[r, :], wsp_s.at[r, :], o_wsp + u)

        def out_copy(t, n):
            r = pl.ds(pl.multiple_of(t * TW, TW), n)
            return pltpu.make_async_copy(o_s.at[r, :], out_hbm.at[r, :], sem_out.at[t])

        for cp in small[:1] + kv_copies(0) + small[1:]:
            cp.start()
        for b in range(NCB):
            ssmk_copy(b).start()
            if b + 1 < NCB:
                for cp in kv_copies(b + 1):
                    cp.start()
        q_copy(0).start()
        for b in range(NCB):
            wmod_copy(b).start()
        for cp in win_copies(1) + [q_copy(1)] + win_copies(0):
            cp.start()
        for t in range(2, NT1):
            q_copy(t).start()
        cp_wout.start()
        cp_wgate.start()
        for u in range(1 if wlate else S // TB):
            wsp_copy(u).start()

        def bf(ref):
            return pltpu.bitcast(ref[...], BF16)

        def dft(i, n):
            return pltpu.bitcast(dft_s[i * C // 2:(i + n) * C // 2, :], BF16)

        def low(w):
            return pltpu.bitcast(w << 16, F32)

        def high(w):
            return pltpu.bitcast(w & np.uint32(0xFFFF0000), F32)

        def kv_chunk(b, m):
            kw = [k_s[b, pl.ds(KPAD + m * C + j, C), :] for j in range(-2, 1)]
            vw = v_s[b, m * C:(m + 1) * C, :]
            kk = [high(kw[0]), low(kw[1]), high(kw[1]), low(kw[2]), high(kw[2])]
            for p, vv in enumerate((low(vw), high(vw))):
                kv = _tree_sum([kk[3 + p - t] * taps_s[b, t:t + 1, :] for t in range(4)]) * vv
                halves = [kv[:C // 2], kv[C // 2:]]
                w = pltpu.pack_elementwise([halves[p], halves[1 - p]], packed_dtype=BF16)
                kvt_s[(2 * m + p) * 64:(2 * m + p + 1) * 64, :] = pltpu.bitcast(pltpu.bitcast(w, BF16).T, U32)

        def forward(b, g):
            base = pl.multiple_of(b * (S // 2), S // 2) + g * NC * 4
            top = lax.broadcasted_iota(jnp.int32, (8, C), 0) < 4
            words = [ssmk_s[pl.ds(base + 4 * i, 8), :] if i % 4 < 3 else None for i in range(NC)]
            t0, t1 = [jnp.concatenate([jnp.where(top, words[i + j], words[i + j + 1])
                                       for i in range(0, NC, 4)], axis=0) for j in range(2)]
            odd = (lax.broadcasted_iota(jnp.int32, t0.shape, 1) & 1) == 1
            kt = [jnp.where(odd, pltpu.roll(t1, 1, 1), t0), jnp.where(odd, t0, pltpu.roll(t1, C - 1, 1))]
            out = []
            for p in range(2):
                xt = jnp.concatenate(
                    [jnp.where(top, kvt_s[pl.ds((2 * m + p) * 64 + 4 * g, 8), :],
                               kvt_s[pl.ds((2 * m + 2 + p) * 64 + 4 * g - 4, 8), :])
                     for m in range(0, NL, 2)], axis=0)
                lhs = jnp.concatenate([t[i:i + 8] for i in range(0, 4 * NL, 8) for t in (kt[p], xt)], axis=0)
                out.append([jnp.dot(pltpu.bitcast(lhs, BF16), dft(2 * p + c, 1), preferred_element_type=F32)
                            for c in range(2)])
            return out

        def butterfly(a, b):
            return (a[0] + b[0], a[1] + b[1]), (a[0] - b[0], a[1] - b[1])

        def product(b, g, f):
            def part(i, m, p):
                r = (m // 2 * 4 + i * 2 + m % 2) * 8
                return f[p][0][r:r + 8], f[p][1][r:r + 8]

            def window(m, p):
                re, im = part(0, m, p)
                if m:
                    pre, pim = part(0, m - 1, p)
                    return re - pim, im + pre
                if p == 0:
                    re = re + dsk_s[pl.ds(pl.multiple_of(b * CB + g * 8, 8), 8), :]
                return re, im

            kf = [butterfly(window(m, 0), window(m, 1)) for m in range(NL)]
            xf = [butterfly(part(1, m, 0), part(1, m, 1)) for m in range(NL)]
            out = []
            for i in range(NL):
                z = []
                for h in range(2):
                    terms = [(xf[j][h], kf[i - j][h]) for j in range(i + 1)]
                    if i >= gauss:
                        p1 = _tree_sum([x[0] * k[0] for x, k in terms])
                        p2 = _tree_sum([x[1] * k[1] for x, k in terms])
                        p3 = _tree_sum([(x[0] + x[1]) * (k[0] + k[1]) for x, k in terms])
                        z.append((p1 - p2, p3 - (p1 + p2)))
                    else:
                        z.append((_tree_sum([x[0] * k[0] - x[1] * k[1] for x, k in terms]),
                                  _tree_sum([x[0] * k[1] + x[1] * k[0] for x, k in terms])))
                out.append(butterfly(*z))
            return out

        def inverse(b, g, z):
            rows = pl.ds(pl.multiple_of(b * CB + g * 8, 8), 8)
            for p in range(2):
                zp = jnp.concatenate([jnp.concatenate([z[i][p][c] for i in range(NL)], axis=0)
                                      for c in range(2)], axis=1)
                y = jnp.dot(zp.astype(BF16), dft(4 + 2 * p, 2), preferred_element_type=F32)
                for i in range(NL):
                    yt_s[i, p, rows, :] = y[i * 8:(i + 1) * 8]

        def modulation(blocks):
            with scope("w_mod%d" % len(blocks)):
                for b in blocks:
                    wmod_copy(b).wait()
            acc_s[...] += _tree_sum([jnp.dot(sc_s[b], wmod_s[b], preferred_element_type=F32)[0:8]
                                     for b in blocks])

        def row(i, n):
            return jnp.concatenate([mod_s[i]] * (n // 8), axis=0)

        def time_major(t, blocks):
            for b in blocks:
                for p in range(2):
                    y_s[b, pl.ds(p, C, stride=2), :] = yt_s[t, p, b * CB:(b + 1) * CB, :].T

        def standardize(x):
            xc = x - jnp.sum(x, axis=-1, keepdims=True) * (1.0 / D)
            return xc * lax.rsqrt(jnp.sum(xc * xc, axis=-1, keepdims=True) * (1.0 / D) + EPS)

        def residual(t, r, n, qn=None):
            rows = pl.ds(pl.multiple_of(t * T1 + r, n), n)
            q = q_s[rows, :].astype(F32)
            y = jnp.concatenate([y_s[b, r:r + n, :] for b in range(NCB)], axis=1)
            x = q + ((standardize(q) if qn is None else qn) * row(0, n) + row(1, n)) * y
            x_s[rows, :] = x.astype(x_s.dtype)
            return standardize(x) * row(2, n) + row(3, n)

        def elementwise(t):
            time_major(t, range(NCB))
            return residual(t, 0, T1)

        def conv_block(b, last):
            with scope('w_ssmk'):
                ssmk_copy(b).wait()
            f = {0: forward(b, 0)}
            for g in range(NG):
                if g + 1 < NG:
                    f[g + 1] = forward(b, g + 1)
                if g == wait_at and not last:
                    with scope("w_kv"):
                        for cp in kv_copies(b + 1):
                            cp.wait()
                if g == mod_at and last:
                    q_copy(0).wait()
                    modulation(range(nmod))
                    time_major(0, range(NCB - 1))
                    for r in range(0, T1, RG):
                        qn_s[r:r + RG, :] = standardize(q_s[r:r + RG, :].astype(F32))
                inverse(b, g, product(b, g, f.pop(g)))
            if last:
                time_major(0, [NCB - 1])
                if nmod < NCB:
                    modulation(range(nmod, NCB))
            else:
                for m in range(NL):
                    kv_chunk(b + 1, m)

        with scope("p0_wait0"):
            for b in range(NCB):
                k_s[b, KPAD - 8:KPAD, :] = jnp.zeros((8, CB), U32)
            acc_s[...] = jnp.zeros(acc_s.shape, F32)
            m_s[FH:, :] = jnp.zeros((FP - FH, TB), F32)
            wout_s[FH:, :] = jnp.zeros((FP - FH, D), BF16)
            row_id = lax.broadcasted_iota(jnp.int32, (C, C), 0)
            col_id = lax.broadcasted_iota(jnp.int32, (C, C), 1)
            for p in range(2):
                source = ((row_id & 1) ^ p) * C + (row_id & -2) + p
                for i, (sample, freq, scale) in enumerate([(source, col_id, 1.0),
                                                           (2 * col_id + p, row_id, 1.0 / L)]):
                    turn = (sample * (4 * freq + 1) + 2 * L) & (4 * L - 1)
                    angle = (turn - 2 * L).astype(F32) * (math.pi / (2 * L))
                    for c, w in enumerate([jnp.cos(angle) * scale, jnp.sin(angle) * -scale]):
                        j = 4 * i + 2 * p + c
                        dft_s[j * C // 2:(j + 1) * C // 2, :] = pltpu.bitcast(w.astype(BF16), U32)
            small[0].wait()
            tp = shift_s[...].astype(F32)
            for b in range(NCB):
                taps_s[b, 0:4, :] = tp[:, b * CB:(b + 1) * CB]
            for cp in kv_copies(0):
                cp.wait()

        with scope("p0_pro"):
            for m in range(NL):
                kv_chunk(0, m)
            for cp in small[1:]:
                cp.wait()
            dsk = ssmd_s[...].astype(F32)
            cf = c_s[...].astype(F32)
            sc = jnp.broadcast_to(cf * jax.nn.sigmoid(cf), (16, D)).astype(BF16)
            for b in range(NCB):
                dsk_s[b * CB:(b + 1) * CB, :] = jnp.broadcast_to(dsk[b:b + 1], (CB, CB)).T
                sc_s[b] = sc[:, b * CB:(b + 1) * CB]
            bspf_s[...] = bsp_s[...].astype(F32)

        with scope("p0_main"):
            @pl.loop(0, NCB - 1)
            def _(b):
                conv_block(b, False)

        with scope("p0_epi"):
            conv_block(NCB - 1, True)
            sa, ca, ga, sb, cb_ = (acc_s[:, i * D:(i + 1) * D] for i in range(5))
            mod_s[0] = ga * (1.0 + ca)
            mod_s[1] = ga * sa
            mod_s[2] = 1.0 + cb_
            mod_s[3] = sb

        def split(tiles):
            return tiles[:KH], tiles[KH:]

        def store_h(h):
            blocks = {(i, j): split([h[j * T1 // 2:(j + 1) * T1 // 2, b * CB:(b + 1) * CB]
                                     for b in range(NCB)])[i] for i in range(2) for j in range(2)}
            for i, op in enumerate(_rhs_operands(blocks, 2)):
                h_s[i, :, :KT[i] * CB] = jnp.concatenate(op[0, 0][:KT[i]], axis=1).astype(BF16)

        def store_w_in(z, spare):
            marks = [z[r:r + 8, :C] for r in range(0, FH, FH // wt)]
            for r in range(0, FH // 2, WR):
                if r % (FH // 2 // wt) == 0:
                    wsum_s[spare, 0, 0:8, :] = pltpu.bitcast(marks.pop(0), U32)
                words = [[wint_s[1 - i, b, r:r + WR, :] for b in range(NCB)] for i in range(2)]
                lo, hi = [_lhs_operands({(i, j): split([f(w) for w in words[i]])[j]
                                         for i in range(2) for j in range(2)}, 2) for f in (low, high)]
                for i in range(7):
                    for b in range(KT[i]):
                        if (i, b) not in W_SAME:
                            wsum_s[i, b, r:r + WR, :] = pltpu.pack_elementwise(
                                [lo[i][0, 0][b], hi[i][0, 0][b]], packed_dtype=BF16)

        c1 = math.sqrt(2.0 / math.pi)
        c2 = c1 * 0.044715

        def gelu2(x):
            return x * jnp.tanh((x * x * c2 + c1) * x) + x

        def fold8(x):
            return jnp.sum(x.reshape(x.shape[0] // 8, 8, x.shape[1]), axis=0)

        def proj_in_plain(i, h):
            return jnp.concatenate([lax.dot_general(
                jnp.concatenate([bf(wint_s.at[i, b, r:r + FH // 4]) for b in range(NCB)], axis=1),
                h, NT, preferred_element_type=F32) for r in (0, FH // 4)], axis=0)

        def proj_in():
            prods = []
            for i in range(7):
                w = jnp.concatenate([bf(wint_s.at[W_SAME[i, b]] if (i, b) in W_SAME else wsum_s.at[i, b])
                                     for b in range(KT[i])], axis=1)
                prods.append({(0, 0): lax.dot_general(w, h_s[i, :, :KT[i] * CB], NT,
                                                      preferred_element_type=F32)})
            z = _combine(prods, 2)
            marks = [p[0, 0][r:r + 8] for p in prods[n0:n1] for r in range(0, FH, FH * (n1 - n0) // nt)] if nt else ()
            return [jnp.concatenate([z[i, 0], z[i, 1]], axis=1) for i in range(2)] + [marks]

        def gate_branch(z):
            z = gelu2(z)
            z = z - z[0:1]
            z2f_s[...] = z
            st_s[0] = fold8(z)
            st_s[1] = fold8(z * z)

        def value_branch(t, z):
            z1_s[t] = (z if gelu_late else gelu2(z)).astype(BF16)

        def normalize(t, marks=()):
            mean = jnp.sum(st_s[0], axis=0, keepdims=True) * (1.0 / FH)
            var = jnp.sum(st_s[1], axis=0, keepdims=True) * (1.0 / FH) - mean * mean
            rs = lax.rsqrt(jnp.maximum(var, 0.0) + 4.0 * EPS)
            hf, hs = FH // 2, T1 // 2
            n = hf // max(len(marks), 1)
            for r in range(0, hf, n):
                zn = [(z2f_s[i * hf + r:i * hf + r + n, :] - mean) * rs for i in range(2)]
                blocks = {(i, j): zn[i][:, j * hs:(j + 1) * hs] for i in range(2) for j in range(2)}
                for i, a in enumerate(_lhs_operands(blocks, 2) if lvl1 else _quads(blocks, 2)):
                    z2_s[i, t // (NT1 // 2), pl.ds(pl.multiple_of(t % (NT1 // 2) * (hf + zp) + r, 8), n), :] = a[0, 0]
                if marks:
                    z2_s[spare_s[0], 0, 0:8, :] = marks[r // n]

        with scope("p1_pro"):
            h0 = jnp.concatenate([residual(0, r, RG0, qn_s[r:r + RG0, :]) for r in range(0, T1, RG0)],
                                 axis=0).astype(BF16)
        with scope("p1_pro2"):
            with scope("w_a"):
                for cp in win_copies(1) + [q_copy(1)]:
                    cp.wait()
            gate_branch(proj_in_plain(1, h0))
            store_h(elementwise(1))
            with scope("w_b"):
                for cp in win_copies(0):
                    cp.wait()
            with scope("pro_b"):
                z1 = proj_in_plain(0, h0)
                value_branch(0, z1)
                store_w_in(z1, spare_s[0])

        with scope("p1_main"):
            @pl.loop(1, NT1)
            def _(t):
                @pl.when(t + 1 < NT1)
                def _():
                    q_copy(t + 1).wait()

                z2, z1, marks = proj_in()
                normalize(t - 1, marks)
                gate_branch(z2)
                value_branch(t, z1)
                store_h(elementwise(jnp.minimum(t + 1, NT1 - 1)))

        with scope("p1_epi"):
            cp_wout.wait()
            cp_wgate.wait()
            wsp_copy(0).wait()
            normalize(NT1 - 1)
            sc = jnp.concatenate([sc_s[b] for b in range(NCB)], axis=1)
            mod_s[4] = 0.5 * jnp.dot(sc, wgate_s[...], preferred_element_type=F32)[0:8]

        def spatial(u):
            hs = T1 // 2
            nh = NT1 // 2

            def w_block(si, ti):
                rows = pl.ds(pl.multiple_of(u * TB + ti * HT, HT), HT)
                t0 = (si % 2) * nh
                return jnp.concatenate(
                    [wsp_s[rows, t * T1 + (si // 2) * hs:t * T1 + (si // 2 + 1) * hs]
                     for t in range(t0, t0 + nh)], axis=1).astype(F32)

            def z_operand(i):
                return {(p, q): jnp.concatenate([z2_s[i, q, t * (2 * HF + zp) + p * HF:t * (2 * HF + zp) + (p + 1) * HF, :]
                                                 for t in range(nh)], axis=1)
                        for p in range(2) for q in range(2)}

            def dot_nt(a, b):
                if s16:
                    a, b = a.astype(BF16), b.astype(BF16)
                return lax.dot_general(a, b, NT, preferred_element_type=F32)

            w = {(si, ti): w_block(si, ti) for si in range(4) for ti in range(4)}
            if not lvl1:
                z = {(2 * (i // 2) + p, 2 * (i % 2) + q): v for i in range(4) for (p, q), v in z_operand(i).items()}
                return _assemble(_strassen(z, w, 4, dot_nt), 4)
            return _assemble(_combine([_strassen(z_operand(i), op, 2, dot_nt)
                                       for i, op in enumerate(_rhs_operands(w, 4))], 4), 4)

        def gated(u):
            g = spatial(u)
            bias = jnp.concatenate([bspf_s[pl.ds(u * (TB // C) + i, 1), :] for i in range(TB // C)], axis=1)
            z1 = jnp.concatenate([z1_s[u * (TB // T1) + i] for i in range(TB // T1)], axis=1).astype(F32)
            m_s[:FH, :] = gelu2(z1) * (g + bias)

        def proj_out(u, to, eager):
            so = SO if to == 512 else 2
            groups = {2: [range(4), range(4, 7)], 4: [range(2), range(2, 4), range(4, 6), range(6, 7)]}[so]
            hd, ht = D // so, to // so

            def dot(a, b):
                n = min(len(a), len(b))
                return jnp.dot(jnp.concatenate(a[:n], axis=1).astype(BF16),
                               jnp.concatenate(b[:n], axis=0).astype(BF16), preferred_element_type=F32)

            for j in range(0, TB, to):
                a = {(i, p): [woutt_s[f, i * hd:(i + 1) * hd, :] for f in groups[p]]
                     for i in range(so) for p in range(so)}
                b = {(p, i): [m_s[f * 128:(f + 1) * 128, j + i * ht:j + (i + 1) * ht] for f in groups[p]]
                     for i in range(so) for p in range(so)}
                o = _assemble(_strassen(a, b, so, dot), so)
                for i in range(0, to, TW):
                    t = u * (TB // TW) + (j + i) // TW
                    rows = pl.ds(pl.multiple_of(t * TW, TW), TW)
                    o_s[rows, :] = (x_s[rows, :] + row(4, TW) * o[:, i:i + TW].T).astype(BF16)
                    if eager:
                        out_copy(t, TW).start()

        with scope("p2_pro"):
            gated(0)
            for j in range(FP // 128):
                woutt_s[j] = wout_s[j * 128:(j + 1) * 128, :].astype(F32).T

        with scope("p2_main"):
            @pl.loop(1, S // TB)
            def _(u):
                wsp_copy(u).wait()
                with scope("p2_it"):
                    proj_out(u - 1, TO, False)
                    gated(u)
                if not olate:
                    out_copy((u - 1) * (TB // TW), TB).start()

        with scope("p2_epi"):
            if olate:
                out_copy(0, S - TB).start()
            proj_out(S // TB - 1, TE, True)

        with scope("out_wait"):
            if olate:
                out_copy(0, S - TB).wait()
            else:
                for u in range(S // TB - 1):
                    out_copy(u * (TB // TW), TB).wait()
            for t in range((S - TB) // TW, S // TW):
                out_copy(t, TW).wait()

    vm = pltpu.VMEM
    scratch = [
        vm((S, D), BF16), vm((NCB, S // 2 + KPAD, CB), U32), vm((NCB, S // 2, CB), U32),
        vm((NCB * S // 2, C), U32), vm((2, NCB, FH // 2, CB), U32), vm((S, S), BF16),
        vm((FP, D), BF16), vm((NCB, CB, 5 * D), BF16), vm((D, D), BF16), vm((4 * C, C), U32),
        vm((D, CB), F32), vm((NC * CB // 2, C), U32), vm((NL, 2, D, C), F32), vm((NCB, T1, CB), F32),
        vm((FP // 128, D, 128), F32), vm((8, KH, FH // 2, CB), U32), vm((S, D), F32), vm((T1, D), F32),
        vm((7, T1 // 2, KH * CB), BF16), vm((FH, T1), F32), vm((NT1, FH, T1), BF16),
        vm((zn, 2, NT1 // 2 * (FH // 2 + zp) + zq, T1 // 2), F32), vm((FP, TB), F32), vm((S, D), BF16),
        vm((2, 8, T1), F32), vm((8, 8, D), F32), vm((8, 5 * D), F32), vm((NCB + pa, 8, CB), F32),
        vm((NC, C), F32), vm((NCB, 16, CB), BF16), vm((4, D), BF16), vm((NCB, CB), BF16),
        vm((NC, C), BF16), vm((1, D), BF16),
        pltpu.SemaphoreType.DMA((10 + 4 * NCB + NT1 + S // TB + 6,)), pltpu.SemaphoreType.DMA((S // TW,)),
        pltpu.SMEM((1,), jnp.int32),
    ]

    @jax.jit
    def fn(A_q, A_k, A_v, A_shift_k, A_ssm_k, A_ssm_D, B_x, B_w_in, B_w_sp, B_b_sp, B_w_out, c, w_mod):
        del B_x
        out = pl.pallas_call(
            kernel,
            out_shape=jax.ShapeDtypeStruct((S, D), BF16),
            in_specs=[pl.BlockSpec(memory_space=pltpu.HBM)] * 12,
            out_specs=pl.BlockSpec(memory_space=pltpu.HBM),
            scratch_shapes=scratch,
            compiler_params=pltpu.CompilerParams(vmem_limit_bytes=120 * 2**20, flags=flags),
        )(A_q.reshape(S, D), A_k.reshape(S, D), A_v.reshape(S, D), A_shift_k.T,
          A_ssm_k.reshape(D // 8, 8, NC, C).transpose(0, 2, 1, 3).reshape(NCB * S, C),
          A_ssm_D.reshape(NCB, CB), B_w_in.T, B_w_sp, B_b_sp.reshape(NC, C), B_w_out, c, w_mod)
        return out.reshape(1, S, D)

    return fn


pallas_adaLN_cond__ssm_conv_h3__mixer_gmlp__prompt_kernel = make()
```

```python
import contextlib
import math

import jax
import jax.numpy as jnp
import numpy as np
from jax import lax
from jax.experimental import pallas as pl
from jax.experimental.pallas import tpu as pltpu

S, D, FH = 2048, 640, 864
C = 128
NC = S // C
CB = 128
NCB = D // CB
NG = CB // 8
FP = 896
KH = 3
KT = (3, 2, 3, 2, 2, 3, 3)
W_SAME = {(0, 2): (0, 2), (2, 2): (1, 2), (3, 0): (0, 3), (3, 1): (0, 4),
          (5, 0): (1, 0), (5, 1): (1, 1), (5, 2): (1, 2)}
KPAD = 32
EPS = 1e-5
F32, BF16, U32 = jnp.float32, jnp.bfloat16, jnp.uint32
NT = (((1,), (1,)), ((), ()))


L = 2 * C
NL = S // L


def _tree_sum(xs):
    xs = list(xs)
    while len(xs) > 1:
        xs = [xs[i] + xs[i + 1] if i + 1 < len(xs) else xs[i] for i in range(0, len(xs), 2)]
    return xs[0]


def _quads(x, n):
    h = n // 2
    return [{(i, j): x[i + a * h, j + b * h] for i in range(h) for j in range(h)}
            for a in range(2) for b in range(2)]


def _mix(x, y, sign):
    if isinstance(x, list):
        n = min(len(x), len(y))
        return ([_mix(p, q, sign) for p, q in zip(x, y)] + x[n:]
                + [q if sign > 0 else -q for q in y[n:]])
    return x + y if sign > 0 else x - y


def _add(x, y):
    return {k: _mix(x[k], y[k], 1) for k in x}


def _sub(x, y):
    return {k: _mix(x[k], y[k], -1) for k in x}


def _lhs_operands(a, n):
    a11, a12, a21, a22 = _quads(a, n)
    return [_add(a21, a22), _add(a11, a12), _add(a11, a22), a22, _sub(a12, a22), a11, _sub(a21, a11)]


def _rhs_operands(b, n):
    b11, b12, b21, b22 = _quads(b, n)
    return [b11, b22, _add(b11, b22), _sub(b11, b21), _add(b21, b22), _sub(b12, b22), _add(b11, b12)]


def _combine(products, n):
    m2, m5, m1, m4, m7, m3, m6 = products
    quads = [_add(_sub(_sub(m1, m5), m4), m7), _add(m3, m5),
             _sub(m2, m4), _add(_add(_sub(m1, m2), m3), m6)]
    h, out = n // 2, {}
    for (p, q), c in zip([(0, 0), (0, 1), (1, 0), (1, 1)], quads):
        out.update({(i + p * h, j + q * h): v for (i, j), v in c.items()})
    return out


def _strassen(a, b, n, dot):
    if n == 1:
        return {(0, 0): dot(a[0, 0], b[0, 0])}
    return _combine([_strassen(p, q, n // 2, dot)
                     for p, q in zip(_lhs_operands(a, n), _rhs_operands(b, n))], n)


def _assemble(blocks, n):
    return jnp.concatenate([jnp.concatenate([blocks[i, j] for j in range(n)], axis=1)
                            for i in range(n)], axis=0)


def make(T1=256, TB=512, TO=512, RG=256, scopes=False, flags={'XLA_TPU_EVENLY_DISTRIBUTE_CRITICAL_NODES': True}, gauss=1, wait_at=8, mod_at=12, nmod=4, gelu_late=True, SO=2, TW=128, WR=8, wt=18, UN=1, pk=1, order='pngveh', po='0123456', h32=False, nt=0, x16=False, pa=0, wlate=False, TE=256, olate=False, zp=16, zq=0, zn=7, lvl1=True, n0=0, n1=3, RG0=256, o16=True, s16=False):
    NT1 = S // T1
    HF, HS, HT = FH // 4, 128, TB // 4
    SB = 4 * HS
    NSB = S // SB

    def scope(name):
        return jax.named_scope(name) if scopes else contextlib.nullcontext()

    def kernel(q_hbm, k_hbm, v_hbm, shift_hbm, ssmk_hbm, ssmd_hbm, win_hbm, wsp_hbm, bsp_hbm,
               wout_hbm, c_hbm, wmod_hbm, out_hbm,
               q_s, k_s, v_s, ssmk_s, wint_s, wsp_s, wout_s, wmod_s, wgate_s, dft_s,
               dsk_s, kvt_s, yt_s, y_s, woutt_s, wsum_s, x_s, qn_s, h_s, z2f_s, z1_s, z2_s, m_s, o_s,
               st_s, mod_s, acc_s, taps_s, bspf_s, sc_s, shift_s, ssmd_s, bsp_s, c_s,
               sem_in, sem_out, spare_s):
        spare_s[0] = 7
        o_conv = 6
        o_big = o_conv + 4 * NCB
        o_q = o_big + 4
        o_wsp = o_q + NT1
        o_wout = o_wsp + S // TB

        def copy(src, dst, i):
            return pltpu.make_async_copy(src, dst, sem_in.at[i])

        small = [copy(a, b, i) for i, (a, b) in enumerate(
            [(shift_hbm, shift_s), (ssmd_hbm, ssmd_s), (c_hbm, c_s), (bsp_hbm, bsp_s)])]

        def kv_copies(b):
            ch = pl.ds(pl.multiple_of(b * CB, CB), CB)
            return [copy(k_hbm.at[:, ch], k_s.bitcast(BF16).at[b, pl.ds(2 * KPAD, S), :], o_conv + 4 * b),
                    copy(v_hbm.at[:, ch], v_s.bitcast(BF16).at[b], o_conv + 4 * b + 1)]

        def ssmk_copy(b):
            r = pl.ds(pl.multiple_of(b * S, S), S)
            return copy(ssmk_hbm.at[r, :], ssmk_s.bitcast(BF16).at[r, :], o_conv + 4 * b + 2)

        def wmod_copy(b):
            r = pl.ds(pl.multiple_of(b * CB, CB), CB)
            return copy(wmod_hbm.at[r, pl.ds(0, 5 * D)], wmod_s.at[b], o_conv + 4 * b + 3)

        def win_copies(i):
            return [copy(win_hbm.at[pl.ds(i * FH, FH), pl.ds(j * CB, CB)],
                         wint_s.bitcast(BF16).at[i, j], o_big + i) for j in range(NCB)]

        cp_wout = copy(wout_hbm, wout_s.at[pl.ds(0, FH), :], o_big + 2)
        cp_wgate = copy(wmod_hbm.at[:, pl.ds(5 * D, D)], wgate_s, o_big + 3)

        def q_copy(t):
            r = pl.ds(pl.multiple_of(t * T1, T1), T1)
            return copy(q_hbm.at[r, :], q_s.at[r, :], o_q + t)

        def wsp_copy(u):
            r = pl.ds(pl.multiple_of(u * TB, TB), TB)
            return copy(wsp_hbm.at[r, :], wsp_s.at[r, :], o_wsp + u)

        def out_copy(t, n):
            r = pl.ds(pl.multiple_of(t * TW, TW), n)
            return pltpu.make_async_copy(o_s.at[r, :], out_hbm.at[r, :], sem_out.at[t])

        for cp in small[:1] + kv_copies(0) + small[1:]:
            cp.start()
        for b in range(NCB):
            ssmk_copy(b).start()
            if b + 1 < NCB:
                for cp in kv_copies(b + 1):
                    cp.start()
        q_copy(0).start()
        for b in range(NCB):
            wmod_copy(b).start()
        for cp in win_copies(1) + [q_copy(1)] + win_copies(0):
            cp.start()
        for t in range(2, NT1):
            q_copy(t).start()
        cp_wout.start()
        cp_wgate.start()
        for u in range(1 if wlate else S // TB):
            wsp_copy(u).start()

        def bf(ref):
            return pltpu.bitcast(ref[...], BF16)

        def dft(i, n):
            return pltpu.bitcast(dft_s[i * C // 2:(i + n) * C // 2, :], BF16)

        def low(w):
            return pltpu.bitcast(w << 16, F32)

        def high(w):
            return pltpu.bitcast(w & np.uint32(0xFFFF0000), F32)

        def pack(lo, hi):
            bits = pltpu.bitcast(jnp.concatenate([lo, hi], axis=1).astype(BF16).astype(F32), U32)
            return (bits[:, :C] >> 16) | bits[:, C:]

        def kv_chunk(b, m):
            kw = [k_s[b, pl.ds(KPAD + m * C + j, C), :] for j in range(-2, 1)]
            vw = v_s[b, m * C:(m + 1) * C, :]
            kk = [high(kw[0]), low(kw[1]), high(kw[1]), low(kw[2]), high(kw[2])]
            for p, vv in enumerate((low(vw), high(vw))):
                kv = _tree_sum([kk[3 + p - t] * taps_s[b, t:t + 1, :] for t in range(4)]) * vv
                halves = [kv[:C // 2], kv[C // 2:]]
                w = pltpu.bitcast(pack(halves[p], halves[1 - p]), BF16)
                kvt_s[(2 * m + p) * 64:(2 * m + p + 1) * 64, :] = pltpu.bitcast(w.T, U32)

        def forward(b, g):
            base = pl.multiple_of(b * (S // 2), S // 2) + g * NC * 4
            top = lax.broadcasted_iota(jnp.int32, (8, C), 0) < 4
            words = [ssmk_s[pl.ds(base + 4 * i, 8), :] if i % 4 < 3 else None for i in range(NC)]
            t0, t1 = [jnp.concatenate([jnp.where(top, words[i + j], words[i + j + 1])
                                       for i in range(0, NC, 4)], axis=0) for j in range(2)]
            odd = (lax.broadcasted_iota(jnp.int32, t0.shape, 1) & 1) == 1
            kt = [jnp.where(odd, pltpu.roll(t1, 1, 1), t0), jnp.where(odd, t0, pltpu.roll(t1, C - 1, 1))]
            out = []
            for p in range(2):
                xt = jnp.concatenate(
                    [jnp.where(top, kvt_s[pl.ds((2 * m + p) * 64 + 4 * g, 8), :],
                               kvt_s[pl.ds((2 * m + 2 + p) * 64 + 4 * g - 4, 8), :])
                     for m in range(0, NL, 2)], axis=0)
                lhs = jnp.concatenate([t[i:i + 8] for i in range(0, 4 * NL, 8) for t in (kt[p], xt)], axis=0)
                out.append([jnp.dot(pltpu.bitcast(lhs, BF16), dft(2 * p + c, 1), preferred_element_type=F32)
                            for c in range(2)])
            return out

        def butterfly(a, b):
            return (a[0] + b[0], a[1] + b[1]), (a[0] - b[0], a[1] - b[1])

        def product(b, g, f):
            def part(i, m, p):
                r = (m // 2 * 4 + i * 2 + m % 2) * 8
                return f[p][0][r:r + 8], f[p][1][r:r + 8]

            def window(m, p):
                re, im = part(0, m, p)
                if m:
                    pre, pim = part(0, m - 1, p)
                    return re - pim, im + pre
                if p == 0:
                    re = re + dsk_s[pl.ds(pl.multiple_of(b * CB + g * 8, 8), 8), :]
                return re, im

            kf = [butterfly(window(m, 0), window(m, 1)) for m in range(NL)]
            xf = [butterfly(part(1, m, 0), part(1, m, 1)) for m in range(NL)]
            out = []
            for i in range(NL):
                z = []
                for h in range(2):
                    terms = [(xf[j][h], kf[i - j][h]) for j in range(i + 1)]
                    if i >= gauss:
                        p1 = _tree_sum([x[0] * k[0] for x, k in terms])
                        p2 = _tree_sum([x[1] * k[1] for x, k in terms])
                        p3 = _tree_sum([(x[0] + x[1]) * (k[0] + k[1]) for x, k in terms])
                        z.append((p1 - p2, p3 - (p1 + p2)))
                    else:
                        z.append((_tree_sum([x[0] * k[0] - x[1] * k[1] for x, k in terms]),
                                  _tree_sum([x[0] * k[1] + x[1] * k[0] for x, k in terms])))
                out.append(butterfly(*z))
            return out

        def inverse(b, g, z):
            rows = pl.ds(pl.multiple_of(b * CB + g * 8, 8), 8)
            for p in range(2):
                zp = jnp.concatenate([jnp.concatenate([z[i][p][c] for i in range(NL)], axis=0)
                                      for c in range(2)], axis=1)
                y = jnp.dot(zp.astype(BF16), dft(4 + 2 * p, 2), preferred_element_type=F32)
                for i in range(NL):
                    yt_s[i, p, rows, :] = y[i * 8:(i + 1) * 8]

        def modulation(blocks):
            with scope("w_mod%d" % len(blocks)):
                for b in blocks:
                    wmod_copy(b).wait()
            acc_s[...] += _tree_sum([jnp.dot(sc_s[b], wmod_s[b], preferred_element_type=F32)[0:8]
                                     for b in blocks])

        def row(i, n):
            return jnp.concatenate([mod_s[i]] * (n // 8), axis=0)

        def time_major(t, blocks):
            for b in blocks:
                for p in range(2):
                    y_s[b, pl.ds(p, C, stride=2), :] = yt_s[t, p, b * CB:(b + 1) * CB, :].T

        def standardize(x):
            xc = x - jnp.sum(x, axis=-1, keepdims=True) * (1.0 / D)
            return xc * lax.rsqrt(jnp.sum(xc * xc, axis=-1, keepdims=True) * (1.0 / D) + EPS)

        def residual(t, r, n, qn=None):
            rows = pl.ds(pl.multiple_of(t * T1 + r, n), n)
            q = q_s[rows, :].astype(F32)
            y = jnp.concatenate([y_s[b, r:r + n, :] for b in range(NCB)], axis=1)
            x = q + ((standardize(q) if qn is None else qn) * row(0, n) + row(1, n)) * y
            x_s[rows, :] = x.astype(x_s.dtype)
            return standardize(x) * row(2, n) + row(3, n)

        def elementwise(t):
            time_major(t, range(NCB))
            return residual(t, 0, T1)

        def conv_block(b, last):
            with scope('w_ssmk'):
                ssmk_copy(b).wait()
            f = {0: forward(b, 0)}
            for g in range(NG):
                if g + 1 < NG:
                    f[g + 1] = forward(b, g + 1)
                if g == wait_at and not last:
                    with scope("w_kv"):
                        for cp in kv_copies(b + 1):
                            cp.wait()
                if g == mod_at and last:
                    q_copy(0).wait()
                    modulation(range(nmod))
                    time_major(0, range(NCB - 1))
                    for r in range(0, T1, RG):
                        qn_s[r:r + RG, :] = standardize(q_s[r:r + RG, :].astype(F32))
                inverse(b, g, product(b, g, f.pop(g)))
            if last:
                time_major(0, [NCB - 1])
                if nmod < NCB:
                    modulation(range(nmod, NCB))
            else:
                for m in range(NL):
                    kv_chunk(b + 1, m)

        with scope("p0_wait0"):
            for b in range(NCB):
                k_s[b, KPAD - 8:KPAD, :] = jnp.zeros((8, CB), U32)
            acc_s[...] = jnp.zeros(acc_s.shape, F32)
            m_s[FH:, :] = jnp.zeros((FP - FH, TB), F32)
            wout_s[FH:, :] = jnp.zeros((FP - FH, D), BF16)
            row_id = lax.broadcasted_iota(jnp.int32, (C, C), 0)
            col_id = lax.broadcasted_iota(jnp.int32, (C, C), 1)
            for p in range(2):
                source = ((row_id & 1) ^ p) * C + (row_id & -2) + p
                for i, (sample, freq, scale) in enumerate([(source, col_id, 1.0),
                                                           (2 * col_id + p, row_id, 1.0 / L)]):
                    turn = (sample * (4 * freq + 1) + 2 * L) & (4 * L - 1)
                    angle = (turn - 2 * L).astype(F32) * (math.pi / (2 * L))
                    for c, w in enumerate([jnp.cos(angle) * scale, jnp.sin(angle) * -scale]):
                        j = 4 * i + 2 * p + c
                        dft_s[j * C // 2:(j + 1) * C // 2, :] = pltpu.bitcast(w.astype(BF16), U32)
            small[0].wait()
            tp = shift_s[...].astype(F32)
            for b in range(NCB):
                taps_s[b, 0:4, :] = tp[:, b * CB:(b + 1) * CB]
            for cp in kv_copies(0):
                cp.wait()

        with scope("p0_pro"):
            for m in range(NL):
                kv_chunk(0, m)
            for cp in small[1:]:
                cp.wait()
            dsk = ssmd_s[...].astype(F32)
            cf = c_s[...].astype(F32)
            sc = jnp.broadcast_to(cf * jax.nn.sigmoid(cf), (16, D)).astype(BF16)
            for b in range(NCB):
                dsk_s[b * CB:(b + 1) * CB, :] = jnp.broadcast_to(dsk[b:b + 1], (CB, CB)).T
                sc_s[b] = sc[:, b * CB:(b + 1) * CB]
            bspf_s[...] = bsp_s[...].astype(F32)

        with scope("p0_main"):
            @pl.loop(0, NCB - 1)
            def _(b):
                conv_block(b, False)

        with scope("p0_epi"):
            conv_block(NCB - 1, True)
            sa, ca, ga, sb, cb_ = (acc_s[:, i * D:(i + 1) * D] for i in range(5))
            mod_s[0] = ga * (1.0 + ca)
            mod_s[1] = ga * sa
            mod_s[2] = 1.0 + cb_
            mod_s[3] = sb

        def split(tiles):
            return tiles[:KH], tiles[KH:]

        def store_h(h):
            blocks = {(i, j): split([h[j * T1 // 2:(j + 1) * T1 // 2, b * CB:(b + 1) * CB]
                                     for b in range(NCB)])[i] for i in range(2) for j in range(2)}
            for i, op in enumerate(_rhs_operands(blocks, 2)):
                if h32:
                    for b in range(KT[i]):
                        h_s[i, b] = op[0, 0][b].astype(BF16)
                    continue
                h_s[i, :, :KT[i] * CB] = jnp.concatenate(op[0, 0][:KT[i]], axis=1).astype(BF16)

        def store_w_in(z, spare):
            marks = [z[r:r + 8, :C] for r in range(0, FH, FH // wt)]
            for r in range(0, FH // 2, WR):
                if r % (FH // 2 // wt) == 0:
                    wsum_s[spare, 0, 0:8, :] = pltpu.bitcast(marks.pop(0), U32)
                words = [[wint_s[1 - i, b, r:r + WR, :] for b in range(NCB)] for i in range(2)]
                lo, hi = [_lhs_operands({(i, j): split([f(w) for w in words[i]])[j]
                                         for i in range(2) for j in range(2)}, 2) for f in (low, high)]
                for i in range(7):
                    for b in range(KT[i]):
                        if (i, b) not in W_SAME:
                            wsum_s[i, b, r:r + WR, :] = pack(lo[i][0, 0][b], hi[i][0, 0][b])

        c1 = math.sqrt(2.0 / math.pi)
        c2 = c1 * 0.044715

        def gelu2(x):
            return x * jnp.tanh((x * x * c2 + c1) * x) + x

        def fold8(x):
            return jnp.sum(x.reshape(x.shape[0] // 8, 8, x.shape[1]), axis=0)

        def proj_in_plain(i, h):
            return jnp.concatenate([lax.dot_general(
                jnp.concatenate([bf(wint_s.at[i, b, r:r + FH // 4]) for b in range(NCB)], axis=1),
                h, NT, preferred_element_type=F32) for r in (0, FH // 4)], axis=0)

        def load_h(i):
            if h32:
                return jnp.concatenate([h_s[i, b] for b in range(KT[i])], axis=1)
            return h_s[i, :, :KT[i] * CB]

        def proj_in():
            prods = {}
            for i in map(int, po):
                w = jnp.concatenate([bf(wint_s.at[W_SAME[i, b]] if (i, b) in W_SAME else wsum_s.at[i, b])
                                     for b in range(KT[i])], axis=1)
                prods[i] = {(0, 0): lax.dot_general(w, load_h(i), NT, preferred_element_type=F32)}
            prods = [prods[i] for i in range(7)]
            z = _combine(prods, 2)
            marks = [p[0, 0][r:r + 8] for p in prods[n0:n1] for r in range(0, FH, FH * (n1 - n0) // nt)] if nt else ()
            return [jnp.concatenate([z[i, 0], z[i, 1]], axis=1) for i in range(2)] + [marks]

        def gate_branch(z):
            z = gelu2(z)
            z = z - z[0:1]
            z2f_s[...] = z
            st_s[0] = fold8(z)
            st_s[1] = fold8(z * z)

        def value_branch(t, z):
            z1_s[t] = (z if gelu_late else gelu2(z)).astype(BF16)

        def normalize(t, marks=()):
            mean = jnp.sum(st_s[0], axis=0, keepdims=True) * (1.0 / FH)
            var = jnp.sum(st_s[1], axis=0, keepdims=True) * (1.0 / FH) - mean * mean
            rs = lax.rsqrt(jnp.maximum(var, 0.0) + 4.0 * EPS)
            hf, hs = FH // 2, T1 // 2
            n = hf // max(len(marks), 1)
            for r in range(0, hf, n):
                zn = [(z2f_s[i * hf + r:i * hf + r + n, :] - mean) * rs for i in range(2)]
                blocks = {(i, j): zn[i][:, j * hs:(j + 1) * hs] for i in range(2) for j in range(2)}
                for i, a in enumerate(_lhs_operands(blocks, 2) if lvl1 else _quads(blocks, 2)):
                    z2_s[i, t // (NT1 // 2), pl.ds(pl.multiple_of(t % (NT1 // 2) * (hf + zp) + r, 8), n), :] = a[0, 0]
                if marks:
                    z2_s[spare_s[0], 0, 0:8, :] = marks[r // n]

        with scope("p1_pro"):
            h0 = jnp.concatenate([residual(0, r, RG0, qn_s[r:r + RG0, :]) for r in range(0, T1, RG0)],
                                 axis=0).astype(BF16)
        with scope("p1_pro2"):
            with scope("w_a"):
                for cp in win_copies(1) + [q_copy(1)]:
                    cp.wait()
            gate_branch(proj_in_plain(1, h0))
            store_h(elementwise(1))
            with scope("w_b"):
                for cp in win_copies(0):
                    cp.wait()
            with scope("pro_b"):
                z1 = proj_in_plain(0, h0)
                value_branch(0, z1)
                store_w_in(z1, spare_s[0])

        def mixer_in(t, nxt=False):
            h = None
            for c in order:
                if c == 'n':
                    normalize(t - 1)
                if c == 'p':
                    z2, z1, _ = proj_in()
                if c == 'g':
                    gate_branch(z2)
                if c == 'v':
                    value_branch(t, z1)
                if c == 'e' and nxt:
                    h = elementwise(t + 1)
                if c == 'h' and nxt:
                    store_h(h)

        with scope("p1_main"):
            @pl.loop(0, (NT1 - 2) // UN)
            def _(i):
                for u in range(UN):
                    q_copy(2 + i * UN + u).wait()
                for u in range(UN):
                    t = 1 + i * UN + u
                    mixer_in(t, True)

        with scope("p1_epi"):
            cp_wout.wait()
            cp_wgate.wait()
            wsp_copy(0).wait()
            mixer_in(NT1 - 1)
            normalize(NT1 - 1)
            sc = jnp.concatenate([sc_s[b] for b in range(NCB)], axis=1)
            mod_s[4] = 0.5 * jnp.dot(sc, wgate_s[...], preferred_element_type=F32)[0:8]

        def spatial(u):
            hs = T1 // 2
            nh = NT1 // 2

            def w_block(si, ti):
                rows = pl.ds(pl.multiple_of(u * TB + ti * HT, HT), HT)
                t0 = (si % 2) * nh
                return jnp.concatenate(
                    [wsp_s[rows, t * T1 + (si // 2) * hs:t * T1 + (si // 2 + 1) * hs]
                     for t in range(t0, t0 + nh)], axis=1).astype(F32)

            def z_operand(i):
                return {(p, q): jnp.concatenate([z2_s[i, q, t * (2 * HF + zp) + p * HF:t * (2 * HF + zp) + (p + 1) * HF, :]
                                                 for t in range(nh)], axis=1)
                        for p in range(2) for q in range(2)}

            def dot_nt(a, b):
                if s16:
                    a, b = a.astype(BF16), b.astype(BF16)
                return lax.dot_general(a, b, NT, preferred_element_type=F32)

            w = {(si, ti): w_block(si, ti) for si in range(4) for ti in range(4)}
            if not lvl1:
                z = {(2 * (i // 2) + p, 2 * (i % 2) + q): v for i in range(4) for (p, q), v in z_operand(i).items()}
                return _assemble(_strassen(z, w, 4, dot_nt), 4)
            return _assemble(_combine([_strassen(z_operand(i), op, 2, dot_nt)
                                       for i, op in enumerate(_rhs_operands(w, 4))], 4), 4)

        def gated(u):
            g = spatial(u)
            bias = jnp.concatenate([bspf_s[pl.ds(u * (TB // C) + i, 1), :] for i in range(TB // C)], axis=1)
            z1 = jnp.concatenate([z1_s[u * (TB // T1) + i] for i in range(TB // T1)], axis=1).astype(F32)
            m_s[:FH, :] = gelu2(z1) * (g + bias)

        def proj_out(u, to, eager):
            so = SO if to == 512 else 2
            groups = {2: [range(4), range(4, 7)], 4: [range(2), range(2, 4), range(4, 6), range(6, 7)]}[so]
            hd, ht = D // so, to // so

            def dot(a, b):
                n = min(len(a), len(b))
                return jnp.dot(jnp.concatenate(a[:n], axis=1).astype(BF16),
                               jnp.concatenate(b[:n], axis=0).astype(BF16), preferred_element_type=F32)

            for j in range(0, TB, to):
                a = {(i, p): [woutt_s[f, i * hd:(i + 1) * hd, :] for f in groups[p]]
                     for i in range(so) for p in range(so)}
                b = {(p, i): [m_s[f * 128:(f + 1) * 128, j + i * ht:j + (i + 1) * ht] for f in groups[p]]
                     for i in range(so) for p in range(so)}
                o = _assemble(_strassen(a, b, so, dot), so)
                for i in range(0, to, TW):
                    t = u * (TB // TW) + (j + i) // TW
                    rows = pl.ds(pl.multiple_of(t * TW, TW), TW)
                    o_s[rows, :] = (x_s[rows, :] + row(4, TW) * o[:, i:i + TW].T).astype(BF16)
                    if eager:
                        out_copy(t, TW).start()

        with scope("p2_pro"):
            gated(0)
            for j in range(FP // 128):
                woutt_s[j] = wout_s[j * 128:(j + 1) * 128, :].astype(F32).T

        with scope("p2_main"):
            @pl.loop(1, S // TB)
            def _(u):
                wsp_copy(u).wait()
                with scope("p2_it"):
                    proj_out(u - 1, TO, False)
                    gated(u)
                if not olate:
                    out_copy((u - 1) * (TB // TW), TB).start()

        with scope("p2_epi"):
            if olate:
                out_copy(0, S - TB).start()
            proj_out(S // TB - 1, TE, True)

        with scope("out_wait"):
            if olate:
                out_copy(0, S - TB).wait()
            else:
                for u in range(S // TB - 1):
                    out_copy(u * (TB // TW), TB).wait()
            for t in range((S - TB) // TW, S // TW):
                out_copy(t, TW).wait()

    vm = pltpu.VMEM
    scratch = [
        vm((S, D), BF16), vm((NCB, S // 2 + KPAD, CB), U32), vm((NCB, S // 2, CB), U32),
        vm((NCB * S // 2, C), U32), vm((2, NCB, FH // 2, CB), U32), vm((S, S), BF16),
        vm((FP, D), BF16), vm((NCB, CB, 5 * D), BF16), vm((D, D), BF16), vm((4 * C, C), U32),
        vm((D, CB), F32), vm((NC * CB // 2, C), U32), vm((NL, 2, D, C), F32), vm((NCB, T1, CB), F32),
        vm((FP // 128, D, 128), F32), vm((8, KH, FH // 2, CB), U32), vm((S, D), F32), vm((T1, D), F32),
        vm((7, KH, T1 // 2, CB) if h32 else (7, T1 // 2, KH * CB), BF16), vm((FH, T1), F32), vm((NT1, FH, T1), BF16),
        vm((zn, 2, NT1 // 2 * (FH // 2 + zp) + zq, T1 // 2), F32), vm((FP, TB), F32), vm((S, D), BF16),
        vm((2, 8, T1), F32), vm((8, 8, D), F32), vm((8, 5 * D), F32), vm((NCB + pa, 8, CB), F32),
        vm((NC, C), F32), vm((NCB, 16, CB), BF16), vm((4, D), BF16), vm((NCB, CB), BF16),
        vm((NC, C), BF16), vm((1, D), BF16),
        pltpu.SemaphoreType.DMA((10 + 4 * NCB + NT1 + S // TB + 6,)), pltpu.SemaphoreType.DMA((S // TW,)),
        pltpu.SMEM((1,), jnp.int32),
    ]

    @jax.jit
    def fn(A_q, A_k, A_v, A_shift_k, A_ssm_k, A_ssm_D, B_x, B_w_in, B_w_sp, B_b_sp, B_w_out, c, w_mod):
        del B_x
        out = pl.pallas_call(
            kernel,
            out_shape=jax.ShapeDtypeStruct((S, D), BF16),
            in_specs=[pl.BlockSpec(memory_space=pltpu.HBM)] * 12,
            out_specs=pl.BlockSpec(memory_space=pltpu.HBM),
            scratch_shapes=scratch,
            compiler_params=pltpu.CompilerParams(vmem_limit_bytes=120 * 2**20, flags=flags),
        )(A_q.reshape(S, D), A_k.reshape(S, D), A_v.reshape(S, D), A_shift_k.T,
          A_ssm_k.reshape(D // 8, 8, NC, C).transpose(0, 2, 1, 3).reshape(NCB * S, C),
          A_ssm_D.reshape(NCB, CB), B_w_in.T, B_w_sp, B_b_sp.reshape(NC, C), B_w_out, c, w_mod)
        return out.reshape(1, S, D)

    return fn


pallas_adaLN_cond__ssm_conv_h3__mixer_gmlp__prompt_kernel = make()
```

```python
import math

import jax
import jax.numpy as jnp
import numpy as np
from jax import lax
from jax.experimental import pallas as pl
from jax.experimental.pallas import tpu as pltpu

S, D, FH = 2048, 640, 864
EPS = 1e-5
C = 128
NC = S // C
L = 2 * C
NL = S // L
NCB = D // C
NG = C // 8
FP = 896
TB = 4 * C
NTB = S // TB
KPAD = 32
ZPITCH = FH // 2 + 16
KH = 3
KT = (3, 2, 3, 2, 2, 3, 3)
W_PLAIN = {(0, 2): (0, 2), (2, 2): (1, 2), (3, 0): (0, 3), (3, 1): (0, 4),
           (5, 0): (1, 0), (5, 1): (1, 1), (5, 2): (1, 2)}
OUT_GROUPS = [range(0, 2), range(2, 4), range(4, 6), range(6, 7)]

F32, BF16, U32 = jnp.float32, jnp.bfloat16, jnp.uint32
NT = (((1,), (1,)), ((), ()))


def _tree_sum(xs):
    xs = list(xs)
    while len(xs) > 1:
        xs = [xs[i] + xs[i + 1] if i + 1 < len(xs) else xs[i] for i in range(0, len(xs), 2)]
    return xs[0]


def _mix(x, y, sign):
    if isinstance(x, list):
        n = min(len(x), len(y))
        return ([_mix(p, q, sign) for p, q in zip(x, y)] + x[n:]
                + [q if sign > 0 else -q for q in y[n:]])
    return x + y if sign > 0 else x - y


def _add(x, y):
    return {k: _mix(x[k], y[k], 1) for k in x}


def _sub(x, y):
    return {k: _mix(x[k], y[k], -1) for k in x}


def _quadrants(x, n):
    h = n // 2
    return [{(i, j): x[i + a * h, j + b * h] for i in range(h) for j in range(h)}
            for a in range(2) for b in range(2)]


def _lhs_operands(a, n):
    a11, a12, a21, a22 = _quadrants(a, n)
    return [_add(a21, a22), _add(a11, a12), _add(a11, a22), a22, _sub(a12, a22), a11, _sub(a21, a11)]


def _rhs_operands(b, n):
    b11, b12, b21, b22 = _quadrants(b, n)
    return [b11, b22, _add(b11, b22), _sub(b11, b21), _add(b21, b22), _sub(b12, b22), _add(b11, b12)]


def _leaves(x, n, operands):
    if n == 1:
        return [x[0, 0]]
    return [leaf for op in operands(x, n) for leaf in _leaves(op, n // 2, operands)]


def _recombine(products, n):
    if n == 1:
        return {(0, 0): products[0]}
    k, h = len(products) // 7, n // 2
    m2, m5, m1, m4, m7, m3, m6 = (_recombine(products[i * k:(i + 1) * k], h) for i in range(7))
    quads = [_add(_sub(_sub(m1, m5), m4), m7), _add(m3, m5),
             _sub(m2, m4), _add(_add(_sub(m1, m2), m3), m6)]
    return {(i + q // 2 * h, j + q % 2 * h): v for q, c in enumerate(quads) for (i, j), v in c.items()}


def _assemble(blocks, n):
    return jnp.concatenate([jnp.concatenate([blocks[i, j] for j in range(n)], axis=1)
                            for i in range(n)], axis=0)


KO = [min(len(x), len(y)) for x, y in zip(
    _leaves({(i, p): list(OUT_GROUPS[p]) for i in range(4) for p in range(4)}, 4, _lhs_operands),
    _leaves({(p, i): list(OUT_GROUPS[p]) for i in range(4) for p in range(4)}, 4, _rhs_operands))]


def _low(w):
    return pltpu.bitcast(w << 16, F32)


def _high(w):
    return pltpu.bitcast(w & np.uint32(0xFFFF0000), F32)


def _pack(low, high):
    bits = pltpu.bitcast(jnp.concatenate([low, high], axis=1).astype(BF16).astype(F32), U32)
    return (bits[:, :C] >> 16) | bits[:, C:]


def _gelu2(x):
    c = math.sqrt(2.0 / math.pi)
    return x * jnp.tanh((x * x * (c * 0.044715) + c) * x) + x


def _standardize(x):
    xc = x - jnp.sum(x, axis=-1, keepdims=True) * (1.0 / D)
    return xc * lax.rsqrt(jnp.sum(xc * xc, axis=-1, keepdims=True) * (1.0 / D) + EPS)


def _butterfly(a, b):
    return (a[0] + b[0], a[1] + b[1]), (a[0] - b[0], a[1] - b[1])


SEM_FIRST = 5
SEM_CONV = SEM_FIRST + 2
SEM_WEIGHT = SEM_CONV + 4 * NCB
SEM_Q = SEM_WEIGHT + 4
SEM_WSP = SEM_Q + NL
N_SEM = SEM_WSP + NTB


def _kernel(q_hbm, k_hbm, v_hbm, shift_hbm, ssmk_hbm, ssmd_hbm, win_hbm, wsp_hbm, bsp_hbm,
            wout_hbm, c_hbm, wmod_hbm, out_hbm,
            q_s, k_s, v_s, ssmk_s, win_s, wsp_s, wout_s, wmod_s, wgate_s, dft_s,
            skip_s, kvt_s, yt_s, y_s, woutt_s, wsum_s, x_s, qn_s, h_s, gate_s, z1_s, z2_s, m_s, o_s,
            stat_s, mod_s, acc_s, taps_s, bias_s, sc_s, shift_s, ssmd_s, bsp_s, c_s,
            sem_in, sem_out, spare_s):
    def copy(src, dst, i):
        return pltpu.make_async_copy(src, dst, sem_in.at[i])

    small = [copy(a, b, i) for i, (a, b) in enumerate(
        [(shift_hbm, shift_s), (ssmd_hbm, ssmd_s), (c_hbm, c_s), (bsp_hbm, bsp_s)])]

    def kv_first(i):
        rows = pl.ds(i * S // 2, S // 2)
        return [copy(k_hbm.at[rows, pl.ds(0, C)],
                     k_s.bitcast(BF16).at[0, pl.ds(2 * KPAD + i * S // 2, S // 2), :], SEM_FIRST + i),
                copy(v_hbm.at[rows, pl.ds(0, C)], v_s.bitcast(BF16).at[0, rows, :], SEM_FIRST + i)]

    def kv_copies(b):
        ch = pl.ds(pl.multiple_of(b * C, C), C)
        return [copy(k_hbm.at[:, ch], k_s.bitcast(BF16).at[b, pl.ds(2 * KPAD, S), :], SEM_CONV + 4 * b),
                copy(v_hbm.at[:, ch], v_s.bitcast(BF16).at[b], SEM_CONV + 4 * b + 1)]

    def ssmk_copy(b):
        rows = pl.ds(pl.multiple_of(b * S, S), S)
        return copy(ssmk_hbm.at[rows, :], ssmk_s.bitcast(BF16).at[rows, :], SEM_CONV + 4 * b + 2)

    def wmod_copy(b):
        return copy(wmod_hbm.at[pl.ds(b * C, C), pl.ds(0, 5 * D)], wmod_s.at[b], SEM_CONV + 4 * b + 3)

    def win_copies(half):
        return [copy(win_hbm.at[pl.ds(half * FH, FH), pl.ds(b * C, C)],
                     win_s.bitcast(BF16).at[half, b], SEM_WEIGHT + half) for b in range(NCB)]

    wout_copy = copy(wout_hbm, wout_s.at[pl.ds(0, FH), :], SEM_WEIGHT + 2)
    wgate_copy = copy(wmod_hbm.at[:, pl.ds(5 * D, D)], wgate_s, SEM_WEIGHT + 3)

    def q_copy(t):
        rows = pl.ds(pl.multiple_of(t * L, L), L)
        return copy(q_hbm.at[rows, :], q_s.at[rows, :], SEM_Q + t)

    def wsp_copy(u):
        rows = pl.ds(pl.multiple_of(u * TB, TB), TB)
        return copy(wsp_hbm.at[rows, :], wsp_s.at[rows, :], SEM_WSP + u)

    def out_copy(t, n):
        rows = pl.ds(pl.multiple_of(t * C, C), n)
        return pltpu.make_async_copy(o_s.at[rows, :], out_hbm.at[rows, :], sem_out.at[t])

    def wait(copies):
        for cp in copies:
            cp.wait()

    queue = small[:1] + kv_first(0) + kv_first(1) + small[1:]
    for b in range(NCB):
        queue += [ssmk_copy(b)] + (kv_copies(b + 1) if b + 1 < NCB else [])
    queue += [q_copy(0)] + [wmod_copy(b) for b in range(NCB)]
    queue += win_copies(1) + [q_copy(1)] + win_copies(0) + [q_copy(t) for t in range(2, NL)]
    queue += [wout_copy, wgate_copy] + [wsp_copy(u) for u in range(NTB)]
    for cp in queue:
        cp.start()

    def make_dft():
        def unit(turn):
            angle = (((turn + 2 * L) & (4 * L - 1)) - 2 * L).astype(F32) * (math.pi / (2 * L))
            return jnp.cos(angle), -jnp.sin(angle)

        sub, lane = (lax.broadcasted_iota(jnp.int32, (8, C), a) for a in range(2))
        blk, col = (lax.broadcasted_iota(jnp.int32, (C // 8, C), a) for a in range(2))
        forward_step = unit(8 * blk * (4 * col + 1))
        for p in range(2):
            sample = ((sub & 1) ^ p) * C + (sub & -2) + p
            for i, (first, step, scale) in enumerate([
                    (unit(sample * (4 * lane + 1)), forward_step, 1.0),
                    (unit((2 * lane + p) * (4 * sub + 1)), unit((2 * col + p) * 32 * blk), 1.0 / L)]):
                ar, ai = (jnp.concatenate([v * scale] * (C // 8), axis=0) for v in first)
                br, bi = (jnp.concatenate([jnp.broadcast_to(v[j:j + 1], (8, C)) for j in range(C // 8)],
                                          axis=0) for v in step)
                for c, w in enumerate([ar * br - ai * bi, ar * bi + ai * br]):
                    j = 4 * i + 2 * p + c
                    dft_s[j * C // 2:(j + 1) * C // 2, :] = pltpu.bitcast(w.astype(BF16), U32)

    def dft(i, n):
        return pltpu.bitcast(dft_s[i * C // 2:(i + n) * C // 2, :], BF16)

    def gate_chunk(b, m):
        kw = [k_s[b, pl.ds(KPAD + m * C + j, C), :] for j in range(-2, 1)]
        vw = v_s[b, m * C:(m + 1) * C, :]
        kk = [_high(kw[0]), _low(kw[1]), _high(kw[1]), _low(kw[2]), _high(kw[2])]
        for p, vv in enumerate((_low(vw), _high(vw))):
            kv = _tree_sum([kk[3 + p - t] * taps_s[b, t:t + 1, :] for t in range(4)]) * vv
            halves = [kv[:C // 2], kv[C // 2:]]
            tile = pltpu.bitcast(_pack(halves[p], halves[1 - p]), BF16)
            kvt_s[(2 * m + p) * 64:(2 * m + p + 1) * 64, :] = pltpu.bitcast(tile.T, U32)

    def forward(b, g):
        base = pl.multiple_of(b * (S // 2), S // 2) + g * NC * 4
        top = lax.broadcasted_iota(jnp.int32, (8, C), 0) < 4
        words = [ssmk_s[pl.ds(base + 4 * i, 8), :] if i % 4 < 3 else None for i in range(NC)]
        t0, t1 = [jnp.concatenate([jnp.where(top, words[i + j], words[i + j + 1])
                                   for i in range(0, NC, 4)], axis=0) for j in range(2)]
        odd = (lax.broadcasted_iota(jnp.int32, t0.shape, 1) & 1) == 1
        filt = [jnp.where(odd, pltpu.roll(t1, 1, 1), t0), jnp.where(odd, t0, pltpu.roll(t1, C - 1, 1))]
        out = []
        for p in range(2):
            sig = jnp.concatenate([jnp.where(top, kvt_s[pl.ds((2 * m + p) * 64 + 4 * g, 8), :],
                                             kvt_s[pl.ds((2 * m + 2 + p) * 64 + 4 * g - 4, 8), :])
                                   for m in range(0, NL, 2)], axis=0)
            lhs = jnp.concatenate([t[i:i + 8] for i in range(0, 4 * NL, 8) for t in (filt[p], sig)], axis=0)
            out.append([jnp.dot(pltpu.bitcast(lhs, BF16), dft(2 * p + c, 1), preferred_element_type=F32)
                        for c in range(2)])
        return out

    def product(b, g, f):
        def part(i, m, p):
            r = (m // 2 * 4 + i * 2 + m % 2) * 8
            return f[p][0][r:r + 8], f[p][1][r:r + 8]

        def window(m, p):
            re, im = part(0, m, p)
            if m:
                pre, pim = part(0, m - 1, p)
                return re - pim, im + pre
            if p == 0:
                re = re + skip_s[pl.ds(pl.multiple_of(b * C + g * 8, 8), 8), :]
            return re, im

        kf = [_butterfly(window(m, 0), window(m, 1)) for m in range(NL)]
        xf = [_butterfly(part(1, m, 0), part(1, m, 1)) for m in range(NL)]
        out = []
        for i in range(NL):
            z = []
            for h in range(2):
                terms = [(xf[j][h], kf[i - j][h]) for j in range(i + 1)]
                if i:
                    p1 = _tree_sum([x[0] * k[0] for x, k in terms])
                    p2 = _tree_sum([x[1] * k[1] for x, k in terms])
                    p3 = _tree_sum([(x[0] + x[1]) * (k[0] + k[1]) for x, k in terms])
                    z.append((p1 - p2, p3 - (p1 + p2)))
                else:
                    (x, k), = terms
                    z.append((x[0] * k[0] - x[1] * k[1], x[0] * k[1] + x[1] * k[0]))
            out.append(_butterfly(*z))
        return out

    def inverse(b, g, z):
        rows = pl.ds(pl.multiple_of(b * C + g * 8, 8), 8)
        for p in range(2):
            zp = jnp.concatenate([jnp.concatenate([z[i][p][c] for i in range(NL)], axis=0)
                                  for c in range(2)], axis=1)
            y = jnp.dot(zp.astype(BF16), dft(4 + 2 * p, 2), preferred_element_type=F32)
            for i in range(NL):
                yt_s[i, p, rows, :] = y[i * 8:(i + 1) * 8]

    def modulation(blocks):
        wait([wmod_copy(b) for b in blocks])
        acc_s[...] += _tree_sum([jnp.dot(sc_s[b], wmod_s[b], preferred_element_type=F32)[0:8]
                                 for b in blocks])

    def time_major(t, blocks):
        for b in blocks:
            for p in range(2):
                y_s[b, pl.ds(p, C, stride=2), :] = yt_s[t, p, b * C:(b + 1) * C, :].T

    def conv_block(b, last):
        ssmk_copy(b).wait()
        f = {0: forward(b, 0)}
        for g in range(NG):
            if g + 1 < NG:
                f[g + 1] = forward(b, g + 1)
            if g == 10 and not last:
                wait(kv_copies(b + 1))
            if g == 12 and last:
                q_copy(0).wait()
                modulation(range(NCB - 1))
                time_major(0, range(NCB - 1))
                qn_s[...] = _standardize(q_s[0:L, :].astype(F32))
            inverse(b, g, product(b, g, f.pop(g)))
        if last:
            time_major(0, [NCB - 1])
            modulation([NCB - 1])
        else:
            for m in range(NL):
                gate_chunk(b + 1, m)

    spare_s[0] = 7
    k_s[:, KPAD - 8:KPAD, :] = jnp.zeros((NCB, 8, C), U32)
    acc_s[...] = jnp.zeros(acc_s.shape, F32)
    m_s[FH:, :] = jnp.zeros((FP - FH, TB), F32)
    wout_s[FH:, :] = jnp.zeros((FP - FH, D), BF16)
    make_dft()
    small[0].wait()
    taps = shift_s[...].astype(F32)
    for b in range(NCB):
        taps_s[b, 0:4, :] = taps[:, b * C:(b + 1) * C]
    for m in range(NL):
        if m % (NL // 2) == 0:
            wait(kv_first(m // (NL // 2)))
        gate_chunk(0, m)
    wait(small[1:])
    skip = ssmd_s[...].astype(F32)
    cf = c_s[...].astype(F32)
    silu_c = jnp.broadcast_to(cf * jax.nn.sigmoid(cf), (16, D)).astype(BF16)
    for b in range(NCB):
        skip_s[b * C:(b + 1) * C, :] = jnp.broadcast_to(skip[b:b + 1], (C, C)).T
        sc_s[b] = silu_c[:, b * C:(b + 1) * C]
    bias_s[...] = bsp_s[...].astype(F32)

    pl.loop(0, NCB - 1)(lambda b: conv_block(b, False))
    conv_block(NCB - 1, True)

    sa, ca, ga, sb, cb = (acc_s[:, i * D:(i + 1) * D] for i in range(5))
    mod_s[0] = ga * (1.0 + ca)
    mod_s[1] = ga * sa
    mod_s[2] = 1.0 + cb
    mod_s[3] = sb

    def mod(i, n):
        return jnp.concatenate([mod_s[i]] * (n // 8), axis=0)

    def residual(t, qn=None):
        rows = pl.ds(pl.multiple_of(t * L, L), L)
        q = q_s[rows, :].astype(F32)
        y = jnp.concatenate([y_s[b] for b in range(NCB)], axis=1)
        x = q + ((_standardize(q) if qn is None else qn) * mod(0, L) + mod(1, L)) * y
        x_s[rows, :] = x
        return _standardize(x) * mod(2, L) + mod(3, L)

    def split(tiles):
        return tiles[:KH], tiles[KH:]

    def prepare(t):
        time_major(t, range(NCB))
        h = residual(t)
        blocks = {(i, j): split([h[j * C:(j + 1) * C, b * C:(b + 1) * C] for b in range(NCB)])[i]
                  for i in range(2) for j in range(2)}
        for i, tiles in enumerate(_leaves(blocks, 2, _rhs_operands)):
            h_s[i, :, :KT[i] * C] = jnp.concatenate(tiles[:KT[i]], axis=1).astype(BF16)

    def prepare_w_in(z):
        for r in range(0, FH // 2, 8):
            wsum_s[spare_s[0], 0, 0:8, :] = pltpu.bitcast(z[2 * r:2 * r + 8, :C], U32)
            words = [[win_s[1 - i, b, r:r + 8, :] for b in range(NCB)] for i in range(2)]
            low, high = [_leaves({(i, j): split([f(w) for w in words[i]])[j]
                                  for i in range(2) for j in range(2)}, 2, _lhs_operands)
                         for f in (_low, _high)]
            for i in range(7):
                for b in range(KT[i]):
                    if (i, b) not in W_PLAIN:
                        wsum_s[i, b, r:r + 8, :] = _pack(low[i][b], high[i][b])

    def project_plain(half, h):
        wait(win_copies(half))
        return jnp.concatenate([lax.dot_general(
            jnp.concatenate([pltpu.bitcast(win_s[half, b, r:r + FH // 4, :], BF16) for b in range(NCB)],
                            axis=1), h, NT, preferred_element_type=F32) for r in (0, FH // 4)], axis=0)

    def gate_branch(z):
        z = _gelu2(z)
        z = z - z[0:1]
        gate_s[...] = z
        stat_s[0] = jnp.sum(z.reshape(FH // 8, 8, L), axis=0)
        stat_s[1] = jnp.sum((z * z).reshape(FH // 8, 8, L), axis=0)

    def normalize(t):
        mean = jnp.sum(stat_s[0], axis=0, keepdims=True) * (1.0 / FH)
        var = jnp.sum(stat_s[1], axis=0, keepdims=True) * (1.0 / FH) - mean * mean
        scale = lax.rsqrt(jnp.maximum(var, 0.0) + 4.0 * EPS)
        zn = (gate_s[...] - mean) * scale
        blocks = {(i, j): zn[i * FH // 2:(i + 1) * FH // 2, j * C:(j + 1) * C]
                  for i in range(2) for j in range(2)}
        rows = pl.ds(pl.multiple_of(t % (NL // 2) * ZPITCH, 8), FH // 2)
        for i, a in enumerate(_leaves(blocks, 2, _lhs_operands)):
            z2_s[i, t // (NL // 2), rows, :] = a

    def project(t):
        products = []
        for i in range(7):
            w = [win_s[W_PLAIN[i, b]] if (i, b) in W_PLAIN else wsum_s[i, b] for b in range(KT[i])]
            w = jnp.concatenate([pltpu.bitcast(x, BF16) for x in w], axis=1)
            products.append(lax.dot_general(w, h_s[i, :, :KT[i] * C], NT, preferred_element_type=F32))
        z = _assemble(_recombine(products, 2), 2)
        normalize(t - 1)
        gate_branch(z[:FH])
        z1_s[t] = z[FH:].astype(BF16)

    h0 = residual(0, qn_s[...]).astype(BF16)
    q_copy(1).wait()
    gate_branch(project_plain(1, h0))
    prepare(1)
    z1 = project_plain(0, h0)
    z1_s[0] = z1.astype(BF16)
    prepare_w_in(z1)

    @pl.loop(1, NL - 1)
    def _(t):
        q_copy(t + 1).wait()
        project(t)
        prepare(t + 1)

    wait([wout_copy, wgate_copy, wsp_copy(0)])
    project(NL - 1)
    normalize(NL - 1)
    silu_c = jnp.concatenate([sc_s[b] for b in range(NCB)], axis=1)
    mod_s[4] = 0.5 * jnp.dot(silu_c, wgate_s[...], preferred_element_type=F32)[0:8]

    def mix(u):
        hf = FH // 4

        def w_block(si, ti):
            rows = pl.ds(pl.multiple_of(u * TB + ti * C, C), C)
            cols = [(si % 2 * NL // 2 + t) * L + si // 2 * C for t in range(NL // 2)]
            return jnp.concatenate([wsp_s[rows, c:c + C] for c in cols], axis=1).astype(F32)

        def z_operand(i):
            return {(p, q): jnp.concatenate([z2_s[i, q, t * ZPITCH + p * hf:t * ZPITCH + (p + 1) * hf, :]
                                             for t in range(NL // 2)], axis=1)
                    for p in range(2) for q in range(2)}

        products = []
        for i, w in enumerate(_rhs_operands({(si, ti): w_block(si, ti)
                                             for si in range(4) for ti in range(4)}, 4)):
            products += [lax.dot_general(a, b, NT, preferred_element_type=F32) for a, b in zip(
                _leaves(z_operand(i), 2, _lhs_operands), _leaves(w, 2, _rhs_operands))]
        g = _assemble(_recombine(products, 4), 4)
        bias = jnp.concatenate([bias_s[pl.ds(u * (TB // C) + i, 1), :] for i in range(TB // C)], axis=1)
        z1 = jnp.concatenate([z1_s[u * (TB // L) + i] for i in range(TB // L)], axis=1).astype(F32)
        m_s[:FH, :] = _gelu2(z1) * (g + bias)

    def prepare_w_out():
        tiles = [wout_s[j * C:(j + 1) * C, :].T.astype(F32) for j in range(FP // C)]
        blocks = {(i, p): [tiles[f][i * D // 4:(i + 1) * D // 4] for f in OUT_GROUPS[p]]
                  for i in range(4) for p in range(4)}
        for i, leaf in enumerate(_leaves(blocks, 4, _lhs_operands)):
            woutt_s[i, :, :KO[i] * C] = jnp.concatenate(leaf[:KO[i]], axis=1).astype(BF16)

    def project_out(u, send):
        blocks = {(p, i): [m_s[f * C:(f + 1) * C, i * C:(i + 1) * C] for f in OUT_GROUPS[p]]
                  for i in range(4) for p in range(4)}
        o = _assemble(_recombine(
            [jnp.dot(woutt_s[i, :, :KO[i] * C], jnp.concatenate(leaf[:KO[i]], axis=0).astype(BF16),
                     preferred_element_type=F32)
             for i, leaf in enumerate(_leaves(blocks, 4, _rhs_operands))], 4), 4)
        for i in range(TB // C):
            t = u * (TB // C) + i
            rows = pl.ds(pl.multiple_of(t * C, C), C)
            o_s[rows, :] = (x_s[rows, :] + mod(4, C) * o[:, i * C:(i + 1) * C].T).astype(BF16)
            if send:
                out_copy(t, C).start()

    mix(0)
    prepare_w_out()

    @pl.loop(1, NTB)
    def _(u):
        wsp_copy(u).wait()
        project_out(u - 1, False)
        mix(u)
        out_copy((u - 1) * (TB // C), TB).start()

    project_out(NTB - 1, True)
    wait([out_copy(u * (TB // C), TB) for u in range(NTB - 1)])
    wait([out_copy(t, C) for t in range(NC - TB // C, NC)])


@jax.jit
def pallas_adaLN_cond__ssm_conv_h3__mixer_gmlp__prompt_kernel(
    A_q: jax.Array,
    A_k: jax.Array,
    A_v: jax.Array,
    A_shift_k: jax.Array,
    A_ssm_k: jax.Array,
    A_ssm_D: jax.Array,
    B_x: jax.Array,
    B_w_in: jax.Array,
    B_w_sp: jax.Array,
    B_b_sp: jax.Array,
    B_w_out: jax.Array,
    c: jax.Array,
    w_mod: jax.Array,
):
    del B_x
    vm = pltpu.VMEM
    scratch = [
        vm((S, D), BF16), vm((NCB, KPAD + S // 2, C), U32), vm((NCB, S // 2, C), U32),
        vm((NCB * S // 2, C), U32), vm((2, NCB, FH // 2, C), U32), vm((S, S), BF16),
        vm((FP, D), BF16), vm((NCB, C, 5 * D), BF16), vm((D, D), BF16), vm((4 * C, C), U32),
        vm((D, C), F32), vm((NC * C // 2, C), U32), vm((NL, 2, D, C), F32), vm((NCB, L, C), F32),
        vm((len(KO) + 1, D // 4, max(KO) * C), BF16), vm((8, KH, FH // 2, C), U32), vm((S, D), F32),
        vm((L, D), F32), vm((7, C, KH * C), BF16), vm((FH, L), F32), vm((NL, FH, L), BF16),
        vm((7, 2, NL // 2 * ZPITCH, C), F32), vm((FP, TB), F32), vm((S, D), BF16),
        vm((2, 8, L), F32), vm((8, 8, D), F32), vm((8, 5 * D), F32), vm((NCB, 8, C), F32),
        vm((NC, C), F32), vm((NCB, 16, C), BF16), vm((4, D), BF16), vm((NCB, C), BF16),
        vm((NC, C), BF16), vm((1, D), BF16),
        pltpu.SemaphoreType.DMA((N_SEM,)), pltpu.SemaphoreType.DMA((NC,)), pltpu.SMEM((1,), jnp.int32),
    ]
    out = pl.pallas_call(
        _kernel,
        out_shape=jax.ShapeDtypeStruct((S, D), BF16),
        in_specs=[pl.BlockSpec(memory_space=pltpu.HBM)] * 12,
        out_specs=pl.BlockSpec(memory_space=pltpu.HBM),
        scratch_shapes=scratch,
        compiler_params=pltpu.CompilerParams(
            vmem_limit_bytes=120 * 2**20,
            flags={"XLA_TPU_EVENLY_DISTRIBUTE_CRITICAL_NODES": True}),
    )(A_q.reshape(S, D), A_k.reshape(S, D), A_v.reshape(S, D), A_shift_k.T,
      A_ssm_k.reshape(D // 8, 8, NC, C).transpose(0, 2, 1, 3).reshape(NCB * S, C),
      A_ssm_D.reshape(NCB, C), B_w_in.T, B_w_sp, B_b_sp.reshape(NC, C), B_w_out, c, w_mod)
    return out.reshape(1, S, D)
```

```python
import math

import jax
import jax.numpy as jnp
import numpy as np
from jax import lax
from jax.experimental import pallas as pl
from jax.experimental.pallas import tpu as pltpu

S, D, FH = 2048, 640, 864
EPS = 1e-5
C = 128
NC = S // C
L = 2 * C
NL = S // L
NCB = D // C
NG = C // 8
FP = 896
TB = 4 * C
NTB = S // TB
KPAD = 32
ZPITCH = FH // 2 + 16
KH = 3
KT = (3, 2, 3, 2, 2, 3, 3)
W_PLAIN = {(0, 2): (0, 2), (2, 2): (1, 2), (3, 0): (0, 3), (3, 1): (0, 4),
           (5, 0): (1, 0), (5, 1): (1, 1), (5, 2): (1, 2)}
OUT_GROUPS = [range(0, 2), range(2, 4), range(4, 6), range(6, 7)]

F32, BF16, U32 = jnp.float32, jnp.bfloat16, jnp.uint32
NT = (((1,), (1,)), ((), ()))


def _tree_sum(xs):
    xs = list(xs)
    while len(xs) > 1:
        xs = [xs[i] + xs[i + 1] if i + 1 < len(xs) else xs[i] for i in range(0, len(xs), 2)]
    return xs[0]


def _mix(x, y, sign):
    if isinstance(x, list):
        n = min(len(x), len(y))
        return ([_mix(p, q, sign) for p, q in zip(x, y)] + x[n:]
                + [q if sign > 0 else -q for q in y[n:]])
    return x + y if sign > 0 else x - y


def _add(x, y):
    return {k: _mix(x[k], y[k], 1) for k in x}


def _sub(x, y):
    return {k: _mix(x[k], y[k], -1) for k in x}


def _quadrants(x, n):
    h = n // 2
    return [{(i, j): x[i + a * h, j + b * h] for i in range(h) for j in range(h)}
            for a in range(2) for b in range(2)]


def _lhs_operands(a, n):
    a11, a12, a21, a22 = _quadrants(a, n)
    return [_add(a21, a22), _add(a11, a12), _add(a11, a22), a22, _sub(a12, a22), a11, _sub(a21, a11)]


def _rhs_operands(b, n):
    b11, b12, b21, b22 = _quadrants(b, n)
    return [b11, b22, _add(b11, b22), _sub(b11, b21), _add(b21, b22), _sub(b12, b22), _add(b11, b12)]


def _leaves(x, n, operands):
    if n == 1:
        return [x[0, 0]]
    return [leaf for op in operands(x, n) for leaf in _leaves(op, n // 2, operands)]


def _recombine(products, n):
    if n == 1:
        return {(0, 0): products[0]}
    k, h = len(products) // 7, n // 2
    m2, m5, m1, m4, m7, m3, m6 = (_recombine(products[i * k:(i + 1) * k], h) for i in range(7))
    quads = [_add(_sub(_sub(m1, m5), m4), m7), _add(m3, m5),
             _sub(m2, m4), _add(_add(_sub(m1, m2), m3), m6)]
    return {(i + q // 2 * h, j + q % 2 * h): v for q, c in enumerate(quads) for (i, j), v in c.items()}


def _assemble(blocks, n):
    return jnp.concatenate([jnp.concatenate([blocks[i, j] for j in range(n)], axis=1)
                            for i in range(n)], axis=0)


KO = [min(len(x), len(y)) for x, y in zip(
    _leaves({(i, p): list(OUT_GROUPS[p]) for i in range(4) for p in range(4)}, 4, _lhs_operands),
    _leaves({(p, i): list(OUT_GROUPS[p]) for i in range(4) for p in range(4)}, 4, _rhs_operands))]


def _low(w):
    return pltpu.bitcast(w << 16, F32)


def _high(w):
    return pltpu.bitcast(w & np.uint32(0xFFFF0000), F32)


def _pack(low, high):
    bits = pltpu.bitcast(jnp.concatenate([low, high], axis=1).astype(BF16).astype(F32), U32)
    return (bits[:, :C] >> 16) | bits[:, C:]


def _gelu2(x):
    c = math.sqrt(2.0 / math.pi)
    return x * jnp.tanh((x * x * (c * 0.044715) + c) * x) + x


def _standardize(x):
    xc = x - jnp.sum(x, axis=-1, keepdims=True) * (1.0 / D)
    return xc * lax.rsqrt(jnp.sum(xc * xc, axis=-1, keepdims=True) * (1.0 / D) + EPS)


def _butterfly(a, b):
    return (a[0] + b[0], a[1] + b[1]), (a[0] - b[0], a[1] - b[1])


SEM_FIRST = 0
SEM_KV = SEM_FIRST + 1
SEM_SSMK = SEM_KV + NCB
SEM_MOD = SEM_SSMK + NCB
SEM_WIN = SEM_MOD + 2
SEM_Q = SEM_WIN + 2
SEM_LATE = SEM_Q + 2
SEM_OUT = SEM_LATE + 1
N_SEM = SEM_OUT + 1


def _kernel(q_hbm, k_hbm, v_hbm, shift_hbm, ssmk_hbm, ssmd_hbm, win_hbm, wsp_hbm, bsp_hbm,
            wout_hbm, c_hbm, wmod_hbm, out_hbm,
            q_s, k_s, v_s, ssmk_s, win_s, wsp_s, wout_s, wmod_s, wgate_s, dft_s,
            skip_s, kvt_s, yt_s, y_s, woutt_s, wsum_s, x_s, qn_s, h_s, gate_s, z1_s, z2_s, m_s, o_s,
            stat_s, mod_s, acc_s, taps_s, bias_s, sc_s, shift_s, ssmd_s, bsp_s, c_s,
            sems, spare_s):
    def copy(src, dst, i):
        return pltpu.make_async_copy(src, dst, sems.at[i])

    small = [copy(a, b, SEM_FIRST) for a, b in
             [(shift_hbm, shift_s), (ssmd_hbm, ssmd_s), (c_hbm, c_s), (bsp_hbm, bsp_s)]]

    def kv_first(i):
        rows = pl.ds(i * S // 2, S // 2)
        return [copy(k_hbm.at[rows, pl.ds(0, C)],
                     k_s.bitcast(BF16).at[0, pl.ds(2 * KPAD + i * S // 2, S // 2), :], SEM_FIRST + i),
                copy(v_hbm.at[rows, pl.ds(0, C)], v_s.bitcast(BF16).at[0, rows, :], SEM_FIRST + i)]

    def kv_copies(b):
        ch = pl.ds(pl.multiple_of(b * C, C), C)
        return [copy(k_hbm.at[:, ch], k_s.bitcast(BF16).at[b, pl.ds(2 * KPAD, S), :], SEM_KV + b),
                copy(v_hbm.at[:, ch], v_s.bitcast(BF16).at[b], SEM_KV + b)]

    def ssmk_copy(b):
        rows = pl.ds(pl.multiple_of(b * S, S), S)
        return copy(ssmk_hbm.at[rows, :], ssmk_s.bitcast(BF16).at[rows, :], SEM_SSMK + b)

    def wmod_copy(b):
        return copy(wmod_hbm.at[pl.ds(b * C, C), pl.ds(0, 5 * D)], wmod_s.at[b],
                    SEM_MOD + b // (NCB - 1))

    def win_copies(half):
        return [copy(win_hbm.at[pl.ds(half * FH, FH), pl.ds(b * C, C)],
                     win_s.bitcast(BF16).at[half, b], SEM_WIN + half) for b in range(NCB)]

    wout_copy = copy(wout_hbm, wout_s.at[pl.ds(0, FH), :], SEM_LATE)
    wgate_copy = copy(wmod_hbm.at[:, pl.ds(5 * D, D)], wgate_s, SEM_LATE)

    wsp_copy = copy(wsp_hbm, wsp_s, SEM_LATE)

    def q_copy(t, n, sem):
        rows = pl.ds(t * L, n * L)
        return copy(q_hbm.at[rows, :], q_s.at[rows, :], sem)

    q_copies = [q_copy(0, 1, SEM_MOD), q_copy(1, 1, SEM_WIN + 1),
                q_copy(2, 1, SEM_Q), q_copy(3, NL - 3, SEM_Q + 1)]

    def out_copy(t, n):
        rows = pl.ds(pl.multiple_of(t * C, C), n)
        return pltpu.make_async_copy(o_s.at[rows, :], out_hbm.at[rows, :], sems.at[SEM_OUT])

    def wait(copies):
        for cp in copies:
            cp.wait()

    queue = small + kv_first(0) + kv_first(1)
    for b in range(NCB):
        queue += [ssmk_copy(b)] + (kv_copies(b + 1) if b + 1 < NCB else [])
    queue += q_copies[:1] + [wmod_copy(b) for b in range(NCB)]
    queue += win_copies(1) + q_copies[1:2] + win_copies(0) + q_copies[2:]
    queue += [wout_copy, wgate_copy, wsp_copy]
    for cp in queue:
        cp.start()

    def make_dft():
        def unit(turn):
            angle = (((turn + 2 * L) & (4 * L - 1)) - 2 * L).astype(F32) * (math.pi / (2 * L))
            return jnp.cos(angle), -jnp.sin(angle)

        sub, lane = (lax.broadcasted_iota(jnp.int32, (8, C), a) for a in range(2))
        blk, col = (lax.broadcasted_iota(jnp.int32, (C // 8, C), a) for a in range(2))
        forward_step = unit(8 * blk * (4 * col + 1))
        for p in range(2):
            sample = ((sub & 1) ^ p) * C + (sub & -2) + p
            for i, (first, step, scale) in enumerate([
                    (unit(sample * (4 * lane + 1)), forward_step, 1.0),
                    (unit((2 * lane + p) * (4 * sub + 1)), unit((2 * col + p) * 32 * blk), 1.0 / L)]):
                ar, ai = (jnp.concatenate([v * scale] * (C // 8), axis=0) for v in first)
                br, bi = (jnp.concatenate([jnp.broadcast_to(v[j:j + 1], (8, C)) for j in range(C // 8)],
                                          axis=0) for v in step)
                for c, w in enumerate([ar * br - ai * bi, ar * bi + ai * br]):
                    j = 4 * i + 2 * p + c
                    dft_s[j * C // 2:(j + 1) * C // 2, :] = pltpu.bitcast(w.astype(BF16), U32)

    def dft(i, n):
        return pltpu.bitcast(dft_s[i * C // 2:(i + n) * C // 2, :], BF16)

    def gate_chunk(b, m):
        kw = [k_s[b, pl.ds(KPAD + m * C + j, C), :] for j in range(-2, 1)]
        vw = v_s[b, m * C:(m + 1) * C, :]
        kk = [_high(kw[0]), _low(kw[1]), _high(kw[1]), _low(kw[2]), _high(kw[2])]
        for p, vv in enumerate((_low(vw), _high(vw))):
            kv = _tree_sum([kk[3 + p - t] * taps_s[b, t:t + 1, :] for t in range(4)]) * vv
            halves = [kv[:C // 2], kv[C // 2:]]
            tile = pltpu.bitcast(_pack(halves[p], halves[1 - p]), BF16)
            kvt_s[(2 * m + p) * 64:(2 * m + p + 1) * 64, :] = pltpu.bitcast(tile.T, U32)

    def forward(b, g):
        base = pl.multiple_of(b * (S // 2), S // 2) + g * NC * 4
        top = lax.broadcasted_iota(jnp.int32, (8, C), 0) < 4
        words = [ssmk_s[pl.ds(base + 4 * i, 8), :] if i % 4 < 3 else None for i in range(NC)]
        t0, t1 = [jnp.concatenate([jnp.where(top, words[i + j], words[i + j + 1])
                                   for i in range(0, NC, 4)], axis=0) for j in range(2)]
        odd = (lax.broadcasted_iota(jnp.int32, t0.shape, 1) & 1) == 1
        filt = [jnp.where(odd, pltpu.roll(t1, 1, 1), t0), jnp.where(odd, t0, pltpu.roll(t1, C - 1, 1))]
        out = []
        for p in range(2):
            sig = jnp.concatenate([jnp.where(top, kvt_s[pl.ds((2 * m + p) * 64 + 4 * g, 8), :],
                                             kvt_s[pl.ds((2 * m + 2 + p) * 64 + 4 * g - 4, 8), :])
                                   for m in range(0, NL, 2)], axis=0)
            lhs = jnp.concatenate([t[i:i + 8] for i in range(0, 4 * NL, 8) for t in (filt[p], sig)], axis=0)
            r = jnp.dot(pltpu.bitcast(lhs, BF16), jnp.concatenate([dft(2 * p, 1), dft(2 * p + 1, 1)], axis=1),
                        preferred_element_type=F32)
            out.append([r[:, :C], r[:, C:]])
        return out

    def product(b, g, f):
        def part(i, m, p):
            r = (m // 2 * 4 + i * 2 + m % 2) * 8
            return f[p][0][r:r + 8], f[p][1][r:r + 8]

        def window(m, p):
            re, im = part(0, m, p)
            if m:
                pre, pim = part(0, m - 1, p)
                return re - pim, im + pre
            if p == 0:
                re = re + skip_s[pl.ds(pl.multiple_of(b * C + g * 8, 8), 8), :]
            return re, im

        kf = [_butterfly(window(m, 0), window(m, 1)) for m in range(NL)]
        xf = [_butterfly(part(1, m, 0), part(1, m, 1)) for m in range(NL)]
        out = []
        for i in range(NL):
            z = []
            for h in range(2):
                terms = [(xf[j][h], kf[i - j][h]) for j in range(i + 1)]
                if i:
                    p1 = _tree_sum([x[0] * k[0] for x, k in terms])
                    p2 = _tree_sum([x[1] * k[1] for x, k in terms])
                    p3 = _tree_sum([(x[0] + x[1]) * (k[0] + k[1]) for x, k in terms])
                    z.append((p1 - p2, p3 - (p1 + p2)))
                else:
                    (x, k), = terms
                    z.append((x[0] * k[0] - x[1] * k[1], x[0] * k[1] + x[1] * k[0]))
            out.append(_butterfly(*z))
        return out

    def inverse(b, g, z):
        rows = pl.ds(pl.multiple_of(b * C + g * 8, 8), 8)
        for p in range(2):
            zp = jnp.concatenate([jnp.concatenate([z[i][p][c] for i in range(NL)], axis=0)
                                  for c in range(2)], axis=1)
            y = jnp.dot(zp.astype(BF16), dft(4 + 2 * p, 2), preferred_element_type=F32)
            for i in range(NL):
                yt_s[i, p, rows, :] = y[i * 8:(i + 1) * 8]

    def modulation(blocks):
        wait([wmod_copy(b) for b in blocks])
        acc_s[...] += _tree_sum([jnp.dot(sc_s[b], wmod_s[b], preferred_element_type=F32)[0:8]
                                 for b in blocks])

    def time_major(t, blocks):
        for b in blocks:
            for p in range(2):
                y_s[b, pl.ds(p, C, stride=2), :] = yt_s[t, p, b * C:(b + 1) * C, :].T

    def conv_block(b, last):
        ssmk_copy(b).wait()
        f = {0: forward(b, 0)}
        for g in range(NG):
            if g + 1 < NG:
                f[g + 1] = forward(b, g + 1)
            if g == 10 and not last:
                wait(kv_copies(b + 1))
            if g == 12 and last:
                q_copies[0].wait()
                modulation(range(NCB - 1))
                time_major(0, range(NCB - 1))
                qn_s[...] = _standardize(q_s[0:L, :].astype(F32))
            inverse(b, g, product(b, g, f.pop(g)))
        if last:
            time_major(0, [NCB - 1])
            modulation([NCB - 1])
        else:
            for m in range(NL):
                gate_chunk(b + 1, m)

    spare_s[0] = 7
    k_s[:, KPAD - 8:KPAD, :] = jnp.zeros((NCB, 8, C), U32)
    acc_s[...] = jnp.zeros(acc_s.shape, F32)
    m_s[FH:, :] = jnp.zeros((FP - FH, TB), F32)
    wout_s[FH:, :] = jnp.zeros((FP - FH, D), BF16)
    make_dft()
    wait(small + kv_first(0))
    taps = shift_s[...].astype(F32)
    for b in range(NCB):
        taps_s[b, 0:4, :] = taps[:, b * C:(b + 1) * C]
    skip = ssmd_s[...].astype(F32)
    cf = c_s[...].astype(F32)
    silu_c = jnp.broadcast_to(cf * jax.nn.sigmoid(cf), (16, D)).astype(BF16)
    for b in range(NCB):
        skip_s[b * C:(b + 1) * C, :] = jnp.broadcast_to(skip[b:b + 1], (C, C)).T
        sc_s[b] = silu_c[:, b * C:(b + 1) * C]
    bias_s[...] = bsp_s[...].astype(F32)
    for m in range(NL):
        if m == NL // 2:
            wait(kv_first(1))
        gate_chunk(0, m)

    pl.loop(0, NCB - 1)(lambda b: conv_block(b, False))
    conv_block(NCB - 1, True)

    sa, ca, ga, sb, cb = (acc_s[:, i * D:(i + 1) * D] for i in range(5))
    mod_s[0] = ga * (1.0 + ca)
    mod_s[1] = ga * sa
    mod_s[2] = 1.0 + cb
    mod_s[3] = sb

    def mod(i, n):
        return jnp.concatenate([mod_s[i]] * (n // 8), axis=0)

    def residual(t, qn=None):
        rows = pl.ds(pl.multiple_of(t * L, L), L)
        q = q_s[rows, :].astype(F32)
        y = jnp.concatenate([y_s[b] for b in range(NCB)], axis=1)
        x = q + ((_standardize(q) if qn is None else qn) * mod(0, L) + mod(1, L)) * y
        x_s[rows, :] = x
        return _standardize(x) * mod(2, L) + mod(3, L)

    def split(tiles):
        return tiles[:KH], tiles[KH:]

    def prepare(t):
        time_major(t, range(NCB))
        h = residual(t)
        blocks = {(i, j): split([h[j * C:(j + 1) * C, b * C:(b + 1) * C] for b in range(NCB)])[i]
                  for i in range(2) for j in range(2)}
        for i, tiles in enumerate(_leaves(blocks, 2, _rhs_operands)):
            h_s[i, :, :KT[i] * C] = jnp.concatenate(tiles[:KT[i]], axis=1).astype(BF16)

    def prepare_w_in(z):
        for r in range(0, FH // 2, 8):
            wsum_s[spare_s[0], 0, 0:8, :] = pltpu.bitcast(z[2 * r:2 * r + 8, :C], U32)
            words = [[win_s[1 - i, b, r:r + 8, :] for b in range(NCB)] for i in range(2)]
            low, high = [_leaves({(i, j): split([f(w) for w in words[i]])[j]
                                  for i in range(2) for j in range(2)}, 2, _lhs_operands)
                         for f in (_low, _high)]
            for i in range(7):
                for b in range(KT[i]):
                    if (i, b) not in W_PLAIN:
                        wsum_s[i, b, r:r + 8, :] = _pack(low[i][b], high[i][b])

    def project_plain(half, h):
        wait(win_copies(half))
        return jnp.concatenate([lax.dot_general(
            jnp.concatenate([pltpu.bitcast(win_s[half, b, r:r + FH // 4, :], BF16) for b in range(NCB)],
                            axis=1), h, NT, preferred_element_type=F32) for r in (0, FH // 4)], axis=0)

    def gate_branch(z):
        z = _gelu2(z)
        z = z - z[0:1]
        gate_s[...] = z
        stat_s[0] = jnp.sum(z.reshape(FH // 8, 8, L), axis=0)
        stat_s[1] = jnp.sum((z * z).reshape(FH // 8, 8, L), axis=0)

    def normalize(t):
        mean = jnp.sum(stat_s[0], axis=0, keepdims=True) * (1.0 / FH)
        var = jnp.sum(stat_s[1], axis=0, keepdims=True) * (1.0 / FH) - mean * mean
        scale = lax.rsqrt(jnp.maximum(var, 0.0) + 4.0 * EPS)
        zn = (gate_s[...] - mean) * scale
        blocks = {(i, j): zn[i * FH // 2:(i + 1) * FH // 2, j * C:(j + 1) * C]
                  for i in range(2) for j in range(2)}
        rows = pl.ds(pl.multiple_of(t % (NL // 2) * ZPITCH, 8), FH // 2)
        for i, a in enumerate(_leaves(blocks, 2, _lhs_operands)):
            z2_s[i, t // (NL // 2), rows, :] = a

    def project(t):
        products = []
        for i in range(7):
            w = [win_s[W_PLAIN[i, b]] if (i, b) in W_PLAIN else wsum_s[i, b] for b in range(KT[i])]
            w = jnp.concatenate([pltpu.bitcast(x, BF16) for x in w], axis=1)
            products.append(lax.dot_general(w, h_s[i, :, :KT[i] * C], NT, preferred_element_type=F32))
        z = _assemble(_recombine(products, 2), 2)
        normalize(t - 1)
        gate_branch(z[:FH])
        z1_s[t] = z[FH:].astype(BF16)
        return products

    def prepare_w_out():
        tiles = [wout_s[j * C:(j + 1) * C, :].T.astype(F32) for j in range(FP // C)]
        blocks = {(i, p): [tiles[f][i * D // 4:(i + 1) * D // 4] for f in OUT_GROUPS[p]]
                  for i in range(4) for p in range(4)}
        for i, leaf in enumerate(_leaves(blocks, 4, _lhs_operands)):
            for j in range(KO[i]):
                woutt_s[i, j] = pltpu.bitcast(leaf[j].astype(BF16), U32)

    h0 = residual(0, qn_s[...]).astype(BF16)
    q_copies[1].wait()
    gate_branch(project_plain(1, h0))
    prepare(1)
    z1 = project_plain(0, h0)
    z1_s[0] = z1.astype(BF16)
    prepare_w_in(z1)

    @pl.loop(1, NL - 1)
    def _(t):
        pl.when(t == 1)(q_copies[2].wait)
        pl.when(t == 2)(q_copies[3].wait)
        project(t)
        prepare(t + 1)

    wait([wout_copy, wgate_copy, wsp_copy])
    prepare_w_out()
    project(NL - 1)
    normalize(NL - 1)
    silu_c = jnp.concatenate([sc_s[b] for b in range(NCB)], axis=1)
    mod_s[4] = 0.5 * jnp.dot(silu_c, wgate_s[...], preferred_element_type=F32)[0:8]

    def mix(u):
        hf = FH // 4

        w = wsp_s[pl.ds(pl.multiple_of(u * TB, TB), TB), :].astype(F32)

        def w_block(si, ti):
            cols = [(si % 2 * NL // 2 + t) * L + si // 2 * C for t in range(NL // 2)]
            return jnp.concatenate([w[ti * C:(ti + 1) * C, c:c + C] for c in cols], axis=1)

        def z_operand(i):
            return {(p, q): jnp.concatenate([z2_s[i, q, t * ZPITCH + p * hf:t * ZPITCH + (p + 1) * hf, :]
                                             for t in range(NL // 2)], axis=1)
                    for p in range(2) for q in range(2)}

        products = []
        for i, op in enumerate(_rhs_operands({(si, ti): w_block(si, ti)
                                             for si in range(4) for ti in range(4)}, 4)):
            products += [lax.dot_general(a, b, NT, preferred_element_type=F32) for a, b in zip(
                _leaves(z_operand(i), 2, _lhs_operands), _leaves(op, 2, _rhs_operands))]
        g = _assemble(_recombine(products, 4), 4)
        bias = jnp.concatenate([bias_s[pl.ds(u * (TB // C) + i, 1), :] for i in range(TB // C)], axis=1)
        z1 = jnp.concatenate([z1_s[u * (TB // L) + i] for i in range(TB // L)], axis=1).astype(F32)
        m_s[:FH, :] = _gelu2(z1) * (g + bias)

    def project_out(u, send):
        blocks = {(p, i): [m_s[f * C:(f + 1) * C, i * C:(i + 1) * C] for f in OUT_GROUPS[p]]
                  for i in range(4) for p in range(4)}
        o = _assemble(_recombine(
            [jnp.dot(jnp.concatenate([pltpu.bitcast(woutt_s[i, j], BF16) for j in range(KO[i])], axis=1),
                     jnp.concatenate(leaf[:KO[i]], axis=0).astype(BF16),
                     preferred_element_type=F32)
             for i, leaf in enumerate(_leaves(blocks, 4, _rhs_operands))], 4), 4)
        for i in range(TB // C):
            t = u * (TB // C) + i
            rows = pl.ds(pl.multiple_of(t * C, C), C)
            o_s[rows, :] = (x_s[rows, :] + mod(4, C) * o[:, i * C:(i + 1) * C].T).astype(BF16)
            if send:
                out_copy(t, C).start()

    mix(0)

    @pl.loop(1, NTB)
    def _(u):
        project_out(u - 1, False)
        mix(u)
        out_copy((u - 1) * (TB // C), TB).start()

    project_out(NTB - 1, True)
    wait([out_copy(u * (TB // C), TB) for u in range(NTB - 1)])
    wait([out_copy(t, C) for t in range(NC - TB // C, NC)])


@jax.jit
def pallas_adaLN_cond__ssm_conv_h3__mixer_gmlp__prompt_kernel(
    A_q: jax.Array,
    A_k: jax.Array,
    A_v: jax.Array,
    A_shift_k: jax.Array,
    A_ssm_k: jax.Array,
    A_ssm_D: jax.Array,
    B_x: jax.Array,
    B_w_in: jax.Array,
    B_w_sp: jax.Array,
    B_b_sp: jax.Array,
    B_w_out: jax.Array,
    c: jax.Array,
    w_mod: jax.Array,
):
    del B_x
    vm = pltpu.VMEM
    scratch = [
        vm((S, D), BF16), vm((NCB, KPAD + S // 2, C), U32), vm((NCB, S // 2, C), U32),
        vm((NCB * S // 2, C), U32), vm((2, NCB, FH // 2, C), U32), vm((S, S), BF16),
        vm((FP, D), BF16), vm((NCB, C, 5 * D), BF16), vm((D, D), BF16), vm((4 * C, C), U32),
        vm((D, C), F32), vm((NC * C // 2, C), U32), vm((NL, 2, D, C), F32), vm((NCB, L, C), F32),
        vm((len(KO), max(KO), D // 8, C), U32), vm((8, KH, FH // 2, C), U32), vm((S, D), F32),
        vm((L, D), F32), vm((7, C, KH * C), BF16), vm((FH, L), F32), vm((NL, FH, L), BF16),
        vm((7, 2, NL // 2 * ZPITCH, C), F32), vm((FP, TB), F32), vm((S, D), BF16),
        vm((2, 8, L), F32), vm((8, 8, D), F32), vm((8, 5 * D), F32), vm((NCB, 8, C), F32),
        vm((NC, C), F32), vm((NCB, 16, C), BF16), vm((4, D), BF16), vm((NCB, C), BF16),
        vm((NC, C), BF16), vm((1, D), BF16),
        pltpu.SemaphoreType.DMA((N_SEM,)), pltpu.SMEM((1,), jnp.int32),
    ]
    out = pl.pallas_call(
        _kernel,
        out_shape=jax.ShapeDtypeStruct((S, D), BF16),
        in_specs=[pl.BlockSpec(memory_space=pltpu.HBM)] * 12,
        out_specs=pl.BlockSpec(memory_space=pltpu.HBM),
        scratch_shapes=scratch,
        compiler_params=pltpu.CompilerParams(
            vmem_limit_bytes=120 * 2**20,
            flags={"XLA_TPU_EVENLY_DISTRIBUTE_CRITICAL_NODES": True}),
    )(A_q.reshape(S, D), A_k.reshape(S, D), A_v.reshape(S, D), A_shift_k.T,
      A_ssm_k.reshape(D // 8, 8, NC, C).transpose(0, 2, 1, 3).reshape(NCB * S, C),
      A_ssm_D.reshape(NCB, C), B_w_in.T, B_w_sp, B_b_sp.reshape(NC, C), B_w_out, c, w_mod)
    return out.reshape(1, S, D)
```

```python
import math

import jax
import jax.numpy as jnp
import numpy as np
from jax import lax
from jax.experimental import pallas as pl
from jax.experimental.pallas import tpu as pltpu

S, D, FH = 2048, 640, 864
EPS = 1e-5
C = 128
NC = S // C
L = 2 * C
NL = S // L
NCB = D // C
NG = C // 8
FP = 896
TB = 4 * C
NTB = S // TB
KPAD = 32
ZPITCH = FH // 2 + 16
KH = 3
KT = (3, 2, 3, 2, 2, 3, 3)
W_PLAIN = {(0, 2): (0, 2), (2, 2): (1, 2), (3, 0): (0, 3), (3, 1): (0, 4),
           (5, 0): (1, 0), (5, 1): (1, 1), (5, 2): (1, 2)}
OUT_GROUPS = [range(0, 2), range(2, 4), range(4, 6), range(6, 7)]

F32, BF16, U32 = jnp.float32, jnp.bfloat16, jnp.uint32
NT = (((1,), (1,)), ((), ()))


def _tree_sum(xs):
    xs = list(xs)
    while len(xs) > 1:
        xs = [xs[i] + xs[i + 1] if i + 1 < len(xs) else xs[i] for i in range(0, len(xs), 2)]
    return xs[0]


def _mix(x, y, sign):
    if isinstance(x, list):
        n = min(len(x), len(y))
        return ([_mix(p, q, sign) for p, q in zip(x, y)] + x[n:]
                + [q if sign > 0 else -q for q in y[n:]])
    return x + y if sign > 0 else x - y


def _add(x, y):
    return {k: _mix(x[k], y[k], 1) for k in x}


def _sub(x, y):
    return {k: _mix(x[k], y[k], -1) for k in x}


def _quadrants(x, n):
    h = n // 2
    return [{(i, j): x[i + a * h, j + b * h] for i in range(h) for j in range(h)}
            for a in range(2) for b in range(2)]


def _lhs_operands(a, n):
    a11, a12, a21, a22 = _quadrants(a, n)
    return [_add(a21, a22), _add(a11, a12), _add(a11, a22), a22, _sub(a12, a22), a11, _sub(a21, a11)]


def _rhs_operands(b, n):
    b11, b12, b21, b22 = _quadrants(b, n)
    return [b11, b22, _add(b11, b22), _sub(b11, b21), _add(b21, b22), _sub(b12, b22), _add(b11, b12)]


def _leaves(x, n, operands):
    if n == 1:
        return [x[0, 0]]
    return [leaf for op in operands(x, n) for leaf in _leaves(op, n // 2, operands)]


def _recombine(products, n):
    if n == 1:
        return {(0, 0): products[0]}
    k, h = len(products) // 7, n // 2
    m2, m5, m1, m4, m7, m3, m6 = (_recombine(products[i * k:(i + 1) * k], h) for i in range(7))
    quads = [_add(_sub(_sub(m1, m5), m4), m7), _add(m3, m5),
             _sub(m2, m4), _add(_add(_sub(m1, m2), m3), m6)]
    return {(i + q // 2 * h, j + q % 2 * h): v for q, c in enumerate(quads) for (i, j), v in c.items()}


def _assemble(blocks, n):
    return jnp.concatenate([jnp.concatenate([blocks[i, j] for j in range(n)], axis=1)
                            for i in range(n)], axis=0)


KO = [min(len(x), len(y)) for x, y in zip(
    _leaves({(i, p): list(OUT_GROUPS[p]) for i in range(4) for p in range(4)}, 4, _lhs_operands),
    _leaves({(p, i): list(OUT_GROUPS[p]) for i in range(4) for p in range(4)}, 4, _rhs_operands))]


def _low(w):
    return pltpu.bitcast(w << 16, F32)


def _high(w):
    return pltpu.bitcast(w & np.uint32(0xFFFF0000), F32)


def _pack(low, high):
    bits = pltpu.bitcast(jnp.concatenate([low, high], axis=1).astype(BF16).astype(F32), U32)
    return (bits[:, :C] >> 16) | bits[:, C:]


def _whole(ref, *index):
    return pltpu.bitcast(ref.bitcast(U32)[index], BF16)


def _gelu2(x):
    c = math.sqrt(2.0 / math.pi)
    return x * jnp.tanh((x * x * (c * 0.044715) + c) * x) + x


def _standardize(x):
    xc = x - jnp.sum(x, axis=-1, keepdims=True) * (1.0 / D)
    return xc * lax.rsqrt(jnp.sum(xc * xc, axis=-1, keepdims=True) * (1.0 / D) + EPS)


def _butterfly(a, b):
    return (a[0] + b[0], a[1] + b[1]), (a[0] - b[0], a[1] - b[1])


SEM_FIRST = 0
SEM_KV = SEM_FIRST + 1
SEM_SSMK = SEM_KV + NCB
SEM_MOD = SEM_SSMK + NCB
SEM_WIN = SEM_MOD + 2
SEM_Q = SEM_WIN + 2
SEM_LATE = SEM_Q + 2
SEM_OUT = SEM_LATE + 1
N_SEM = SEM_OUT + 1


def _kernel(q_hbm, k_hbm, v_hbm, shift_hbm, ssmk_hbm, ssmd_hbm, win_hbm, wsp_hbm, bsp_hbm,
            wout_hbm, c_hbm, wmod_hbm, out_hbm,
            q_s, k_s, v_s, ssmk_s, win_s, wsp_s, wout_s, wmod_s, wgate_s, dft_s,
            skip_s, kvt_s, yt_s, y_s, woutt_s, wsum_s, x_s, qn_s, h_s, gate_s, z1_s, z2_s, m_s, o_s,
            stat_s, mod_s, acc_s, taps_s, bias_s, sc_s, shift_s, ssmd_s, bsp_s, c_s,
            sems, spare_s):
    def copy(src, dst, i):
        return pltpu.make_async_copy(src, dst, sems.at[i])

    small = [copy(a, b, SEM_FIRST) for a, b in
             [(shift_hbm, shift_s), (ssmd_hbm, ssmd_s), (c_hbm, c_s), (bsp_hbm, bsp_s)]]

    def kv_first(i):
        rows = pl.ds(i * S // 2, S // 2)
        return [copy(k_hbm.at[rows, pl.ds(0, C)],
                     k_s.bitcast(BF16).at[0, pl.ds(2 * KPAD + i * S // 2, S // 2), :], SEM_FIRST + i),
                copy(v_hbm.at[rows, pl.ds(0, C)], v_s.bitcast(BF16).at[0, rows, :], SEM_FIRST + i)]

    def kv_copies(b):
        ch = pl.ds(pl.multiple_of(b * C, C), C)
        return [copy(k_hbm.at[:, ch], k_s.bitcast(BF16).at[b, pl.ds(2 * KPAD, S), :], SEM_KV + b),
                copy(v_hbm.at[:, ch], v_s.bitcast(BF16).at[b], SEM_KV + b)]

    def ssmk_copy(b):
        rows = pl.ds(pl.multiple_of(b * S, S), S)
        return copy(ssmk_hbm.at[rows, :], ssmk_s.bitcast(BF16).at[rows, :], SEM_SSMK + b)

    def wmod_copy(b):
        return copy(wmod_hbm.at[pl.ds(b * C, C), pl.ds(0, 5 * D)], wmod_s.at[b],
                    SEM_MOD + b // (NCB - 1))

    def win_copies(half):
        return [copy(win_hbm.at[pl.ds(half * FH, FH), pl.ds(b * C, C)],
                     win_s.at[half, b], SEM_WIN + half) for b in range(NCB)]

    wout_copy = copy(wout_hbm, wout_s.at[pl.ds(0, FH), :], SEM_LATE)
    wgate_copy = copy(wmod_hbm.at[:, pl.ds(5 * D, D)], wgate_s, SEM_LATE)

    wsp_copy = copy(wsp_hbm, wsp_s, SEM_LATE)

    def q_copy(t, n, sem):
        rows = pl.ds(t * L, n * L)
        return copy(q_hbm.at[rows, :], q_s.at[rows, :], sem)

    q_copies = [q_copy(0, 1, SEM_MOD), q_copy(1, 1, SEM_WIN + 1),
                q_copy(2, 1, SEM_Q), q_copy(3, NL - 3, SEM_Q + 1)]

    def out_copy(t, n):
        rows = pl.ds(pl.multiple_of(t * C, C), n)
        return pltpu.make_async_copy(o_s.at[rows, :], out_hbm.at[rows, :], sems.at[SEM_OUT])

    def wait(copies):
        for cp in copies:
            cp.wait()

    k_s[:, KPAD - 8:KPAD, :] = jnp.zeros((NCB, 8, C), U32)
    wout_s[FH:, :] = jnp.zeros((FP - FH, D), BF16)

    queue = small + kv_first(0) + kv_first(1)
    for b in range(NCB):
        queue += [ssmk_copy(b)] + (kv_copies(b + 1) if b + 1 < NCB else [])
    queue += q_copies[:1] + [wmod_copy(b) for b in range(NCB)]
    queue += win_copies(1) + q_copies[1:2] + win_copies(0) + q_copies[2:]
    queue += [wout_copy, wgate_copy, wsp_copy]
    for cp in queue:
        cp.start()

    def make_dft():
        def unit(turn):
            angle = (((turn + 2 * L) & (4 * L - 1)) - 2 * L).astype(F32) * (math.pi / (2 * L))
            return jnp.cos(angle), -jnp.sin(angle)

        sub, lane = (lax.broadcasted_iota(jnp.int32, (8, C), a) for a in range(2))
        blk, col = (lax.broadcasted_iota(jnp.int32, (C // 8, C), a) for a in range(2))
        forward_step = unit(8 * blk * (4 * col + 1))
        for p in range(2):
            sample = ((sub & 1) ^ p) * C + (sub & -2) + p
            for i, (first, step, scale) in enumerate([
                    (unit(sample * (4 * lane + 1)), forward_step, 1.0),
                    (unit((2 * lane + p) * (4 * sub + 1)), unit((2 * col + p) * 32 * blk), 1.0 / L)]):
                ar, ai = (jnp.concatenate([v * scale] * (C // 8), axis=0) for v in first)
                br, bi = (jnp.concatenate([jnp.broadcast_to(v[j:j + 1], (8, C)) for j in range(C // 8)],
                                          axis=0) for v in step)
                for c, w in enumerate([ar * br - ai * bi, ar * bi + ai * br]):
                    j = 4 * i + 2 * p + c
                    dft_s[j * C // 2:(j + 1) * C // 2, :] = pltpu.bitcast(w.astype(BF16), U32)

    def dft(i, n):
        return pltpu.bitcast(dft_s[i * C // 2:(i + n) * C // 2, :], BF16)

    def gate_chunk(b, m):
        kw = [k_s[b, pl.ds(KPAD + m * C + j, C), :] for j in range(-2, 1)]
        vw = v_s[b, m * C:(m + 1) * C, :]
        kk = [_high(kw[0]), _low(kw[1]), _high(kw[1]), _low(kw[2]), _high(kw[2])]
        for p, vv in enumerate((_low(vw), _high(vw))):
            kv = _tree_sum([kk[3 + p - t] * taps_s[b, t:t + 1, :] for t in range(4)]) * vv
            halves = [kv[:C // 2], kv[C // 2:]]
            tile = pltpu.bitcast(_pack(halves[p], halves[1 - p]), BF16)
            kvt_s[(2 * m + p) * 64:(2 * m + p + 1) * 64, :] = pltpu.bitcast(tile.T, U32)

    def forward(b, g):
        base = pl.multiple_of(b * (S // 2), S // 2) + g * NC * 4
        top = lax.broadcasted_iota(jnp.int32, (8, C), 0) < 4
        words = [ssmk_s[pl.ds(base + 4 * i, 8), :] if i % 4 < 3 else None for i in range(NC)]
        t0, t1 = [jnp.concatenate([jnp.where(top, words[i + j], words[i + j + 1])
                                   for i in range(0, NC, 4)], axis=0) for j in range(2)]
        odd = (lax.broadcasted_iota(jnp.int32, t0.shape, 1) & 1) == 1
        filt = [jnp.where(odd, pltpu.roll(t1, 1, 1), t0), jnp.where(odd, t0, pltpu.roll(t1, C - 1, 1))]
        out = []
        for p in range(2):
            sig = jnp.concatenate([jnp.where(top, kvt_s[pl.ds((2 * m + p) * 64 + 4 * g, 8), :],
                                             kvt_s[pl.ds((2 * m + 2 + p) * 64 + 4 * g - 4, 8), :])
                                   for m in range(0, NL, 2)], axis=0)
            lhs = jnp.concatenate([t[i:i + 8] for i in range(0, 4 * NL, 8) for t in (filt[p], sig)], axis=0)
            r = jnp.dot(pltpu.bitcast(lhs, BF16), jnp.concatenate([dft(2 * p, 1), dft(2 * p + 1, 1)], axis=1),
                        preferred_element_type=F32)
            out.append([r[:, :C], r[:, C:]])
        return out

    def product(b, g, f):
        def part(i, m, p):
            r = (m // 2 * 4 + i * 2 + m % 2) * 8
            return f[p][0][r:r + 8], f[p][1][r:r + 8]

        def window(m, p):
            re, im = part(0, m, p)
            if m:
                pre, pim = part(0, m - 1, p)
                return re - pim, im + pre
            if p == 0:
                re = re + skip_s[pl.ds(pl.multiple_of(b * C + g * 8, 8), 8), :]
            return re, im

        kf = [_butterfly(window(m, 0), window(m, 1)) for m in range(NL)]
        xf = [_butterfly(part(1, m, 0), part(1, m, 1)) for m in range(NL)]
        out = []
        for i in range(NL):
            z = []
            for h in range(2):
                terms = [(xf[j][h], kf[i - j][h]) for j in range(i + 1)]
                if i:
                    p1 = _tree_sum([x[0] * k[0] for x, k in terms])
                    p2 = _tree_sum([x[1] * k[1] for x, k in terms])
                    p3 = _tree_sum([(x[0] + x[1]) * (k[0] + k[1]) for x, k in terms])
                    z.append((p1 - p2, p3 - (p1 + p2)))
                else:
                    (x, k), = terms
                    z.append((x[0] * k[0] - x[1] * k[1], x[0] * k[1] + x[1] * k[0]))
            out.append(_butterfly(*z))
        return out

    def inverse(b, g, z):
        rows = pl.ds(pl.multiple_of(b * C + g * 8, 8), 8)
        for p in range(2):
            zp = jnp.concatenate([jnp.concatenate([z[i][p][c] for i in range(NL)], axis=0)
                                  for c in range(2)], axis=1)
            y = jnp.dot(zp.astype(BF16), dft(4 + 2 * p, 2), preferred_element_type=F32)
            for i in range(NL):
                yt_s[i, p, rows, :] = y[i * 8:(i + 1) * 8]

    def modulation(blocks):
        wait([wmod_copy(b) for b in blocks])
        acc_s[...] += _tree_sum([jnp.dot(sc_s[b], wmod_s[b], preferred_element_type=F32)[0:8]
                                 for b in blocks])

    def time_major(t, blocks):
        for b in blocks:
            for p in range(2):
                y_s[b, pl.ds(p, C, stride=2), :] = yt_s[t, p, b * C:(b + 1) * C, :].T

    def conv_block(b, last):
        ssmk_copy(b).wait()
        f = {0: forward(b, 0)}
        for g in range(NG):
            if g + 1 < NG:
                f[g + 1] = forward(b, g + 1)
            if g == 10 and not last:
                wait(kv_copies(b + 1))
            if g == 12 and last:
                q_copies[0].wait()
                modulation(range(NCB - 1))
                time_major(0, range(NCB - 1))
                qn_s[...] = _standardize(q_s[0:L, :].astype(F32))
            inverse(b, g, product(b, g, f.pop(g)))
        if last:
            time_major(0, [NCB - 1])
            modulation([NCB - 1])
        else:
            for m in range(NL):
                gate_chunk(b + 1, m)

    spare_s[0] = 7
    acc_s[...] = jnp.zeros(acc_s.shape, F32)
    m_s[FH:, :] = jnp.zeros((FP - FH, TB), F32)
    make_dft()
    wait(small + kv_first(0))
    taps = shift_s[...].astype(F32)
    for b in range(NCB):
        taps_s[b, 0:4, :] = taps[:, b * C:(b + 1) * C]
    skip = ssmd_s[...].astype(F32)
    cf = c_s[...].astype(F32)
    silu_c = jnp.broadcast_to(cf * jax.nn.sigmoid(cf), (16, D)).astype(BF16)
    for b in range(NCB):
        skip_s[b * C:(b + 1) * C, :] = jnp.broadcast_to(skip[b:b + 1], (C, C)).T
        sc_s[b] = silu_c[:, b * C:(b + 1) * C]
    bias_s[...] = bsp_s[...].astype(F32)
    for m in range(NL):
        if m == NL // 2:
            wait(kv_first(1))
        gate_chunk(0, m)

    pl.loop(0, NCB - 1)(lambda b: conv_block(b, False))
    conv_block(NCB - 1, True)

    sa, ca, ga, sb, cb = (acc_s[:, i * D:(i + 1) * D] for i in range(5))
    mod_s[0] = ga * (1.0 + ca)
    mod_s[1] = ga * sa
    mod_s[2] = 1.0 + cb
    mod_s[3] = sb

    def mod(i, n):
        return jnp.concatenate([mod_s[i]] * (n // 8), axis=0)

    def residual(t, qn=None):
        rows = pl.ds(pl.multiple_of(t * L, L), L)
        q = q_s[rows, :].astype(F32)
        y = jnp.concatenate([y_s[b] for b in range(NCB)], axis=1)
        x = q + ((_standardize(q) if qn is None else qn) * mod(0, L) + mod(1, L)) * y
        x_s[rows, :] = x
        return _standardize(x) * mod(2, L) + mod(3, L)

    def split(tiles):
        return tiles[:KH], tiles[KH:]

    def prepare(t):
        time_major(t, range(NCB))
        h = residual(t)
        blocks = {(i, j): split([h[j * C:(j + 1) * C, b * C:(b + 1) * C] for b in range(NCB)])[i]
                  for i in range(2) for j in range(2)}
        for i, tiles in enumerate(_leaves(blocks, 2, _rhs_operands)):
            h_s[i, :, :KT[i] * C] = jnp.concatenate(tiles[:KT[i]], axis=1).astype(BF16)

    def prepare_w_in(z):
        for r in range(0, FH, 16):
            wsum_s[spare_s[0], 0, 0:16, :] = z[r:r + 16, :C].astype(BF16)
            tiles = [[win_s[1 - i, b, r:r + 16, :].astype(F32) for b in range(NCB)] for i in range(2)]
            sums = _leaves({(i, j): split(tiles[i])[j] for i in range(2) for j in range(2)},
                           2, _lhs_operands)
            for i in range(7):
                for b in range(KT[i]):
                    if (i, b) not in W_PLAIN:
                        wsum_s[i, b, r:r + 16, :] = sums[i][b].astype(BF16)

    def project_plain(half, h):
        wait(win_copies(half))
        return jnp.concatenate([lax.dot_general(
            jnp.concatenate([_whole(win_s, half, b, pl.ds(r, FH // 4)) for b in range(NCB)],
                            axis=1), h, NT, preferred_element_type=F32) for r in (0, FH // 4)], axis=0)

    def gate_branch(z):
        z = _gelu2(z)
        z = z - z[0:1]
        gate_s[...] = z
        stat_s[0] = jnp.sum(z.reshape(FH // 8, 8, L), axis=0)
        stat_s[1] = jnp.sum((z * z).reshape(FH // 8, 8, L), axis=0)

    def normalize(t):
        mean = jnp.sum(stat_s[0], axis=0, keepdims=True) * (1.0 / FH)
        var = jnp.sum(stat_s[1], axis=0, keepdims=True) * (1.0 / FH) - mean * mean
        scale = lax.rsqrt(jnp.maximum(var, 0.0) + 4.0 * EPS)
        zn = (gate_s[...] - mean) * scale
        blocks = {(i, j): zn[i * FH // 2:(i + 1) * FH // 2, j * C:(j + 1) * C]
                  for i in range(2) for j in range(2)}
        rows = pl.ds(pl.multiple_of(t % (NL // 2) * ZPITCH, 8), FH // 2)
        for i, a in enumerate(_leaves(blocks, 2, _lhs_operands)):
            z2_s[i, t // (NL // 2), rows, :] = a

    def project(t):
        products = []
        for i in range(7):
            w = jnp.concatenate([_whole(win_s, *W_PLAIN[i, b]) if (i, b) in W_PLAIN else _whole(wsum_s, i, b)
                                 for b in range(KT[i])], axis=1)
            products.append(lax.dot_general(w, h_s[i, :, :KT[i] * C], NT, preferred_element_type=F32))
        z = _assemble(_recombine(products, 2), 2)
        normalize(t - 1)
        gate_branch(z[:FH])
        z1_s[t] = z[FH:].astype(BF16)

    def prepare_w_out():
        tiles = [wout_s[j * C:(j + 1) * C, :].T.astype(F32) for j in range(FP // C)]
        blocks = {(i, p): [tiles[f][i * D // 4:(i + 1) * D // 4] for f in OUT_GROUPS[p]]
                  for i in range(4) for p in range(4)}
        for i, leaf in enumerate(_leaves(blocks, 4, _lhs_operands)):
            for j in range(KO[i]):
                woutt_s[i, j] = leaf[j].astype(BF16)

    h0 = residual(0, qn_s[...]).astype(BF16)
    q_copies[1].wait()
    gate_branch(project_plain(1, h0))
    prepare(1)
    z1 = project_plain(0, h0)
    z1_s[0] = z1.astype(BF16)
    prepare_w_in(z1)

    @pl.loop(1, NL - 1)
    def _(t):
        pl.when(t == 1)(q_copies[2].wait)
        pl.when(t == 2)(q_copies[3].wait)
        project(t)
        prepare(t + 1)

    wait([wout_copy, wgate_copy, wsp_copy])
    prepare_w_out()
    project(NL - 1)
    normalize(NL - 1)
    silu_c = jnp.concatenate([sc_s[b] for b in range(NCB)], axis=1)
    mod_s[4] = 0.5 * jnp.dot(silu_c, wgate_s[...], preferred_element_type=F32)[0:8]

    def mix(u):
        hf = FH // 4

        w = wsp_s[pl.ds(pl.multiple_of(u * TB, TB), TB), :].astype(F32)

        def w_block(si, ti):
            cols = [(si % 2 * NL // 2 + t) * L + si // 2 * C for t in range(NL // 2)]
            return jnp.concatenate([w[ti * C:(ti + 1) * C, c:c + C] for c in cols], axis=1)

        def z_operand(i):
            return {(p, q): jnp.concatenate([z2_s[i, q, t * ZPITCH + p * hf:t * ZPITCH + (p + 1) * hf, :]
                                             for t in range(NL // 2)], axis=1)
                    for p in range(2) for q in range(2)}

        products = []
        for i, op in enumerate(_rhs_operands({(si, ti): w_block(si, ti)
                                             for si in range(4) for ti in range(4)}, 4)):
            products += [lax.dot_general(a, b, NT, preferred_element_type=F32) for a, b in zip(
                _leaves(z_operand(i), 2, _lhs_operands), _leaves(op, 2, _rhs_operands))]
        g = _assemble(_recombine(products, 4), 4)
        bias = jnp.concatenate([bias_s[pl.ds(u * (TB // C) + i, 1), :] for i in range(TB // C)], axis=1)
        z1 = jnp.concatenate([z1_s[u * (TB // L) + i] for i in range(TB // L)], axis=1).astype(F32)
        m_s[:FH, :] = _gelu2(z1) * (g + bias)

    def project_out(u, send):
        blocks = {(p, i): [m_s[f * C:(f + 1) * C, i * C:(i + 1) * C] for f in OUT_GROUPS[p]]
                  for i in range(4) for p in range(4)}
        o = _assemble(_recombine(
            [jnp.dot(jnp.concatenate([_whole(woutt_s, i, j) for j in range(KO[i])], axis=1),
                     jnp.concatenate(leaf[:KO[i]], axis=0).astype(BF16),
                     preferred_element_type=F32)
             for i, leaf in enumerate(_leaves(blocks, 4, _rhs_operands))], 4), 4)
        for i in range(TB // C):
            t = u * (TB // C) + i
            rows = pl.ds(pl.multiple_of(t * C, C), C)
            o_s[rows, :] = (x_s[rows, :] + mod(4, C) * o[:, i * C:(i + 1) * C].T).astype(BF16)
            if send:
                out_copy(t, C).start()

    mix(0)

    @pl.loop(1, NTB)
    def _(u):
        project_out(u - 1, False)
        mix(u)
        out_copy((u - 1) * (TB // C), TB).start()

    project_out(NTB - 1, True)
    wait([out_copy(u * (TB // C), TB) for u in range(NTB - 1)])
    wait([out_copy(t, C) for t in range(NC - TB // C, NC)])


@jax.jit
def pallas_adaLN_cond__ssm_conv_h3__mixer_gmlp__prompt_kernel(
    A_q: jax.Array,
    A_k: jax.Array,
    A_v: jax.Array,
    A_shift_k: jax.Array,
    A_ssm_k: jax.Array,
    A_ssm_D: jax.Array,
    B_x: jax.Array,
    B_w_in: jax.Array,
    B_w_sp: jax.Array,
    B_b_sp: jax.Array,
    B_w_out: jax.Array,
    c: jax.Array,
    w_mod: jax.Array,
):
    del B_x
    vm = pltpu.VMEM
    scratch = [
        vm((S, D), BF16), vm((NCB, KPAD + S // 2, C), U32), vm((NCB, S // 2, C), U32),
        vm((NCB * S // 2, C), U32), vm((2, NCB, FH, C), BF16), vm((S, S), BF16),
        vm((FP, D), BF16), vm((NCB, C, 5 * D), BF16), vm((D, D), BF16), vm((4 * C, C), U32),
        vm((D, C), F32), vm((NC * C // 2, C), U32), vm((NL, 2, D, C), F32), vm((NCB, L, C), F32),
        vm((len(KO), max(KO), D // 4, C), BF16), vm((8, KH, FH, C), BF16), vm((S, D), F32),
        vm((L, D), F32), vm((7, C, KH * C), BF16), vm((FH, L), F32), vm((NL, FH, L), BF16),
        vm((7, 2, NL // 2 * ZPITCH, C), F32), vm((FP, TB), F32), vm((S, D), BF16),
        vm((2, 8, L), F32), vm((8, 8, D), F32), vm((8, 5 * D), F32), vm((NCB, 8, C), F32),
        vm((NC, C), F32), vm((NCB, 16, C), BF16), vm((4, D), BF16), vm((NCB, C), BF16),
        vm((NC, C), BF16), vm((1, D), BF16),
        pltpu.SemaphoreType.DMA((N_SEM,)), pltpu.SMEM((1,), jnp.int32),
    ]
    out = pl.pallas_call(
        _kernel,
        out_shape=jax.ShapeDtypeStruct((S, D), BF16),
        in_specs=[pl.BlockSpec(memory_space=pltpu.HBM)] * 12,
        out_specs=pl.BlockSpec(memory_space=pltpu.HBM),
        scratch_shapes=scratch,
        compiler_params=pltpu.CompilerParams(
            vmem_limit_bytes=120 * 2**20,
            flags={"XLA_TPU_EVENLY_DISTRIBUTE_CRITICAL_NODES": True}),
    )(A_q.reshape(S, D), A_k.reshape(S, D), A_v.reshape(S, D), A_shift_k.T,
      A_ssm_k.reshape(D // 8, 8, NC, C).transpose(0, 2, 1, 3).reshape(NCB * S, C),
      A_ssm_D.reshape(NCB, C), B_w_in.T, B_w_sp, B_b_sp.reshape(NC, C), B_w_out, c, w_mod)
    return out.reshape(1, S, D)
```
